```python
import jax
import jax.numpy as jnp

def _softmax(x, axis=-1):
    return jax.nn.softmax(x, axis=axis)
def _gelu(x):
    return jax.nn.gelu(x, approximate=True)
def _silu(x):
    return jax.nn.silu(x)
def _sigmoid(x):
    return jax.nn.sigmoid(x)
def _layernorm(x, axis=-1, eps=1e-5):
    m = jnp.mean(x, axis=axis, keepdims=True)
    v = jnp.var(x, axis=axis, keepdims=True)
    return (x - m) / jnp.sqrt(v + eps)
def _scatter_add(tgt, idx, src, axis=0):
    return tgt.at[idx].add(src)
def _segment_sum(src, seg, n):
    return jax.ops.segment_sum(src, seg, n)
class _Rng:
    def __init__(self, key):
        self._k = key
    def _next(self):
        self._k, sub = jax.random.split(self._k)
        return sub
    def normal(self, shape):
        return jax.random.normal(self._next(), shape, dtype=jnp.bfloat16)
    def randint(self, lo, hi, shape):
        return jax.random.randint(self._next(), shape, lo, hi, dtype=jnp.int32)
    def uniform(self, shape, lo=0.0, hi=1.0):
        return jax.random.uniform(self._next(), shape, jnp.bfloat16, lo, hi)
    def permutation(self, n):
        return jax.random.permutation(self._next(), n)


kernel_name = 'parallel_sum__sliding_local_dilated__glu_gated_bilinear__prompt'

def setup_inputs():
    _rng = _Rng(jax.random.key(int.from_bytes(__import__("os").urandom(4), "little")))
    _w = (lambda a: (lambda t: t.astype(jnp.bfloat16) if jnp.issubdtype(t.dtype, jnp.floating) else t)(jnp.asarray(a)))
    def _A_setup():
        B, S, D = 1, 2048, 1024
        return {
            "x": _w((lambda *s: _rng.normal(s) * 0.05)(B, S, D)),
            "wqkv": _w((lambda *s: _rng.normal(s) * 0.05)(D, 3 * D)),
            "wo": _w((lambda *s: _rng.normal(s) * 0.05)(D, D)),
        }
    _A_in = _A_setup()

    def _B_setup():
        B, S, D, F = 1, 2048, 1024, 3584
        return {
            "x": _w((lambda *s: _rng.normal(s) * 0.05)(B, S, D)),
            "w_gate": _w((lambda *s: _rng.normal(s) * 0.05)(D, F) * (D ** -0.5)),
            "w_up": _w((lambda *s: _rng.normal(s) * 0.05)(D, F) * (D ** -0.5)),
            "w_down": _w((lambda *s: _rng.normal(s) * 0.05)(F, D) * (F ** -0.5)),
        }
    _B_in = _B_setup()

    return {
        "A_x": _A_in["x"],
        "A_wqkv": _A_in["wqkv"],
        "A_wo": _A_in["wo"],
        "B_x": _B_in["x"],
        "B_w_gate": _B_in["w_gate"],
        "B_w_up": _B_in["w_up"],
        "B_w_down": _B_in["w_down"],
    }

def reference(A_x, A_wqkv, A_wo, B_x, B_w_gate, B_w_up, B_w_down):
    def _A_ref(x, wqkv, wo):
        B, S, D = x.shape
        H = 32; Dh = D // H
        W, dil = 8, 2
        qkv = (lambda x, *d: x.transpose(*d))((x @ wqkv).reshape(B, S, 3, H, Dh), 2, 0, 3, 1, 4)
        q, k, v = qkv[0], qkv[1], qkv[2]
        scale = Dh ** -0.5
        pos = jnp.arange(S)
        off = jnp.arange(W) * dil
        idx = pos[:, None] - off[None, :]
        mask = idx >= 0
        idx_c = jnp.where(mask, idx, 0).reshape(-1)
        kg = k[:, :, idx_c, :].reshape(B, H, S, W, Dh)
        vg = v[:, :, idx_c, :].reshape(B, H, S, W, Dh)
        logits = jnp.einsum("bhsd,bhswd->bhsw", q, kg) * scale
        logits = jnp.where(mask[None, None, :, :], logits, -1e9)
        attn = _softmax(logits, axis=-1)
        o = jnp.einsum("bhsw,bhswd->bhsd", attn, vg)
        return (lambda x, *d: x.transpose(*d))(o, 0, 2, 1, 3).reshape(B, S, D) @ wo

    def _B_ref(x, w_gate, w_up, w_down):
        g = jnp.einsum("bsd,df->bsf", x, w_gate)
        u = jnp.einsum("bsd,df->bsf", x, w_up)
        h = g * u
        return jnp.einsum("bsf,fd->bsd", h, w_down)

    x = A_x
    xn = _layernorm(x, axis=-1)
    return x + _A_ref(xn, A_wqkv, A_wo) + _B_ref(xn, B_w_gate, B_w_up, B_w_down)
```

```python
import functools
import numpy as np
import jax
import jax.numpy as jnp
import jax.experimental.pallas as pl
import jax.experimental.pallas.tpu as pltpu

S, D, F = 2048, 1024, 3584
H, DH, W, DIL = 32, 32, 8, 2
HALO = 16
SH, DHF = S // 2, D // 2
FC = 512
NCH = F // FC
P_QKV = 512
P_FFN = 512
P_OUT = 256
SUB = 1
RG = 16
F32, BF16, U32 = jnp.float32, jnp.bfloat16, jnp.uint32


def _pk(x):
    return pltpu.bitcast(x.astype(BF16), U32)


def _unpk(x):
    return pltpu.bitcast(x, BF16)


def _skew(vs, axis, unit):
    n = len(vs)
    size = vs[0].shape[axis]
    g = jax.lax.broadcasted_iota(jnp.int32, vs[0].shape, axis) // unit
    r = [v if j == 0 else pltpu.roll(v, unit * j, axis) for j, v in enumerate(vs)]
    cur = [r[(-t) % n] for t in range(n)]
    b = 1
    while b < n:
        m = (g & b) != 0
        cur = [jnp.where(m, cur[(t - b) % n], cur[t]) for t in range(n)]
        b *= 2
    return [c if t == 0 else pltpu.roll(c, size - unit * t, axis) for t, c in enumerate(cur)]


def _lhs_ops(a11, a12, a21, a22):
    return [_pk(v) for v in (a11 + a22, a21 + a22, a11, a22, a11 + a12, a21 - a11, a12 - a22)]


def _rhs_ops(b11, b12, b21, b22):
    f11, f12, f21, f22 = (_unpk(v).astype(F32) for v in (b11, b12, b21, b22))
    return [_pk(f11 + f22), b11, _pk(f12 - f22), _pk(f21 - f11), b22, _pk(f11 + f12), _pk(f21 + f22)]


def _combine(m):
    m1, m2, m3, m4, m5, m6, m7 = m
    return (m1 + m4 - m5 + m7, m3 + m5, m2 + m4, m1 - m2 + m3 + m6)


def _rows(start, n):
    return pl.ds(start if isinstance(start, int) else pl.multiple_of(start, 16), n)


def _words(start, n):
    return pl.ds(start // 2 if isinstance(start, int) else pl.multiple_of(start >> 1, 8), n // 2)


def _mm(a, b):
    return jnp.dot(_unpk(a), _unpk(b), preferred_element_type=F32)


def _kernel(x_hbm, wqkv_hbm, wo_hbm, wg_hbm, wu_hbm, wd_hbm, o_hbm,
            x_v, wsq_v, wg_v, wu_v, wd_v, a_s, b1_s, b2_s, bo_s, h_s, acc_s, q_s, k_s, v_s, t_s, ao_s,
            sem_x, sem_sq, sem_f, sem_o):
    XB = 256

    def x_copies(b):
        return [pltpu.make_async_copy(x_hbm.at[pl.ds(hf * SH + b * XB, XB)], x_v.at[pl.ds(hf * SH + b * XB, XB)],
                                      sem_x.at[2 * b + hf]) for hf in range(2)]

    def sq_copy(i):
        src = wo_hbm if i == 3 else wqkv_hbm.at[:, pl.ds((1, 0, 2)[i] * D, D)]
        return pltpu.make_async_copy(src, wsq_v.at[i], sem_sq.at[i])

    def f_copies(c):
        s = c % 2
        col = pl.ds(pl.multiple_of(c * FC, FC), FC)
        return [pltpu.make_async_copy(wg_hbm.at[:, col], wg_v.at[s], sem_f.at[3 * s]),
                pltpu.make_async_copy(wu_hbm.at[:, col], wu_v.at[s], sem_f.at[3 * s + 1]),
                pltpu.make_async_copy(wd_hbm.at[col, :], wd_v.at[s], sem_f.at[3 * s + 2])]

    def ln(p, n):
        hs = []
        for hf in range(2):
            x = x_v[pl.ds(hf * SH + p, n), :].astype(F32)
            xc = x - jnp.mean(x, axis=-1, keepdims=True)
            xn = xc * jax.lax.rsqrt(jnp.mean(xc * xc, axis=-1, keepdims=True) + 1e-5)
            hs += [xn[:, :DHF], xn[:, DHF:]]
        for i, v in enumerate(_lhs_ops(*hs)):
            a_s[i, _words(p, n), :] = v

    def prep_qkv(i, slot, k, n):
        th = [_skew([pltpu.bitcast(wsq_v[i, pl.ds(hf * DHF + k, n), pl.ds(j * 128, 128)], U32) for j in range(8)], 1, 4)
              for hf in range(2)]
        for t in range(4):
            for m, v in enumerate(_rhs_ops(th[0][t], th[0][t + 4], th[1][t], th[1][t + 4])):
                b1_s[slot, m, _words(k, n), pl.ds(t * 128, 128)] = v

    def prep_wo(hl, jh):
        base = hl * 32
        res = []
        for th in range(2):
            res.append(_skew([pltpu.bitcast(wsq_v[3, _rows((jh * 4 + jl) * 128 + base + th * 16, 16), :], U32)
                              for jl in range(4)], 0, 2))
        for tl in range(4):
            lo, hi = res[0][tl], res[1][tl]
            for m, v in enumerate(_rhs_ops(lo[:, :DHF], lo[:, DHF:], hi[:, :DHF], hi[:, DHF:])):
                bo_s[m, _words(tl * 128 + base + jh * 16, 16), :] = v

    def prep_gu(s, slot, k, n):
        for off, w in ((0, wg_v), (FC // 2, wu_v)):
            lo = pltpu.bitcast(w[s, pl.ds(k, n), :], U32)
            hi = pltpu.bitcast(w[s, pl.ds(DHF + k, n), :], U32)
            for m, v in enumerate(_rhs_ops(lo[:, :FC // 2], lo[:, FC // 2:], hi[:, :FC // 2], hi[:, FC // 2:])):
                b1_s[slot, m, _words(k, n), pl.ds(off, FC // 2)] = v

    def prep_d(s, slot, k, n):
        lo = pltpu.bitcast(wd_v[s, pl.ds(k, n), :], U32)
        hi = pltpu.bitcast(wd_v[s, pl.ds(FC // 2 + k, n), :], U32)
        for m, v in enumerate(_rhs_ops(lo[:, :DHF], lo[:, DHF:], hi[:, :DHF], hi[:, DHF:])):
            b2_s[slot, m, _words(k, n), :] = v

    def spread(items, n):
        return [items[(len(items) * i) // n:(len(items) * (i + 1)) // n] for i in range(n)]

    def run(fs):
        for f in fs:
            f()

    def stage1(slot, p, n, side):
        ms = []
        for m, fs in enumerate(spread(side, 7)):
            ms.append(_mm(a_s[m, _words(p, n), :], b1_s[slot, m]))
            run(fs)
        return _combine(ms)

    for b in range(SH // XB):
        for cp in x_copies(b):
            cp.start()
        if b == 0:
            sq_copy(0).start()
    sq_copy(1).start()
    k_s[:, pl.ds(0, HALO), :] = jnp.zeros((8, HALO, 128), F32)

    def zero(i, c):
        acc_s[:, pl.ds(pl.multiple_of(i * 64, 64), 64), :] = jnp.zeros((7, 64, DHF), F32)
        return c
    jax.lax.fori_loop(0, SH // 64, zero, 0)

    for b in range(SH // XB):
        for cp in x_copies(b):
            cp.wait()

        def body(i, c, b=b):
            p = pl.multiple_of(b * XB + i * 64, 64)
            for r in range(0, 64, 16):
                ln(p + r, 16)
            return c
        jax.lax.fori_loop(0, XB // 64, body, 0)
        if b == 0:
            sq_copy(0).wait()

            def body(i, c):
                k = pl.multiple_of(i * 64, 64)
                for r in range(0, 64, 16):
                    prep_qkv(0, 1, k + r, 16)
                return c
            jax.lax.fori_loop(0, DHF // 64, body, 0)

    nq = SH // P_QKV
    for u, (dst, off) in enumerate(((k_s, HALO), (q_s, 0), (v_s, HALO))):
        if u == 0:
            sq_copy(2).start()
            sq_copy(1).wait()
        elif u == 1:
            for cp in f_copies(0):
                cp.start()
            sq_copy(3).start()
            sq_copy(2).wait()
        else:
            for cp in f_copies(1):
                cp.start()
            for cp in f_copies(0):
                cp.wait()
            sq_copy(3).wait()

        def body(b, c, u=u, dst=dst, off=off):
            p = pl.multiple_of(b * P_QKV, P_QKV)
            kk = DHF // nq
            k0 = pl.multiple_of(b * kk, kk)
            if u < 2:
                side = [functools.partial(prep_qkv, u + 1, u % 2, k0 + r, 16) for r in range(0, kk, 16)]
            else:
                k1 = pl.multiple_of(b * (kk // 2), kk // 2)
                side = [functools.partial(prep_gu, 0, 0, k0 + r, 16) for r in range(0, kk, 16)]
                side += [functools.partial(prep_d, 0, 0, k1 + r, 16) for r in range(0, kk // 2, 16)]
                side += [functools.partial(prep_wo, b * (4 // nq) + i, jh) for i in range(4 // nq) for jh in range(2)]
            cs = stage1((u + 1) % 2, p, P_QKV, side)
            for i, val in enumerate(cs):
                for t in range(4):
                    dst[(i % 2) * 4 + t, pl.ds(off + (i // 2) * SH + p, P_QKV), :] = val[:, t * 128:(t + 1) * 128]
            return c
        jax.lax.fori_loop(0, nq, body, 0)

    for t in range(8):
        v_s[t, pl.ds(0, HALO), :] = jnp.broadcast_to(v_s[t, pl.ds(HALO, 1), :], (HALO, 128))

    scale = DH ** -0.5

    def attend(p, hf):
        lane = jax.lax.broadcasted_iota(jnp.int32, (RG, 128), 1)
        row = jax.lax.broadcasted_iota(jnp.int32, (RG, 128), 0)
        r = hf * SH + p
        q = [q_s[t, pl.ds(r, RG), :] for t in range(8)]
        ls = []
        for w in range(W):
            acc = None
            for t in range(8):
                y = q[t] * k_s[t, pl.ds(r + (HALO - DIL * w), RG), :]
                acc = y if acc is None else acc + y
            acc = acc + jnp.take_along_axis(acc, lane ^ 1, axis=1)
            acc = acc + jnp.take_along_axis(acc, lane ^ 2, axis=1)
            acc = acc * scale
            if hf == 0 and w > 0:
                acc = jnp.where(r + row >= DIL * w, acc, -1e9)
            ls.append(acc)
        mx = functools.reduce(jnp.maximum, ls)
        es = [jnp.exp(l - mx) for l in ls]
        inv = 1.0 / functools.reduce(jnp.add, es)
        ps = [e * inv for e in es]
        for t in range(8):
            acc = None
            for w in range(W):
                y = ps[w] * v_s[t, pl.ds(r + (HALO - DIL * w), RG), :]
                acc = y if acc is None else acc + y
            t_s[hf, t] = acc

    def attend_pack(p):
        for t in range(4):
            for m, v in enumerate(_lhs_ops(t_s[0, t], t_s[0, t + 4], t_s[1, t], t_s[1, t + 4])):
                ao_s[m, _words(p, RG), pl.ds(t * 128, 128)] = v

    nf = SH // P_FFN
    ngroups = SH // RG
    per = -(-ngroups // (NCH * nf))
    PS = P_FFN // SUB

    def ffn_chunk(c, carry):
        nxt = jnp.minimum(c + 1, NCH - 1)

        @pl.when(c + 1 < NCH)
        def _():
            for cp in f_copies(c + 1):
                cp.wait()

        @pl.when(c + 2 < NCH)
        def _():
            for cp in f_copies(c + 2):
                cp.start()

        def body(b, carry):
            slot = c % 2
            kk = DHF // nf
            k0 = pl.multiple_of(b * kk, kk)
            k1 = pl.multiple_of(b * (kk // 2), kk // 2)
            prep = [functools.partial(prep_gu, nxt % 2, 1 - slot, k0 + r, 16) for r in range(0, kk, 16)]
            prep += [functools.partial(prep_d, nxt % 2, 1 - slot, k1 + r, 16) for r in range(0, kk // 2, 16)]
            att = []
            for i in range(per):
                pa = pl.multiple_of(jnp.minimum((c * nf + b) * per + i, ngroups - 1) * RG, RG)
                att += [functools.partial(attend, pa, 0), functools.partial(attend, pa, 1),
                        functools.partial(attend_pack, pa)]
            att = spread(att, SUB)
            prep = spread(prep, SUB)
            p0 = pl.multiple_of(b * P_FFN, P_FFN)
            for s in range(SUB):
                cs = stage1(slot, p0 + s * PS, PS, att[s])
                hs = [v[:, :FC // 2] * v[:, FC // 2:] for v in cs]
                for m, v in enumerate(_lhs_ops(*hs)):
                    h_s[s, m] = v
            for s in range(SUB):
                sp = spread(prep[s], 7)
                for j, m in enumerate((1, 2, 4, 3, 5, 6, 0)):
                    acc_s[m, pl.ds(p0 + s * PS, PS), :] += _mm(h_s[s, m], b2_s[slot, m])
                    run(sp[j])
            return carry
        jax.lax.fori_loop(0, nf, body, 0)
        return carry
    jax.lax.fori_loop(0, NCH, ffn_chunk, 0)

    no = SH // P_OUT

    def o_copies(b):
        return [pltpu.make_async_copy(x_v.at[pl.ds(hf * SH + b * P_OUT, P_OUT)],
                                      o_hbm.at[pl.ds(hf * SH + b * P_OUT, P_OUT)], sem_o.at[2 * b + hf]) for hf in range(2)]

    def body(b, c):
        p = pl.multiple_of(b * P_OUT, P_OUT)
        ms = [acc_s[m, pl.ds(p, P_OUT), :] + _mm(ao_s[m, _words(p, P_OUT), :], bo_s[m]) for m in range(7)]
        for i, val in enumerate(_combine(ms)):
            idx = (pl.ds((i // 2) * SH + p, P_OUT), pl.ds((i % 2) * DHF, DHF))
            x_v[idx] = (x_v[idx].astype(F32) + val).astype(BF16)
        for cp in o_copies(b):
            cp.start()
        return c
    jax.lax.fori_loop(0, no, body, 0)
    for b in range(no):
        for cp in o_copies(b):
            cp.wait()


@jax.jit
def pallas_parallel_sum__sliding_local_dilated__glu_gated_bilinear__prompt_kernel(A_x, A_wqkv, A_wo, B_x, B_w_gate, B_w_up, B_w_down):
    x = A_x.reshape(S, D)
    hbm = pl.BlockSpec(memory_space=pl.ANY)
    V = pltpu.VMEM
    out = pl.pallas_call(
        _kernel,
        in_specs=[hbm] * 6,
        out_specs=hbm,
        out_shape=jax.ShapeDtypeStruct((S, D), BF16),
        scratch_shapes=[
            V((S, D), BF16), V((4, D, D), BF16), V((2, D, FC), BF16), V((2, D, FC), BF16), V((2, FC, D), BF16),
            V((7, SH // 2, DHF), U32), V((2, 7, DHF // 2, FC), U32), V((2, 7, FC // 4, DHF), U32),
            V((7, DHF // 2, DHF), U32), V((SUB, 7, P_FFN // SUB // 2, FC // 2), U32), V((7, SH, DHF), F32),
            V((8, S, 128), F32), V((8, S + HALO, 128), F32), V((8, S + HALO, 128), F32), V((2, 8, RG, 128), F32),
            V((7, SH // 2, DHF), U32),
            pltpu.SemaphoreType.DMA((8,)), pltpu.SemaphoreType.DMA((4,)), pltpu.SemaphoreType.DMA((6,)),
            pltpu.SemaphoreType.DMA((2 * SH // P_OUT,)),
        ],
        compiler_params=pltpu.CompilerParams(vmem_limit_bytes=120 * 2**20),
        name="fused",
    )(x, A_wqkv, A_wo, B_w_gate, B_w_up, B_w_down)
    return out.reshape(A_x.shape)
```

```python
import functools
import jax
import jax.numpy as jnp
import jax.experimental.pallas as pl
import jax.experimental.pallas.tpu as pltpu

E = lambda k, d: d
S, D, F = 2048, 1024, 3584
DH, W, DIL = 32, 8, 2
HALO = 16
SH, DHF = S // 2, D // 2
FC = 512
NCH = F // FC
XB = 128
P = 512
P_OUT = E("P_OUT", 256)
R_OUT = E("R_OUT", 128)
AG = E("AG", 2)
F32, BF16, U32 = jnp.float32, jnp.bfloat16, jnp.uint32
K_, Q_, V_, O_, GU_, DN_ = 0, 1, 2, 3, 4, 6


def _ds(start, n, align):
    return pl.ds(start if isinstance(start, int) else pl.multiple_of(start, align), n)


def _rows(start, n):
    return _ds(start, n, 16)


def _skew4(vs, pos, unit):
    cur = [vs[(-t) % 4] for t in range(4)]
    for b in (1, 2):
        m = (pos & (b * unit)) != 0
        cur = [jnp.where(m, cur[(t - b) % 4], cur[t]) for t in range(4)]
    return cur


def _perm_lanes(vs):
    lane = jax.lax.broadcasted_iota(jnp.int32, vs[0].shape, 1)
    lo, hi = _skew4(vs[:4], lane, 4), _skew4(vs[4:], lane, 4)
    m = (lane & 16) != 0
    mixed = [jnp.where(m, b, a) for a, b in zip(lo, hi)] + [jnp.where(m, a, b) for a, b in zip(lo, hi)]
    return [v if t == 0 else
            jnp.take_along_axis(v, ((lane & 115) ^ (t // 4 * 16)) | ((lane + t % 4 * 4) & 12), axis=1)
            for t, v in enumerate(mixed)]


def _perm_words(vs):
    row = jax.lax.broadcasted_iota(jnp.int32, vs[0].shape, 0)
    return [v if t == 0 else pltpu.roll(v, 8 - 2 * t, 0) for t, v in enumerate(_skew4(vs, row, 2))]


def _lhs_ops(a11, a12, a21, a22):
    return (a11 + a22, a21 + a22, a11, a22, a11 + a12, a21 - a11, a12 - a22)


def _rhs_ops(b11, b12, b21, b22):
    f11, f12, f21, f22 = (v.astype(F32) for v in (b11, b12, b21, b22))
    return (f11 + f22, f11, f12 - f22, f21 - f11, f22, f11 + f12, f21 + f22)


def _combine(m):
    m1, m2, m3, m4, m5, m6, m7 = m
    return (m1 + m4 - m5 + m7, m3 + m5, m2 + m4, m1 - m2 + m3 + m6)


def _mm(a, b):
    cat = lambda v: v[0] if len(v) == 1 else jnp.concatenate(v, axis=1)
    return jnp.dot(cat(a), cat(b), preferred_element_type=F32)


def _merge(*lists):
    keyed = []
    for xs in lists:
        tot, done = sum(w for w, _ in xs), 0
        for w, f in xs:
            keyed.append(((done + w / 2) / tot, w, f))
            done += w
    return [(w, f) for _, w, f in sorted(keyed, key=lambda t: t[0])]


def _pipeline(jobs, dist):
    n, out = len(jobs[0]), []
    for i in range(len(jobs) + (n - 1) * dist):
        for st in range(n):
            if 0 <= i - st * dist < len(jobs):
                out += jobs[i - st * dist][st]
    return out


def _interleave(dots, side, lag=0):
    tot, share = sum(w for w, _ in side), sum(w for w, _ in dots)
    outs, done, j, cum = [], 0, 0, 0
    for i, (_, dot) in enumerate(dots):
        outs.append(dot())
        if i < lag:
            continue
        src = outs[i - lag]
        lo = tot * cum / share
        cum += dots[i - lag][0]
        hi = tot * cum / share
        while j < len(side) and done < hi - 1e-6:
            pos = min(max((done - lo) / (hi - lo), 0.0), 0.999) * (src.shape[1] // 128)
            r0, c0 = int(pos % 1 * src.shape[0]) // 8 * 8, int(pos) * 128
            side[j][1](src[r0:r0 + 8, c0:c0 + 128])
            done += side[j][0]
            j += 1
    assert j == len(side)


def _kernel(x_hbm, wqkv_hbm, wo_hbm, wg_hbm, wu_hbm, wd_hbm, o_hbm,
            x_v, w_v, a_s, b1_s, g1_s, b2_s, bo_s, h_s, acc_s, qkv_s, t_s, ao_s,
            sem_x, sem_k, sem_w, sem_f, sem_o):
    part = functools.partial
    count = [0, 0]

    def zero():
        count[0] += 1
        return jax.lax.shift_right_logical(count[1] + count[0], 24) * 16

    def tie_x(tok):
        if tok is not None:
            x_v[0, _rows(zero() + SH, 16), pl.ds(0, 128)] = pltpu.bitcast(tok, BF16)

    def tie_w(tok):
        if tok is not None:
            w_v[0, 0, _rows(zero() + DHF, 16), pl.ds(0, 128)] = pltpu.bitcast(tok, BF16)

    def tie_qkv(tok):
        qkv_s[0, 0, _ds(zero() + S + HALO, 8, 8), :] = tok

    def x_copy(b):
        return pltpu.make_async_copy(x_hbm.at[:, pl.ds(b * XB, XB)], x_v.at[:, pl.ds(b * XB, XB)], sem_x.at[b])

    def k_copy(s):
        return pltpu.make_async_copy(wqkv_hbm.at[:, _rows(s * 128, 128), pl.ds(D, D)],
                                     w_v.at[K_, :, _rows(s * 128, 128)], sem_k.at[s])

    def w_copy(i):
        src = wo_hbm if i == O_ else wqkv_hbm.at[:, :, pl.ds(0 if i == Q_ else 2 * D, D)]
        return pltpu.make_async_copy(src, w_v.at[i, :, pl.ds(0, DHF)], sem_w.at[i])

    def f_copies(c):
        s = c % 2
        col = _ds(c * FC, FC, FC)
        return [pltpu.make_async_copy(wg_hbm.at[:, :, col], w_v.at[GU_ + s, :, pl.ds(0, DHF), pl.ds(0, FC)], sem_f.at[3 * s]),
                pltpu.make_async_copy(wu_hbm.at[:, :, col], w_v.at[GU_ + s, :, pl.ds(0, DHF), pl.ds(FC, FC)], sem_f.at[3 * s + 1]),
                pltpu.make_async_copy(wd_hbm.at[col, :], w_v.at[DN_, s, pl.ds(0, DHF)], sem_f.at[3 * s + 2])]

    def o_copy(i):
        rows = _ds(i * R_OUT, R_OUT, R_OUT)
        return pltpu.make_async_copy(x_v.at[:, rows], o_hbm.at[:, rows], sem_o.at[i])

    def row_mean(x):
        y = functools.reduce(jnp.add, [x[:, c:c + 128] for c in range(0, D, 128)])
        return jnp.sum(y, axis=-1, keepdims=True) * (1.0 / D)

    def ln_stats(st, p, hf, tok):
        tie_x(tok)
        x = x_v[hf, _rows(p, 16), :].astype(F32)
        mu = row_mean(x)
        xc = x - mu
        st[hf] = (mu, jax.lax.rsqrt(row_mean(xc * xc) + 1e-5))

    def ln_apply(st, p, t, tok):
        tie_x(tok)
        qs = [(x_v[hf, _rows(p, 16), pl.ds(c + t * 128, 128)].astype(F32) - st[hf][0]) * st[hf][1]
              for hf in range(2) for c in (0, DHF)]
        for m, v in enumerate(_lhs_ops(*qs)):
            a_s[m, t, _rows(p, 16), :] = v.astype(BF16)

    def ln(p, n):
        jobs = []
        for r in range(0, n, 16):
            st = {}
            jobs.append([[(90, part(ln_stats, st, p + r, hf)) for hf in range(2)],
                         [(45, part(ln_apply, st, p + r, t)) for t in range(4)]])
        return _pipeline(jobs, E("LND", 2))

    def perm_half(st, src, k, n, hf, tok):
        tie_w(tok)
        st[hf] = _perm_lanes([pltpu.bitcast(w_v[src, hf, _rows(k, n), pl.ds(j * 128, 128)], U32) for j in range(8)])

    def perm_ops(st, slot, k, n, t, tok):
        for m, v in enumerate(_rhs_ops(*[pltpu.bitcast(st[hf][t + c], BF16) for hf in range(2) for c in (0, 4)])):
            b1_s[slot, m, t, _rows(k, n), :] = v.astype(BF16)

    def prep_qkv(src, slot, k, rows, n):
        jobs = []
        for r in range(0, rows, n):
            st = {}
            jobs.append([[(40, part(perm_half, st, src, k + r, n, hf)) for hf in range(2)],
                         [(22, part(perm_ops, st, slot, k + r, n, t)) for t in range(4)]])
        return _pipeline(jobs, E("PD", 0))

    def wo_rows(st, hl, jh, c, i, tok):
        tie_w(tok)
        st[i] = _perm_words([pltpu.bitcast(w_v[O_, jh, _rows(jl * 128 + hl * 32 + (i // 2 ^ jh) * 16, 16),
                                               pl.ds(i % 2 * DHF + c, 128)], U32) for jl in range(4)])

    def wo_ops(st, hl, jh, c, tl, tok):
        for m, v in enumerate(_rhs_ops(*[pltpu.bitcast(st[i][tl], BF16) for i in range(4)])):
            bo_s[m, c // 128, _rows(tl * 128 + hl * 32 + jh * 16, 16), :] = v.astype(BF16)

    def prep_wo(hl, jh, c):
        st = {}
        return ([(15, part(wo_rows, st, hl, jh, c, i)) for i in range(4)] +
                [(25, part(wo_ops, st, hl, jh, c, i)) for i in range(4)])

    def prep_gu(src, slot, k, n, tok):
        tie_w(tok)
        c = (n % 2) * FC + (n // 2) * 128
        qs = [w_v[src, hf, _rows(k, 16), pl.ds(c + c0, 128)] for hf in range(2) for c0 in (0, FC // 2)]
        for m, v in enumerate(_rhs_ops(*qs)):
            g1_s[slot, m, n, _rows(k, 16), :] = v.astype(BF16)

    def prep_d(src, s, slot, k, c, tok):
        tie_w(tok)
        qs = [w_v[src, s, _rows(k + r0, 16), pl.ds(c + c0, 128)] for r0 in (0, FC // 2) for c0 in (0, DHF)]
        for m, v in enumerate(_rhs_ops(*qs)):
            b2_s[slot, m, c // 128, _rows(k, 16), :] = v.astype(BF16)

    def prep_ffn(src_gu, src_d, s, slot, i, n):
        kk = DHF // n
        return ([(27, part(prep_gu, src_gu, slot, i * kk + r, c)) for r in range(0, kk, 16) for c in range(4)],
                [(27, part(prep_d, src_d, s, slot, i * (kk // 2) + r, c)) for r in range(0, kk // 2, 16)
                 for c in range(0, DHF, 128)])

    def clear_acc(m, r, tok):
        acc_s[0, _ds(zero() + SH, 8, 8), pl.ds(0, 128)] = tok
        acc_s[m, _rows(r, 32), :] = jnp.zeros((32, DHF), F32)

    def lane_add(x, bit):
        lane = jax.lax.broadcasted_iota(jnp.int32, x.shape, 1)
        return x + jnp.take_along_axis(x, lane ^ bit, axis=1)

    def qk(st, r, w0, tok):
        tie_qkv(tok)
        if w0 == 0:
            st["q"] = [qkv_s[Q_, t, pl.ds(r + HALO, 8), :] for t in range(8)]
            st["l"] = []
        for w in range(w0, w0 + AG):
            l = functools.reduce(jnp.add, [st["q"][t] * qkv_s[K_, t, pl.ds(r + (HALO - DIL * w), 8), :] for t in range(8)])
            st["l"].append(lane_add(l, 1))

    def logits(st, r, masked, tok):
        row = r + jax.lax.broadcasted_iota(jnp.int32, (8, 128), 0)
        ls = [lane_add(l, 2) * DH ** -0.5 for l in st["l"]]
        st["l"] = [jnp.where(row >= DIL * w, l, -1e9) if masked and w else l for w, l in enumerate(ls)]

    def soft_exp(st, tok):
        mx = functools.reduce(jnp.maximum, st["l"])
        st["e"] = [jnp.exp(l - mx) for l in st["l"]]

    def soft_norm(st, tok):
        inv = 1.0 / functools.reduce(jnp.add, st["e"])
        st["p"] = [e * inv for e in st["e"]]

    def pv(st, r, dst, t0, tok):
        tie_qkv(tok)
        for t in range(t0, t0 + AG):
            t_s[dst[0], dst[1], t, pl.ds(dst[2], 8), :] = functools.reduce(
                jnp.add, [st["p"][w] * qkv_s[V_, t, pl.ds(r + (HALO - DIL * w), 8), :] for w in range(W)])

    def attn_ops(p, s, t, tok):
        t_s[2, 0, 0, _ds(zero(), 8, 8), :] = tok
        for m, v in enumerate(_lhs_ops(t_s[s, 0, t], t_s[s, 0, t + 4], t_s[s, 1, t], t_s[s, 1, t + 4])):
            ao_s[m, t, _rows(p, 16), :] = v.astype(BF16)

    def attend(ps):
        out, late, n = [], [], 8 // AG
        for i, p in enumerate(ps):
            for hf in range(2):
                for sub in (0, 8):
                    st, r = {}, hf * SH + p + sub
                    cut = [late[len(late) * j // 4:len(late) * (j + 1) // 4] for j in range(4)]
                    out += [(16 * AG, part(qk, st, r, w0)) for w0 in range(0, W, AG)] + cut[0]
                    out += [(30, part(logits, st, r, hf == 0))] + cut[1]
                    out += [(30, part(soft_exp, st))] + cut[2]
                    out += [(25, part(soft_norm, st))] + cut[3]
                    late = [(15 * AG, part(pv, st, r, (i % 2, hf, sub), t0)) for t0 in range(0, 8, AG)]
            late += [(17, part(attn_ops, p, i % 2, t)) for t in range(4)]
        return out + late

    def project(u, slot, p, n):
        ms = {}

        def dot(m, t):
            rows = _rows(p + (0 if isinstance(p, int) else zero()), n)
            ms[m] = _mm([a_s[m, i, rows, :] for i in range(4)], [b1_s[slot, m, t]])
            if m == 6:
                for i, v in enumerate(_combine([ms[j] for j in range(7)])):
                    qkv_s[u, (i % 2) * 4 + t, _ds(HALO + (i // 2) * SH + p, n, 8), :] = v
            return ms[m]
        return [(n, part(dot, m, t)) for t in range(4) for m in range(7)]

    def glu(slot, p):
        ms = {}

        def up(m, n):
            rows = _rows(p + zero(), P)
            ms[m, n] = _mm([a_s[m, i, rows, :] for i in range(4)], [g1_s[slot, m, n]])
            if m == 6 and n % 2 == 1:
                g, u = (_combine([ms[j, i] for j in range(7)]) for i in (n - 1, n))
                for j, v in enumerate(_lhs_ops(*[a * b for a, b in zip(g, u)])):
                    h_s[j, n // 2] = v.astype(BF16)
            return ms[m, n]

        def down(m):
            y = _mm([h_s[m, i] for i in range(2)], [b2_s[slot, m, t] for t in range(4)])
            acc_s[m, _rows(p, P), :] += y
            return y
        return ([(0 if (m, n) == (6, 3) else 1, part(up, m, n)) for n in range(4) for m in range(7)] +
                [(E('DW', 1) if m < 7 - E('TAILF', 1) else 0, part(down, m)) for m in range(7)])

    x_copy(0).start()
    for s in range(4):
        k_copy(s).start()
    for b in range(1, SH // XB):
        x_copy(b).start()
    w_copy(Q_).start()
    w_copy(V_).start()
    for cp in f_copies(0):
        cp.start()
    w_copy(O_).start()
    for cp in f_copies(1):
        cp.start()
    qkv_s[K_, :, pl.ds(0, HALO), :] = jnp.zeros((8, HALO, 128), F32)

    x_copy(0).wait()

    for _, f in ln(0, XB):
        f(None)

    def first_weights(s, c):
        k_copy(s).wait()
        for _, f in prep_qkv(K_, 0, s * 128, 128, E("PN", 32)):
            f(None)
        return (c + s) >> 1

    z0 = count[1] = jax.lax.fori_loop(0, 4, first_weights, 0)

    for p, n in E("FIRST", ((0, 128), (128, 128), (256, 256))) if 'p' in E('PH', 'pafo') else ():
        for b in range((p + n) // XB, 2 * (p + n) // XB):
            x_copy(b).wait()
        dots = project(K_, 0, p, n)
        tail = E("TAIL0", 256) // n
        _interleave(dots[:-tail] + [(0, f) for _, f in dots[-tail:]], ln(p + n, p + n))

    @(pl.loop(0, 5) if 'a' in E('PH', 'pafo') else (lambda f: None))
    def _(it):
        count[1] = it
        u = (it + 1) // 2

        @pl.when(it == 0)
        def _():
            w_copy(Q_).wait()

        @pl.when(it == 1)
        def _():
            w_copy(V_).wait()
            for cp in f_copies(0):
                cp.wait()

        perm = prep_qkv(jnp.minimum(u + 1, V_), 1 - u % 2, 0, DHF, E("PNA", 16))
        gu, dn = prep_ffn(jnp.where(it == 0, K_, GU_), jnp.where(it == 0, K_, DN_), 0, 0, jnp.maximum(it - 1, 0), 4)
        dots = project(u, u % 2, (it + 1) % 2 * P, P)
        dots = dots[:-E('TAILA', 2)] + [(0, f) for _, f in dots[-E('TAILA', 2):]]
        r0 = jnp.maximum(it - 1, 0) * (SH // 4)
        clr = [(16, part(clear_acc, m, r0 + r)) for m in range(7) for r in range(0, SH // 4, 32)]
        _interleave(dots, _merge(perm, gu, dn, clr), lag=E("LAGA", 1))

    for t in range(8):
        qkv_s[V_, t, pl.ds(0, HALO), :] = jnp.broadcast_to(qkv_s[V_, t, pl.ds(HALO, 1), :], (HALO, 128))
    w_copy(O_).wait()

    nf = SH // P
    groups = SH // 16
    per = -(-groups // (NCH * nf))

    @(pl.loop(0, NCH * nf) if 'f' in E('PH', 'pafo') else (lambda f: None))
    def _(it):
        count[1] = it
        c, b = it // nf, it % nf

        @pl.when((b == 0) & (c + 1 < NCH))
        def _():
            for cp in f_copies(c + 1):
                cp.wait()

        @pl.when((b == 0) & (c + 2 < NCH))
        def _():
            for cp in f_copies(c + 2):
                cp.start()

        s = jnp.minimum(c + 1, NCH - 1) % 2
        gu, dn = prep_ffn(GU_ + s, DN_, s, 1 - c % 2, b, nf)
        att = attend([jnp.minimum(it * per + i, groups - 1) * 16 for i in range(per)])
        j = jnp.minimum(it, 7)
        wo = [x for col in range(0, DHF, 128) for x in prep_wo(j // 2, j % 2, col)]
        mode = E("MODE", 0)
        if E('NOWO', 0): wo = wo[:8]
        prep = _merge(gu, dn) if mode != 1 else dn + gu
        side = _merge(att, prep, wo) if mode < 2 else (_merge(att[:len(att) * 2 // 5], prep, wo) + att[len(att) * 2 // 5:])
        _interleave(glu(c % 2, b * P), side, lag=E("LAG", 1))

    count[1] = z0

    @pl.loop(0, SH // P_OUT)
    def _(it):
        count[1] = it
        for r in range(0, P_OUT, R_OUT):
            p = it * P_OUT + r
            for t in range(4):
                col = pl.ds(t * 128, 128)
                rows = _rows(p + zero(), R_OUT)
                ms = [acc_s[m, _rows(p, R_OUT), col] + _mm([ao_s[m, i, rows, :] for i in range(4)], [bo_s[m, t]])
                      for m in range(7)]
                for i, v in enumerate(_combine(ms)):
                    idx = (i // 2, _rows(p, R_OUT), pl.ds((i % 2) * DHF + t * 128, 128))
                    x_v[idx] = (x_v[idx].astype(F32) + v).astype(BF16)
            o_copy(it * (P_OUT // R_OUT) + r // R_OUT).start()

    count[1] = z0
    for i in range(SH // R_OUT):
        o_copy(i).wait()
    if E('PH', 'pafo') != 'pafo':
        x_v[0, pl.ds(0, 16), pl.ds(0, 128)] = qkv_s[zero(), 0, pl.ds(0, 16), :].astype(BF16)
        x_v[0, pl.ds(16, 16), pl.ds(0, 128)] = a_s[zero(), 0, pl.ds(0, 16), :] + b1_s[zero(), 0, 0, pl.ds(0, 16), :] + g1_s[zero(), 0, 0, pl.ds(0, 16), :] + b2_s[zero(), 0, 0, pl.ds(0, 16), :]
        o_copy(0).start()
        o_copy(0).wait()


@jax.jit
def pallas_parallel_sum__sliding_local_dilated__glu_gated_bilinear__prompt_kernel(A_x, A_wqkv, A_wo, B_x, B_w_gate, B_w_up, B_w_down):
    hbm = pl.BlockSpec(memory_space=pl.ANY)
    V = pltpu.VMEM
    dma = pltpu.SemaphoreType.DMA
    out = pl.pallas_call(
        _kernel,
        grid=(1,),
        in_specs=[hbm] * 6,
        out_specs=hbm,
        out_shape=jax.ShapeDtypeStruct((2, SH, D), BF16),
        scratch_shapes=[
            V((2, SH + 16, D), BF16), V((7, 2, DHF + 16, D), BF16), V((7, 4, SH, 128), BF16),
            V((2, 7, 4, DHF, 128), BF16), V((2, 7, 4, DHF, 128), BF16), V((2, 7, 4, FC // 2, 128), BF16),
            V((7, 4, DHF, 128), BF16), V((7, 2, P, 128), BF16), V((7, SH + 8, DHF), F32),
            V((3, 8, S + HALO + 8, 128), F32), V((3, 2, 8, 16, 128), F32), V((7, 4, SH, 128), BF16),
            dma((SH // XB,)), dma((4,)), dma((4,)), dma((6,)), dma((SH // R_OUT,)),
        ],
        compiler_params=pltpu.CompilerParams(vmem_limit_bytes=120 * 2**20, flags=E("FLAGS", None)),
        name="fused",
    )(A_x.reshape(2, SH, D), A_wqkv.reshape(2, DHF, 3 * D), A_wo.reshape(2, DHF, D),
      B_w_gate.reshape(2, DHF, F), B_w_up.reshape(2, DHF, F), B_w_down)
    return out.reshape(A_x.shape)
```

```python
import functools
import jax
import jax.numpy as jnp
import jax.experimental.pallas as pl
import jax.experimental.pallas.tpu as pltpu

E = lambda k, d: d
S, D, F = 2048, 1024, 3584
DH, W, DIL = 32, 8, 2
HALO = 16
SH, DHF = S // 2, D // 2
FC = 512
NCH = F // FC
XB = E('XB', 128)
P = 512
P_OUT = E("P_OUT", 256)
R_OUT = E("R_OUT", (192, 64))
O_CUT = E("O_CUT", (192, 256))
AG = E("AG", 2)
F32, BF16, U32 = jnp.float32, jnp.bfloat16, jnp.uint32
K_, Q_, V_, O_, GU_, DN_ = 0, 1, 2, 3, 4, 6


import contextlib
def _scope(n):
    return jax.named_scope(n) if E("SCOPES", 0) else contextlib.nullcontext()


def _scoped(n, deco):
    def go(f):
        with _scope(n):
            return deco(f)
    return go


def _ds(start, n, align):
    return pl.ds(start if isinstance(start, int) else pl.multiple_of(start, align), n)


def _rows(start, n):
    return _ds(start, n, 16)


def _put(ref, idx, start, v):
    v = v.astype(BF16)
    if ref.dtype == U32:
        ref[(*idx, _ds(start >> 1, v.shape[0] // 2, 8))] = pltpu.bitcast(v, U32)
    else:
        ref[(*idx, _rows(start, v.shape[0]))] = v


def _get(ref, idx, start=0, n=None):
    if ref.dtype == U32:
        return pltpu.bitcast(ref[(*idx, _ds(start >> 1, n // 2 if n else ref.shape[-2], 8))], BF16)
    return ref[(*idx, _rows(start, n or ref.shape[-2]))]


def _skew4(vs, pos, unit):
    cur = [vs[(-t) % 4] for t in range(4)]
    for b in (1, 2):
        m = (pos & (b * unit)) != 0
        cur = [jnp.where(m, cur[(t - b) % 4], cur[t]) for t in range(4)]
    return cur


def _perm_lanes(vs):
    lane = jax.lax.broadcasted_iota(jnp.int32, vs[0].shape, 1)
    lo, hi = _skew4(vs[:4], lane, 4), _skew4(vs[4:], lane, 4)
    m = (lane & 16) != 0
    mixed = [jnp.where(m, b, a) for a, b in zip(lo, hi)] + [jnp.where(m, a, b) for a, b in zip(lo, hi)]
    return [v if t == 0 else
            jnp.take_along_axis(v, ((lane & 115) ^ (t // 4 * 16)) | ((lane + t % 4 * 4) & 12), axis=1)
            for t, v in enumerate(mixed)]


def _perm_words(vs):
    row = jax.lax.broadcasted_iota(jnp.int32, vs[0].shape, 0)
    return [v if t == 0 else pltpu.roll(v, 8 - 2 * t, 0) for t, v in enumerate(_skew4(vs, row, 2))]


def _lhs_ops(a11, a12, a21, a22):
    return (a11 + a22, a21 + a22, a11, a22, a11 + a12, a21 - a11, a12 - a22)


def _rhs_ops(b11, b12, b21, b22, raw=False):
    f11, f12, f21, f22 = (v.astype(F32) for v in (b11, b12, b21, b22))
    return (f11 + f22, b11 if raw else f11, f12 - f22, f21 - f11, b22 if raw else f22, f11 + f12, f21 + f22)


def _combine(m):
    m1, m2, m3, m4, m5, m6, m7 = m
    return (m1 + m4 - m5 + m7, m3 + m5, m2 + m4, m1 - m2 + m3 + m6)


def _mm(a, b):
    cat = lambda v: v[0] if len(v) == 1 else jnp.concatenate(v, axis=1)
    return jnp.dot(cat(a), cat(b), preferred_element_type=F32)


def _merge(*lists):
    keyed = []
    for xs in lists:
        tot, done = sum(w for w, _ in xs), 0
        for w, f in xs:
            keyed.append(((done + w / 2) / tot, w, f))
            done += w
    return [(w, f) for _, w, f in sorted(keyed, key=lambda t: t[0])]


def _pipeline(jobs, dist):
    n, out = len(jobs[0]), []
    for i in range(len(jobs) + (n - 1) * dist):
        for st in range(n):
            if 0 <= i - st * dist < len(jobs):
                out += jobs[i - st * dist][st]
    return out


def _interleave(dots, side, lag=0):
    tot, share = sum(w for w, _ in side), sum(w for w, _ in dots)
    outs, done, j, cum = [], 0, 0, 0
    for i, (_, dot) in enumerate(dots):
        outs.append(dot())
        if i < lag:
            continue
        src = outs[i - lag]
        lo = tot * cum / share
        cum += dots[i - lag][0]
        hi = tot * cum / share
        while j < len(side) and done < hi - 1e-6:
            pos = min(max((done - lo) / (hi - lo), 0.0), 0.999) * (src.shape[1] // 128)
            r0, c0 = int(pos % 1 * src.shape[0]) // 8 * 8, int(pos) * 128
            side[j][1](src[r0:r0 + 8, c0:c0 + 128])
            done += side[j][0]
            j += 1
    assert j == len(side)


def _kernel(x_hbm, wqkv_hbm, wo_hbm, wg_hbm, wu_hbm, wd_hbm, o_hbm,
            x_v, w_v, a_s, b1_s, g1_s, b2_s, bo_s, h_s, acc_s, qkv_s, t_s, ao_s,
            sem_x, sem_k, sem_w, sem_f, sem_o):
    part = functools.partial
    count = [0, 0]

    def zero():
        count[0] += 1
        return jax.lax.shift_right_logical(count[1] + count[0], 24) * 16

    def tie_x(tok):
        if tok is not None:
            x_v[0, _rows(zero() + SH, 16), pl.ds(0, 128)] = pltpu.bitcast(tok, BF16)

    def tie_w(tok):
        if tok is not None:
            w_v[0, 0, _rows(zero() + DHF, 16), pl.ds(0, 128)] = pltpu.bitcast(tok, BF16)

    def tie_qkv(tok):
        qkv_s[0, 0, _ds(zero() + S + HALO, 8, 8), :] = tok

    def x_copy(b):
        return pltpu.make_async_copy(x_hbm.at[:, _rows(b * XB, XB)], x_v.at[:, _rows(b * XB, XB)], sem_x.at[b])

    def k_copy(s):
        return pltpu.make_async_copy(wqkv_hbm.at[:, _rows(s * 128, 128), pl.ds(D, D)],
                                     w_v.at[K_, :, _rows(s * 128, 128)], sem_k.at[s])

    def w_copy(i):
        src = wo_hbm if i == O_ else wqkv_hbm.at[:, :, pl.ds(0 if i == Q_ else 2 * D, D)]
        return pltpu.make_async_copy(src, w_v.at[i, :, pl.ds(0, DHF)], sem_w.at[i])

    def f_copies(c):
        s = c % 2
        col = _ds(c * FC, FC, FC)
        return [pltpu.make_async_copy(wg_hbm.at[:, :, col], w_v.at[GU_ + s, :, pl.ds(0, DHF), pl.ds(0, FC)], sem_f.at[3 * s]),
                pltpu.make_async_copy(wu_hbm.at[:, :, col], w_v.at[GU_ + s, :, pl.ds(0, DHF), pl.ds(FC, FC)], sem_f.at[3 * s + 1]),
                pltpu.make_async_copy(wd_hbm.at[col, :], w_v.at[DN_, s, pl.ds(0, DHF)], sem_f.at[3 * s + 2])]

    def o_copy(i, r, n):
        rows = _rows(i * P_OUT + r, n)
        return pltpu.make_async_copy(x_v.at[:, rows], o_hbm.at[:, rows], sem_o.at[i])

    def row_mean(x):
        y = functools.reduce(jnp.add, [x[:, c:c + 128] for c in range(0, D, 128)])
        return jnp.sum(y, axis=-1, keepdims=True) * (1.0 / D)

    def ln_stats(st, p, hf, tok):
        tie_x(tok)
        x = x_v[hf, _rows(p, 16), :].astype(F32)
        mu = row_mean(x)
        xc = x - mu
        st[hf] = (mu, jax.lax.rsqrt(row_mean(xc * xc) + 1e-5))

    def ln_apply(st, p, t, tok):
        tie_x(tok)
        qs = [(x_v[hf, _rows(p, 16), pl.ds(c + t * 128, 128)].astype(F32) - st[hf][0]) * st[hf][1]
              for hf in range(2) for c in (0, DHF)]
        for m, v in enumerate(_lhs_ops(*qs)):
            _put(a_s, (m, t), p, v)

    def ln(p, n, dist=E('LND', 3)):
        jobs = []
        for r in range(0, n, 16):
            st = {}
            jobs.append([[(90, part(ln_stats, st, p + r, hf)) for hf in range(2)],
                         [(45, part(ln_apply, st, p + r, t)) for t in range(4)]])
        return _pipeline(jobs, dist)

    def perm_half(st, src, k, n, hf, tok):
        tie_w(tok)
        st[hf] = _perm_lanes([pltpu.bitcast(w_v[src, hf, _rows(k, n), pl.ds(j * 128, 128)], U32) for j in range(8)])

    def perm_ops(st, slot, k, n, t, tok):
        for m, v in enumerate(_rhs_ops(*[pltpu.bitcast(st[hf][t + c], BF16) for hf in range(2) for c in (0, 4)], raw=True)):
            _put(b1_s, (slot, m, t), k, v)

    def prep_qkv(src, slot, k, rows, n):
        jobs = []
        for r in range(0, rows, n):
            st = {}
            jobs.append([[(40, part(perm_half, st, src, k + r, n, hf)) for hf in range(2)],
                         [(22, part(perm_ops, st, slot, k + r, n, t)) for t in range(4)]])
        return _pipeline(jobs, E("PD", 1))

    def wo_rows(st, hl, jh, c, i, tok):
        tie_w(tok)
        st[i] = _perm_words([pltpu.bitcast(w_v[O_, jh, _rows(jl * 128 + hl * 32 + (i // 2 ^ jh) * 16, 16),
                                               pl.ds(i % 2 * DHF + c, 128)], U32) for jl in range(4)])

    def wo_ops(st, hl, jh, c, tl, tok):
        for m, v in enumerate(_rhs_ops(*[pltpu.bitcast(st[i][tl], BF16) for i in range(4)], raw=True)):
            _put(bo_s, (m, c // 128), tl * 128 + hl * 32 + jh * 16, v)

    def prep_wo(hl, jh, c):
        st = {}
        return ([(15, part(wo_rows, st, hl, jh, c, i)) for i in range(4)] +
                [(25, part(wo_ops, st, hl, jh, c, i)) for i in range(4)])

    def prep_gu(src, slot, k, n, tok):
        tie_w(tok)
        c = (n % 2) * FC + (n // 2) * 128
        qs = [w_v[src, hf, _rows(k, 16), pl.ds(c + c0, 128)] for hf in range(2) for c0 in (0, FC // 2)]
        for m, v in enumerate(_rhs_ops(*qs, raw=g1_s.dtype == U32)):
            _put(g1_s, (slot, m, n), k, v)

    def prep_d(src, s, slot, k, c, tok):
        tie_w(tok)
        qs = [w_v[src, s, _rows(k + r0, 16), pl.ds(c + c0, 128)] for r0 in (0, FC // 2) for c0 in (0, DHF)]
        for m, v in enumerate(_rhs_ops(*qs, raw=b2_s.dtype == U32)):
            _put(b2_s, (slot, m, c // 128), k, v)

    def prep_ffn(src_gu, src_d, s, slot, i, n):
        kk = DHF // n
        return ([(27, part(prep_gu, src_gu, slot, i * kk + r, c)) for r in range(0, kk, 16) for c in range(4)],
                [(27, part(prep_d, src_d, s, slot, i * (kk // 2) + r, c)) for r in range(0, kk // 2, 16)
                 for c in range(0, DHF, 128)])

    def clear_acc(m, r, tok):
        acc_s[0, _ds(zero() + SH, 8, 8), pl.ds(0, 128)] = tok
        acc_s[m, _rows(r, 16), :] = jnp.zeros((16, DHF), F32)

    def lane_add(x, bit):
        lane = jax.lax.broadcasted_iota(jnp.int32, x.shape, 1)
        return x + jnp.take_along_axis(x, lane ^ bit, axis=1)

    def qk(st, r, w0, tok):
        tie_qkv(tok)
        if w0 == 0:
            st["q"] = [qkv_s[Q_, t, pl.ds(r + HALO, 8), :] for t in range(8)]
            st["l"] = []
        for w in range(w0, w0 + AG):
            l = functools.reduce(jnp.add, [st["q"][t] * qkv_s[K_, t, pl.ds(r + (HALO - DIL * w), 8), :] for t in range(8)])
            st["l"].append(lane_add(l, 1))

    def logits(st, r, masked, tok):
        row = r + jax.lax.broadcasted_iota(jnp.int32, (8, 128), 0)
        ls = [lane_add(l, 2) * DH ** -0.5 for l in st["l"]]
        st["l"] = [jnp.where(row >= DIL * w, l, -1e9) if masked and w else l for w, l in enumerate(ls)]

    def soft_exp(st, tok):
        mx = functools.reduce(jnp.maximum, st["l"])
        st["e"] = [jnp.exp(l - mx) for l in st["l"]]

    def soft_norm(st, tok):
        inv = 1.0 / functools.reduce(jnp.add, st["e"])
        st["p"] = [e * inv for e in st["e"]]

    def pv(st, r, dst, t0, tok):
        tie_qkv(tok)
        for t in range(t0, t0 + AG):
            t_s[dst[0], dst[1], t, pl.ds(dst[2], 8), :] = functools.reduce(
                jnp.add, [st["p"][w] * qkv_s[V_, t, pl.ds(r + (HALO - DIL * w), 8), :] for w in range(W)])

    def attn_ops(p, s, t, tok):
        t_s[2, 0, 0, _ds(zero(), 8, 8), :] = tok
        for m, v in enumerate(_lhs_ops(t_s[s, 0, t], t_s[s, 0, t + 4], t_s[s, 1, t], t_s[s, 1, t + 4])):
            _put(ao_s, (m, t), p, v)

    def attend(ps):
        out, late, n = [], [], 8 // AG
        for i, p in enumerate(ps):
            for hf in range(2):
                for sub in (0, 8):
                    st, r = {}, hf * SH + p + sub
                    cut = [late[len(late) * j // 4:len(late) * (j + 1) // 4] for j in range(4)]
                    out += [(16 * AG, part(qk, st, r, w0)) for w0 in range(0, W, AG)] + cut[0]
                    out += [(30, part(logits, st, r, hf == 0))] + cut[1]
                    out += [(30, part(soft_exp, st))] + cut[2]
                    out += [(25, part(soft_norm, st))] + cut[3]
                    late = [(15 * AG, part(pv, st, r, (i % 2, hf, sub), t0)) for t0 in range(0, 8, AG)]
            late += [(17, part(attn_ops, p, i % 2, t)) for t in range(4)]
        return out + late

    def project(u, slot, p, n):
        ms = {}

        def dot(m, t):
            r = p + (0 if isinstance(p, int) else zero())
            ms[m] = _mm([_get(a_s, (m, i), r, n) for i in range(4)], [_get(b1_s, (slot, m, t))])
            if m == 6:
                for i, v in enumerate(_combine([ms[j] for j in range(7)])):
                    qkv_s[u, (i % 2) * 4 + t, _ds(HALO + (i // 2) * SH + p, n, 8), :] = v
            return ms[m]
        return [(n, part(dot, m, t)) for t in range(4) for m in range(7)]

    def glu(slot, p):
        ms = {}

        def up(m, n):
            r = p + zero()
            ms[m, n] = _mm([_get(a_s, (m, i), r, P) for i in range(4)], [_get(g1_s, (slot, m, n))])
            if m == 6 and n % 2 == 1:
                g, u = (_combine([ms[j, i] for j in range(7)]) for i in (n - 1, n))
                for j, v in enumerate(_lhs_ops(*[a * b for a, b in zip(g, u)])):
                    _put(h_s, (j, n // 2), 0, v)
            return ms[m, n]

        def down(m):
            y = _mm([_get(h_s, (m, i)) for i in range(2)], [_get(b2_s, (slot, m, t)) for t in range(4)])
            acc_s[m, _rows(p, P), :] += y
            return y
        return ([(0 if (m, n) == (6, 3) else (E('W13', 0) if (m, n) == (6, 1) else 1), part(up, m, n)) for n in range(4) for m in range(7)] +
                [(E('DW', 0.9) if m < 7 - E('TAILF', 1) else 0, part(down, m)) for m in range(7)])

    x_copy(0).start()
    x_copy(1).start()
    for s in range(4):
        k_copy(s).start()
    for b in range(2, SH // XB):
        x_copy(b).start()
    w_copy(Q_).start()
    w_copy(V_).start()
    for cp in f_copies(0):
        cp.start()
    w_copy(O_).start()
    for cp in f_copies(1):
        cp.start()
    qkv_s[K_, :, pl.ds(0, HALO), :] = jnp.zeros((8, HALO, 128), F32)


    def first_rows(i, c):
        x_copy(i).wait()
        for _, f in ln(i * XB, XB):
            f(None)
        return (c + i) >> 1

    z0 = count[1] = jax.lax.fori_loop(0, 2, first_rows, 0)
    k_copy(0).wait()
    for _, f in prep_qkv(K_, 0, 0, 128, E("PN", 32)):
        f(None)

    def k_slice(s, m):
        y = _mm([_get(a_s, (m, s), 0, 2 * XB)], [_get(b1_s, (0, m, t), s * 128, 128) for t in range(4)])
        rows = pl.ds(0, 2 * XB)
        if (s, m) != (3, 6):
            acc_s[m, rows, :] = y if s == 0 else acc_s[m, rows, :] + y
        else:
            for i, v in enumerate(_combine([acc_s[j, rows, :] for j in range(6)] + [acc_s[6, rows, :] + y])):
                for t in range(4):
                    qkv_s[K_, (i % 2) * 4 + t, pl.ds(HALO + (i // 2) * SH, 2 * XB), :] = v[:, t * 128:(t + 1) * 128]
        return y

    if 'p' in E('PH', 'pafo'):
        for s, blocks in enumerate(E("XS", ((), (), (2,), (3,), (4, 5, 6, 7)))):
            side = []
            if s < 3:
                k_copy(s + 1).wait()
                side.append(prep_qkv(K_, 0, (s + 1) * 128, 128, E("PN1", 16)))
            for b in blocks:
                x_copy(b).wait()
            if blocks:
                side.append(ln(blocks[0] * XB, len(blocks) * XB))
            if s < 4:
                dots = [(int(m < E("KW", 6)), part(k_slice, s, m)) for m in range(7)]
            else:
                dots = project(K_, 0, 2 * XB, 2 * XB)
                dots = dots[:-E("TAIL0", 2)] + [(0, f) for _, f in dots[-E("TAIL0", 2):]]
            _interleave(dots, _merge(*side))

    @(_scoped('loopA', pl.loop(0, 5)) if 'a' in E('PH', 'pafo') else (lambda f: None))
    def _(it):
        count[1] = it
        u = (it + 1) // 2

        @pl.when(it == 0)
        def _():
            w_copy(Q_).wait()

        @pl.when(it == 1)
        def _():
            w_copy(V_).wait()
            for cp in f_copies(0):
                cp.wait()

        perm = prep_qkv(jnp.minimum(u + 1, V_), 1 - u % 2, 0, DHF, E("PNA", 16))
        gu, dn = prep_ffn(jnp.where(it == 0, K_, GU_), jnp.where(it == 0, K_, DN_), 0, 0, jnp.maximum(it - 1, 0), 4)
        dots = project(u, u % 2, (it + 1) % 2 * P, P)
        dots = dots[:-E('TAILA', 1)] + [(0, f) for _, f in dots[-E('TAILA', 1):]]
        r0 = jnp.maximum(it - 1, 0) * (SH // 4)
        clr = [(16, part(clear_acc, m, r0 + r)) for m in range(7) for r in range(0, SH // 4, 16)]
        side = _merge(perm, gu, dn, clr)
        dots = [(w * (E("W6", 0) if i % 7 == 6 else 1), f) for i, (w, f) in enumerate(dots)]
        _interleave(dots, side, lag=E("LAGA", 1))

    for t in range(8):
        qkv_s[V_, t, pl.ds(0, HALO), :] = jnp.broadcast_to(qkv_s[V_, t, pl.ds(HALO, 1), :], (HALO, 128))
    w_copy(O_).wait()

    nf = SH // P
    groups = SH // 16
    per = -(-groups // (NCH * nf))

    @(_scoped('ffn', pl.loop(0, NCH * nf)) if 'f' in E('PH', 'pafo') else (lambda f: None))
    def _(it):
        count[1] = it
        c, b = it // nf, it % nf

        @pl.when((b == 0) & (c + 1 < NCH))
        def _():
            for cp in f_copies(c + 1):
                cp.wait()

        @pl.when((b == 0) & (c + 2 < NCH))
        def _():
            for cp in f_copies(c + 2):
                cp.start()

        s = jnp.minimum(c + 1, NCH - 1) % 2
        gu, dn = prep_ffn(GU_ + s, DN_, s, 1 - c % 2, b, nf)
        att = attend([it * 64 + i * 16 for i in range(4)] + [NCH * nf * 64 + jnp.minimum(it, 7) * 16])
        j = jnp.minimum(it, 7)
        wo = [x for col in range(0, DHF, 128) for x in prep_wo(j // 2, j % 2, col)]
        mode = E("MODE", 0)
        if E('NOWO', 0): wo = wo[:8]
        prep = _merge(gu, dn) if mode != 1 else dn + gu
        side = _merge(att, prep, wo) if mode < 2 else (_merge(att[:len(att) * 2 // 5], prep, wo) + att[len(att) * 2 // 5:])
        _interleave(glu(c % 2, b * P), side, lag=E("LAG", 1))

    count[1] = z0

    @_scoped('out', pl.loop(0, SH // P_OUT))
    def _(it):
        count[1] = it
        r = 0
        for n in R_OUT:
            p = it * P_OUT + r
            for t in range(4):
                col = pl.ds(t * 128, 128)
                q = p + zero()
                ms = [acc_s[m, _rows(p, n), col] + _mm([_get(ao_s, (m, i), q, n) for i in range(4)], [_get(bo_s, (m, t))])
                      for m in range(7)]
                for i, v in enumerate(_combine(ms)):
                    idx = (i // 2, _rows(p, n), pl.ds((i % 2) * DHF + t * 128, 128))
                    x_v[idx] = (x_v[idx].astype(F32) + v).astype(BF16)
            r += n
            if r in O_CUT:
                lo = ([0] + list(O_CUT))[O_CUT.index(r)]
                o_copy(it, lo, r - lo).start()

    count[1] = z0
    for i in range(SH // P_OUT):
        o_copy(i, 0, P_OUT).wait()
    if E('PH', 'pafo') != 'pafo':
        x_v[0, pl.ds(0, 16), pl.ds(0, 128)] = qkv_s[zero(), 0, pl.ds(0, 16), :].astype(BF16)
        x_v[0, pl.ds(16, 16), pl.ds(0, 128)] = _get(a_s, (zero(), 0), 0, 16) + _get(b1_s, (zero(), 0, 0), 0, 16) + _get(g1_s, (zero(), 0, 0), 0, 16) + _get(b2_s, (zero(), 0, 0), 0, 16)
        o_copy(0, 0, 16).start()
        o_copy(0, 0, 16).wait()


@jax.jit
def pallas_parallel_sum__sliding_local_dilated__glu_gated_bilinear__prompt_kernel(A_x, A_wqkv, A_wo, B_x, B_w_gate, B_w_up, B_w_down):
    hbm = pl.BlockSpec(memory_space=pl.ANY)
    V = pltpu.VMEM
    dma = pltpu.SemaphoreType.DMA
    op = lambda k, *s: V((*s[:-1], s[-1] // 2, 128), U32) if k in E("U32", "bgdo") else V((*s, 128), BF16)
    out = pl.pallas_call(
        _kernel,
        grid=(1,),
        in_specs=[hbm] * 6,
        out_specs=hbm,
        out_shape=jax.ShapeDtypeStruct((2, SH, D), BF16),
        scratch_shapes=[
            V((2, SH + 16, D), BF16), V((7, 2, DHF + 16, D), BF16), op("a", 7, 4, SH),
            op("b", 2, 7, 4, DHF), op("g", 2, 7, 4, DHF), op("d", 2, 7, 4, FC // 2),
            op("o", 7, 4, DHF), op("h", 7, 2, P), V((7, SH + 8, DHF), F32),
            V((3, 8, S + HALO + 8, 128), F32), V((3, 2, 8, 16, 128), F32), op("t", 7, 4, SH),
            dma((SH // XB,)), dma((4,)), dma((4,)), dma((6,)), dma((SH // P_OUT,)),
        ],
        compiler_params=pltpu.CompilerParams(vmem_limit_bytes=120 * 2**20, flags=E("FLAGS", None)),
        name="fused",
    )(A_x.reshape(2, SH, D), A_wqkv.reshape(2, DHF, 3 * D), A_wo.reshape(2, DHF, D),
      B_w_gate.reshape(2, DHF, F), B_w_up.reshape(2, DHF, F), B_w_down)
    return out.reshape(A_x.shape)
```

```python
import functools
import jax
import jax.numpy as jnp
import jax.experimental.pallas as pl
import jax.experimental.pallas.tpu as pltpu

E = lambda k, d: d
S, D, F = 2048, 1024, 3584
DH, W, DIL = 32, 8, 2
HALO = 16
SH, DHF = S // 2, D // 2
FC = 512
NCH = F // FC
XB = E('XB', 128)
P = 512
P_OUT = E("P_OUT", 256)
R_OUT = E("R_OUT", (192, 64))
O_CUT = E("O_CUT", (192, 256))
EX = E('EX', 0)
AG = E("AG", 2)
F32, BF16, U32 = jnp.float32, jnp.bfloat16, jnp.uint32
K_, Q_, V_, O_, GU_ = 0, 1, 2, 3, 4
DN_ = 2 * (GU_ + NCH)


import contextlib
def _scope(n):
    return jax.named_scope(n) if E("SCOPES", 0) else contextlib.nullcontext()


def _scoped(n, deco):
    def go(f):
        with _scope(n):
            return deco(f)
    return go


def _ds(start, n, align):
    return pl.ds(start if isinstance(start, int) else pl.multiple_of(start, align), n)


def _rows(start, n):
    return _ds(start, n, 16)


def _put(ref, idx, start, v):
    v = v.astype(BF16)
    if ref.dtype == U32:
        ref[(*idx, _ds(start >> 1, v.shape[0] // 2, 8))] = pltpu.bitcast(v, U32)
    else:
        ref[(*idx, _rows(start, v.shape[0]))] = v


def _get(ref, idx, start=0, n=None):
    if ref.dtype == U32:
        return pltpu.bitcast(ref[(*idx, _ds(start >> 1, n // 2 if n else ref.shape[-2], 8))], BF16)
    return ref[(*idx, _rows(start, n or ref.shape[-2]))]


def _skew4(vs, pos, unit):
    cur = [vs[(-t) % 4] for t in range(4)]
    for b in (1, 2):
        m = (pos & (b * unit)) != 0
        cur = [jnp.where(m, cur[(t - b) % 4], cur[t]) for t in range(4)]
    return cur


def _perm_lanes(vs):
    lane = jax.lax.broadcasted_iota(jnp.int32, vs[0].shape, 1)
    lo, hi = _skew4(vs[:4], lane, 4), _skew4(vs[4:], lane, 4)
    m = (lane & 16) != 0
    mixed = [jnp.where(m, b, a) for a, b in zip(lo, hi)] + [jnp.where(m, a, b) for a, b in zip(lo, hi)]
    return [v if t == 0 else
            jnp.take_along_axis(v, ((lane & 115) ^ (t // 4 * 16)) | ((lane + t % 4 * 4) & 12), axis=1)
            for t, v in enumerate(mixed)]


def _perm_words(vs):
    row = jax.lax.broadcasted_iota(jnp.int32, vs[0].shape, 0)
    return [v if t == 0 else pltpu.roll(v, 8 - 2 * t, 0) for t, v in enumerate(_skew4(vs, row, 2))]


def _lhs_ops(a11, a12, a21, a22):
    return (a11 + a22, a21 + a22, a11, a22, a11 + a12, a21 - a11, a12 - a22)


def _rhs_ops(b11, b12, b21, b22, raw=False):
    f11, f12, f21, f22 = (v.astype(F32) for v in (b11, b12, b21, b22))
    return (f11 + f22, b11 if raw else f11, f12 - f22, f21 - f11, b22 if raw else f22, f11 + f12, f21 + f22)


def _combine(m):
    m1, m2, m3, m4, m5, m6, m7 = m
    return (m1 + m4 - m5 + m7, m3 + m5, m2 + m4, m1 - m2 + m3 + m6)


ORDER = (1, 3, 4, 2, 0, 6, 5)
DONE = {3: 2, 2: 1, 6: 0, 5: 3}
LHS = (((0, 1), (3, 1)), ((2, 1), (3, 1)), ((0, 1),), ((3, 1),), ((0, 1), (1, 1)), ((2, 1), (0, -1)), ((1, 1), (3, -1)))
RHS = (((0, 1), (3, 1)), ((0, 1),), ((1, 1), (3, -1)), ((2, 1), (0, -1)), ((3, 1),), ((0, 1), (1, 1)), ((2, 1), (3, 1)))
OUT = (((0, 1), (3, 1), (4, -1), (6, 1)), ((2, 1), (4, 1)), ((1, 1), (3, 1)), ((0, 1), (1, -1), (2, 1), (5, 1)))


def _lin(terms, get):
    acc = get(terms[0][0])
    for i, sign in terms[1:]:
        acc = acc + get(i) if sign > 0 else acc - get(i)
    return acc


def _mm(a, b):
    cat = lambda v: v[0] if len(v) == 1 else jnp.concatenate(v, axis=1)
    return jnp.dot(cat(a), cat(b), preferred_element_type=F32)


def _merge(*lists):
    keyed = []
    for xs in lists:
        tot, done = sum(w for w, _ in xs), 0
        for w, f in xs:
            keyed.append(((done + w / 2) / tot, w, f))
            done += w
    return [(w, f) for _, w, f in sorted(keyed, key=lambda t: t[0])]


def _pipeline(jobs, dist):
    n, out = len(jobs[0]), []
    for i in range(len(jobs) + (n - 1) * dist):
        for st in range(n):
            if 0 <= i - st * dist < len(jobs):
                out += jobs[i - st * dist][st]
    return out


def _interleave(dots, side, lag=0):
    tot, share = sum(w for w, _ in side), sum(w for w, _ in dots)
    outs, done, j, cum = [], 0, 0, 0
    for i, (_, dot) in enumerate(dots):
        outs.append(dot())
        if i < lag:
            continue
        src = outs[i - lag]
        lo = tot * cum / share
        cum += dots[i - lag][0]
        hi = tot * cum / share
        while j < len(side) and done < hi - 1e-6:
            pos = min(max((done - lo) / (hi - lo), 0.0), 0.999) * (src.shape[1] // 128)
            r0, c0 = int(pos % 1 * src.shape[0]) // 8 * 8, int(pos) * 128
            side[j][1](src[r0:r0 + 8, c0:c0 + 128])
            done += side[j][0]
            j += 1
    assert j == len(side)


def _kernel(x_hbm, wqkv_hbm, wo_hbm, wg_hbm, wu_hbm, wd_hbm, o_hbm,
            x_v, w_v, a_s, b1_s, g1_s, b2_s, h_s, acc_s, qkv_s, t_s, a2_s,
            sem_x, sem_k, sem_w, sem_f, sem_o):
    part = functools.partial
    ao_s = a_s
    count = [0, 0]

    def zero():
        count[0] += 1
        return jax.lax.shift_right_logical(count[1] + count[0], 24) * 16

    def tie_x(tok):
        if tok is not None:
            x_v[0, _rows(zero() + SH, 16), pl.ds(0, 128)] = pltpu.bitcast(tok, BF16)

    def tie_w(tok):
        if tok is not None:
            w_v[0, _rows(zero() + DHF, 16), pl.ds(0, 128)] = pltpu.bitcast(tok, BF16)

    def tie_qkv(tok):
        qkv_s[0, 0, _ds(zero() + S + HALO, 8, 8), :] = tok

    def x_copy(b):
        return pltpu.make_async_copy(x_hbm.at[:, _rows(b * XB, XB)], x_v.at[:, _rows(b * XB, XB)], sem_x.at[b])

    def k_copy(s):
        return pltpu.make_async_copy(wqkv_hbm.at[:, _rows(s * 128, 128), pl.ds(D, D)],
                                     w_v.at[pl.ds(2 * K_, 2), _rows(s * 128, 128)], sem_k.at[s])

    def w_copy(i):
        src = wo_hbm if i == O_ else wqkv_hbm.at[:, :, pl.ds(0 if i == Q_ else 2 * D, D)]
        return pltpu.make_async_copy(src, w_v.at[pl.ds(2 * i, 2), pl.ds(0, DHF)], sem_w.at[i])

    def f_copies(c):
        col, dst = pl.ds(c * FC, FC), pl.ds(2 * (GU_ + c), 2)
        return [pltpu.make_async_copy(wg_hbm.at[:, :, col], w_v.at[dst, pl.ds(0, DHF), pl.ds(0, FC)], sem_f.at[3 * c]),
                pltpu.make_async_copy(wu_hbm.at[:, :, col], w_v.at[dst, pl.ds(0, DHF), pl.ds(FC, FC)], sem_f.at[3 * c + 1]),
                pltpu.make_async_copy(wd_hbm.at[col, :], w_v.at[DN_ + c, pl.ds(0, DHF)], sem_f.at[3 * c + 2])]

    def o_copy(i, r, n):
        rows = _rows(i * P_OUT + r, n)
        return pltpu.make_async_copy(x_v.at[:, rows], o_hbm.at[:, rows], sem_o.at[i])

    def row_mean(x):
        y = functools.reduce(jnp.add, [x[:, c:c + 128] for c in range(0, D, 128)])
        return jnp.sum(y, axis=-1, keepdims=True) * (1.0 / D)

    def ln_stats(st, p, hf, tok):
        tie_x(tok)
        x = x_v[hf, _rows(p, 16), :].astype(F32)
        mu = row_mean(x)
        xc = x - mu
        st[hf] = (mu, jax.lax.rsqrt(row_mean(xc * xc) + 1e-5))
        for i in range(2):
            acc_s[0, _rows(p, 16), pl.ds(i * 256 + hf * 128, 128)] = jnp.broadcast_to(st[hf][i], (16, 128))

    def ln_apply(st, p, t, tok):
        tie_x(tok)
        qs = [(x_v[hf, _rows(p, 16), pl.ds(c + t * 128, 128)].astype(F32) - st[hf][0]) * st[hf][1]
              for hf in range(2) for c in (0, DHF)]
        for m, v in enumerate(_lhs_ops(*qs)):
            _put(a_s, (m, t), p, v)

    def ln(p, n, dist=E('LND', 4)):
        jobs = []
        for r in range(0, n, 16):
            st = {}
            jobs.append([[(90, part(ln_stats, st, p + r, hf)) for hf in range(2)],
                         [(45, part(ln_apply, st, p + r, t)) for t in range(4)]])
        return _pipeline(jobs, dist)

    def perm_half(st, src, k, n, hf, tok):
        tie_w(tok)
        st[hf] = _perm_lanes([pltpu.bitcast(w_v[2 * src + hf, _rows(k, n), pl.ds(j * 128, 128)], U32) for j in range(8)])

    def perm_ops(st, slot, k, n, t, tok):
        for m, v in enumerate(_rhs_ops(*[pltpu.bitcast(st[hf][t + c], BF16) for hf in range(2) for c in (0, 4)], raw=True)):
            _put(b1_s, (slot, m, t), k, v)

    def prep_qkv(src, slot, k, rows, n):
        jobs = []
        for r in range(0, rows, n):
            st = {}
            jobs.append([[(E('PW0', 40), part(perm_half, st, src, k + r, n, hf)) for hf in range(2)],
                         [(E('PW1', 22), part(perm_ops, st, slot, k + r, n, t)) for t in range(4)]])
        return _pipeline(jobs, E("PD", 1))

    def wo_rows(st, hl, jh, c, i, tok):
        tie_w(tok)
        st[i] = _perm_words([pltpu.bitcast(w_v[2 * O_ + jh, _rows(jl * 128 + hl * 32 + (i // 2 ^ jh) * 16, 16),
                                               pl.ds(i % 2 * DHF + c, 128)], U32) for jl in range(4)])

    def wo_ops(st, hl, jh, c, tl, tok):
        for m, v in enumerate(_rhs_ops(*[pltpu.bitcast(st[i][tl], BF16) for i in range(4)], raw=True)):
            _put(b1_s, (1, m, c // 128), tl * 128 + hl * 32 + jh * 16, v)

    def prep_wo(hl, jh, c):
        st = {}
        return ([(15, part(wo_rows, st, hl, jh, c, i)) for i in range(4)] +
                [(25, part(wo_ops, st, hl, jh, c, i)) for i in range(4)])

    def prep_gu(src, slot, k, n, mo, tok):
        tie_w(tok)
        blk = lambda qo, qi: w_v[src + qo // 2, _rows(k + qi // 2 * 256, 16),
                                 pl.ds(n * FC + qo % 2 * 256 + qi % 2 * 128, 128)].astype(F32)
        qs = [_lin(RHS[mo], lambda qo: blk(qo, qi)) for qi in range(4)]
        for mi, terms in enumerate(RHS):
            _put(g1_s, (slot, mo * 7 + mi, n), k, _lin(terms, qs.__getitem__))

    def lhs2(r, t, mo, tok):
        tie_x(tok)

        def blk(qo, qi):
            row = qi // 2 * (SH // 2) + r
            x = x_v[qo // 2, _rows(row, 16), pl.ds(qo % 2 * DHF + qi % 2 * 256 + t * 128, 128)].astype(F32)
            return (x - acc_s[0, _rows(row, 16), pl.ds(qo // 2 * 128, 128)]) * acc_s[0, _rows(row, 16), pl.ds(256 + qo // 2 * 128, 128)]
        qs = [_lin(LHS[mo], lambda qo: blk(qo, qi)) for qi in range(4)]
        for mi, terms in enumerate(LHS):
            _put(a2_s, (mo * 7 + mi, t), r, _lin(terms, qs.__getitem__))

    def prep_d(src, slot, k, c, tok):
        tie_w(tok)
        qs = [w_v[src, _rows(k + r0, 16), pl.ds(c + c0, 128)] for r0 in (0, FC // 2) for c0 in (0, DHF)]
        for m, v in enumerate(_rhs_ops(*qs, raw=b2_s.dtype == U32)):
            _put(b2_s, (slot, m, c // 128), k, v)

    def prep_ffn(src_gu, src_d, slot, i, n):
        kk = DHF // n
        return ([(E("GW", 70), part(prep_gu, src_gu, slot, i * (kk // 2) + r, c, mo)) for r in range(0, kk // 2, 16)
                 for c in range(2) for mo in range(7)],
                [(27, part(prep_d, src_d, slot, i * (kk // 2) + r, c)) for r in range(0, kk // 2, 16)
                 for c in range(0, DHF, 128)])

    def clear_acc(m, r, tok):
        acc_s[0, _ds(zero() + SH, 8, 8), pl.ds(0, 128)] = tok
        acc_s[m, _ds(r, E('CR', 16), 8), :] = jnp.zeros((E('CR', 16), DHF), F32)

    def lane_add(x, bit):
        lane = jax.lax.broadcasted_iota(jnp.int32, x.shape, 1)
        return x + jnp.take_along_axis(x, lane ^ bit, axis=1)

    def qk(st, r, w0, tok):
        tie_qkv(tok)
        if w0 == 0:
            st["q"] = [qkv_s[Q_, t, pl.ds(r + HALO, 8), :] for t in range(8)]
            st["l"] = []
        for w in range(w0, w0 + AG):
            l = functools.reduce(jnp.add, [st["q"][t] * qkv_s[K_, t, pl.ds(r + (HALO - DIL * w), 8), :] for t in range(8)])
            st["l"].append(lane_add(l, 1))

    def logits(st, r, masked, tok):
        row = r + jax.lax.broadcasted_iota(jnp.int32, (8, 128), 0)
        ls = [lane_add(l, 2) * DH ** -0.5 for l in st["l"]]
        st["l"] = [jnp.where(row >= DIL * w, l, -1e9) if masked and w else l for w, l in enumerate(ls)]

    def soft_exp(st, tok):
        mx = functools.reduce(jnp.maximum, st["l"])
        st["e"] = [jnp.exp(l - mx) for l in st["l"]]

    def soft_norm(st, tok):
        inv = 1.0 / functools.reduce(jnp.add, st["e"])
        st["p"] = [e * inv for e in st["e"]]

    def pv(st, r, dst, t0, tok):
        tie_qkv(tok)
        for t in range(t0, t0 + AG):
            t_s[dst[0], dst[1], t, pl.ds(dst[2], 8), :] = functools.reduce(
                jnp.add, [st["p"][w] * qkv_s[V_, t, pl.ds(r + (HALO - DIL * w), 8), :] for w in range(W)])

    def attn_ops(p, s, t, tok):
        t_s[2, 0, 0, _ds(zero(), 8, 8), :] = tok
        for m, v in enumerate(_lhs_ops(t_s[s, 0, t], t_s[s, 0, t + 4], t_s[s, 1, t], t_s[s, 1, t + 4])):
            _put(ao_s, (m, t), p, v)

    def attend(ps):
        out, late, n = [], [], 8 // AG
        for i, p in enumerate(ps):
            for hf in range(2):
                for sub in (0, 8):
                    st, r = {}, hf * SH + p + sub
                    cut = [late[len(late) * j // 4:len(late) * (j + 1) // 4] for j in range(4)]
                    out += [(16 * AG, part(qk, st, r, w0)) for w0 in range(0, W, AG)] + cut[0]
                    out += [(30, part(logits, st, r, hf == 0))] + cut[1]
                    out += [(30, part(soft_exp, st))] + cut[2]
                    out += [(25, part(soft_norm, st))] + cut[3]
                    late = [(15 * AG, part(pv, st, r, (i % 2, hf, sub), t0)) for t0 in range(0, 8, AG)]
            late += [(17, part(attn_ops, p, i % 2, t)) for t in range(4)]
        return out + late

    def project(u, slot, p, n):
        ms = {}

        def dot(m, t):
            r = p + (0 if isinstance(p, int) else zero())
            ms[m] = _mm([_get(a_s, (m, i), r, n) for i in range(4)], [_get(b1_s, (slot, m, t))])
            if m in DONE:
                i = DONE[m]
                qkv_s[u, (i % 2) * 4 + t, _ds(HALO + (i // 2) * SH + p, n, 8), :] = _lin(OUT[i], ms.get)
            return ms[m]
        return [(n, part(dot, m, t)) for t in range(4) for m in ORDER]

    def glu(slot, r0, first):
        n = P // 2
        inner, outer, hs = {}, {}, {}

        def up(mo, mi):
            r = r0 + zero()
            y = inner[mi] = _mm([_get(a2_s, (mo * 7 + mi, i), r, n) for i in range(2)],
                                [_get(g1_s, (slot, mo * 7 + mi, i)) for i in range(2)])
            if mi in DONE:
                ci = DONE[mi]
                outer[mo, ci] = _lin(OUT[ci], inner.get)
                if mo in DONE:
                    co = DONE[mo]
                    gu = _lin(OUT[co], lambda j: outer[j, ci])
                    hs[co, ci] = gu[:, :128] * gu[:, 128:]
                    for j, terms in enumerate(LHS):
                        need = [i for i, _ in terms]
                        if co in need and all((i, ci) in hs for i in need):
                            _put(h_s, (j, ci % 2), ci // 2 * n, _lin(terms, lambda i: hs[i, ci]))
            return y

        def down(m):
            y = _mm([_get(h_s, (m, i)) for i in range(2)], [_get(b2_s, (slot, m, t)) for t in range(4)])
            for hf in range(2):
                rows = _rows(r0 + hf * (SH // 2), n)
                acc_s[m, rows, :] = jnp.where(first, 0.0, acc_s[m, rows, :]) + y[hf * n:(hf + 1) * n]
            return y
        w6 = E("W7", (1, 1, 1, 1, 1, 0.5, 0.3))
        return ([(w6[k], part(up, mo, mi)) for k, mo in enumerate(ORDER) for mi in ORDER] +
                [(E('DW', 3) if k < 7 - E('TAILF', 2) else 0, part(down, m)) for k, m in enumerate((2, 4, 5, 3, 6, 1, 0))])

    x_copy(0).start()
    x_copy(1).start()
    for s in range(4):
        k_copy(s).start()
    for b in range(2, SH // XB):
        x_copy(b).start()
    w_copy(Q_).start()
    w_copy(V_).start()
    for c in range(NCH if E('PH', 'pafo') == 'pafo' else 1):
        for cp in f_copies(c):
            cp.start()
    w_copy(O_).start()
    qkv_s[K_, :, pl.ds(0, HALO), :] = jnp.zeros((8, HALO, 128), F32)


    def first_rows(i, c):
        x_copy(i).wait()
        for _, f in ln(i * XB, XB):
            f(None)
        return (c + i) >> 1

    z0 = count[1] = jax.lax.fori_loop(0, 2, first_rows, 0)
    k_copy(0).wait()
    for _, f in prep_qkv(K_, 0, 0, 128, E("PN", 32)):
        f(None)

    def k_slice(s, m):
        y = _mm([_get(a_s, (m, s), 0, 2 * XB)], [_get(b1_s, (0, m, t), s * 128, 128) for t in range(4)])
        for t in range(4):
            v = y[:, t * 128:(t + 1) * 128]
            at = lambda j: (V_, t, pl.ds(j * 2 * XB, 2 * XB))
            if s:
                v = qkv_s[at(m)] + v
            if s < 3 or m not in (6, 5):
                qkv_s[at(m)] = v
            if s == 3 and m in DONE:
                i = DONE[m]
                qkv_s[K_, (i % 2) * 4 + t, pl.ds(HALO + (i // 2) * SH, 2 * XB), :] = _lin(
                    OUT[i], lambda j: v if j == m else qkv_s[at(j)])
        return y

    if 'p' in E('PH', 'pafo'):
        for s, blocks in enumerate(E("XS", ((), (), (2,), (3,), (4, 5, 6, 7)))):
            side = []
            if s < 3:
                k_copy(s + 1).wait()
                side.append(prep_qkv(K_, 0, (s + 1) * 128, 128, E("PN1", 16)))
            for b in blocks:
                x_copy(b).wait()
            if blocks:
                side.append(ln(blocks[0] * XB, len(blocks) * XB))
            if s < 4:
                dots = [(int(k < E("KW", 7)), part(k_slice, s, m)) for k, m in enumerate(ORDER)]
            else:
                dots = project(K_, 0, 2 * XB, 2 * XB)
                dots = dots[:-E("TAIL0", 1)] + [(0, f) for _, f in dots[-E("TAIL0", 1):]]
            _interleave(dots, _merge(*side))

    w_copy(Q_).wait()

    @(_scoped('loopA', pl.loop(0, 5)) if 'a' in E('PH', 'pafo') else (lambda f: None))
    def _(it):
        count[1] = it
        u = (it + 1) >> 1

        @pl.when(it == 1)
        def _():
            w_copy(V_).wait()
            for cp in f_copies(0):
                cp.wait()

        perm = prep_qkv(jnp.minimum(u + 1, V_), 1 - (u & 1), 0, DHF, E("PNA", 16))
        gu, dn = prep_ffn(jnp.where(it == 0, 0, 2 * GU_), jnp.where(it == 0, 0, DN_), 0, jnp.maximum(it - 1, 0), 4)
        dots = project(u, u & 1, ((it + 1) & 1) * P, P)
        dots = dots[:-E('TAILA', 1)] + [(0, f) for _, f in dots[-E('TAILA', 1):]]
        r0 = jnp.maximum(it - 1, 0) * (SH // 4)
        a2 = [(60, part(lhs2, jnp.maximum(it - 1, 0) * 128 + r, t, mo)) for r in range(0, 128, 16) for t in range(2) for mo in range(7)]
        side = _merge(perm, gu, dn, a2)
        _interleave(dots, side, lag=E("LAGA", 1))

    for t in range(8):
        qkv_s[V_, t, pl.ds(0, HALO), :] = jnp.broadcast_to(qkv_s[V_, t, pl.ds(HALO, 1), :], (HALO, 128))
    w_copy(O_).wait()
    for c in range(1, NCH if E('PH', 'pafo') == 'pafo' else 1):
        for cp in f_copies(c):
            cp.wait()

    nf = SH // P
    groups = SH // 16
    per = -(-groups // (NCH * nf))

    @(_scoped('ffn', pl.loop(0, NCH * nf)) if 'f' in E('PH', 'pafo') else (lambda f: None))
    def _(it):
        count[1] = it
        c, b = it >> 1, it & 1
        nxt = jnp.minimum(c + 1, NCH - 1)
        gu, dn = prep_ffn(2 * (GU_ + nxt), DN_ + nxt, 1 - (c & 1), b, nf)
        att = attend([it * 64 + i * 16 for i in range(4)] + [NCH * nf * 64 + jnp.minimum(it, 7) * 16])
        j = jnp.minimum(it, 7)
        wo = [x for col in range(0, DHF, 128) for x in prep_wo(j >> 1, j & 1, col)]
        mode = E("MODE", 0)
        if E('NOWO', 0): wo = wo[:8]
        prep = _merge(gu, dn) if mode != 1 else dn + gu
        side = _merge(att, prep, wo) if mode < 2 else (_merge(att[:len(att) * 2 // 5], prep, wo) + att[len(att) * 2 // 5:])
        _interleave(glu(c & 1, b * (P // 2), c == 0), side, lag=E("LAG", 2))

    count[1] = z0

    @_scoped('out', pl.loop(0, SH // P_OUT))
    def _(it):
        count[1] = it
        r = 0
        for n in R_OUT:
            p = it * P_OUT + r
            for t in range(4):
                col = pl.ds(t * 128, 128)
                q = p + zero()
                ms = [acc_s[m, _rows(p, n), col] + _mm([_get(ao_s, (m, i), q, n) for i in range(4)], [_get(b1_s, (1, m, t))])
                      for m in range(7)]
                for i, v in enumerate(_combine(ms)):
                    idx = (i // 2, _rows(p, n), pl.ds((i % 2) * DHF + t * 128, 128))
                    x_v[idx] = (x_v[idx].astype(F32) + v).astype(BF16)
            r += n
            if r in O_CUT:
                lo = ([0] + list(O_CUT))[O_CUT.index(r)]
                o_copy(it, lo, r - lo).start()

    count[1] = z0
    for i in range(SH // P_OUT):
        o_copy(i, 0, P_OUT).wait()
    if E('PH', 'pafo') != 'pafo':
        x_v[0, pl.ds(0, 16), pl.ds(0, 128)] = qkv_s[zero(), 0, pl.ds(0, 16), :].astype(BF16)
        x_v[0, pl.ds(16, 16), pl.ds(0, 128)] = _get(a_s, (zero(), 0), 0, 16) + _get(b1_s, (zero(), 0, 0), 0, 16) + _get(g1_s, (zero(), 0, 0), 0, 16) + _get(a2_s, (zero(), 0), 0, 16) + _get(b2_s, (zero(), 0, 0), 0, 16)
        o_copy(0, 0, 16).start()
        o_copy(0, 0, 16).wait()


@jax.jit
def pallas_parallel_sum__sliding_local_dilated__glu_gated_bilinear__prompt_kernel(A_x, A_wqkv, A_wo, B_x, B_w_gate, B_w_up, B_w_down):
    hbm = pl.BlockSpec(memory_space=pl.ANY)
    V = pltpu.VMEM
    dma = pltpu.SemaphoreType.DMA
    op = lambda k, *s: V((*s[:-1], s[-1] // 2, 128), U32) if k in E("U32", "bgdoh") else V((*s, 128), BF16)
    out = pl.pallas_call(
        _kernel,
        grid=(1,),
        in_specs=[hbm] * 6,
        out_specs=hbm,
        out_shape=jax.ShapeDtypeStruct((2, SH, D), BF16),
        scratch_shapes=[
            V((2, SH + 16, D), BF16), V((DN_ + NCH if E('PH', 'pafo') == 'pafo' else DN_ + 1, DHF + 16, D), BF16), op("a", 7, 4, SH),
            op("b", 2, 7, 4, DHF), op("g", 2, 49, 2, 256), op("d", 2, 7, 4, FC // 2),
            op("h", 7, 2, P), V((7, SH, DHF), F32),
            V((3, 8, S + HALO + 8, 128), F32), V((3, 2, 8, 16, 128), F32), op("A", 49, 2, SH // 2),
            dma((SH // XB,)), dma((4,)), dma((4,)), dma((3 * NCH,)), dma((SH // P_OUT,)),
        ],
        compiler_params=pltpu.CompilerParams(vmem_limit_bytes=int(E('VL', 127) * 2**20), flags=E("FLAGS", None)),
        name="fused",
    )(A_x.reshape(2, SH, D), A_wqkv.reshape(2, DHF, 3 * D), A_wo.reshape(2, DHF, D),
      B_w_gate.reshape(2, DHF, F), B_w_up.reshape(2, DHF, F), B_w_down)
    return out.reshape(A_x.shape)
```

```python
import functools
import jax
import jax.numpy as jnp
import jax.experimental.pallas as pl
import jax.experimental.pallas.tpu as pltpu

E = lambda k, d: d
S, D, F = 2048, 1024, 3584
DH, W, DIL = 32, 8, 2
HALO = 16
SH, DHF = S // 2, D // 2
FC = 512
NCH = F // FC
XB = E('XB', 128)
P = 512
P_OUT = E("P_OUT", 256)
R_OUT = E("R_OUT", (192, 64))
O_CUT = E("O_CUT", (192, 256))
OX = E('OX', 1)
GA = E('GA', 3)
AG = E("AG", 2)
F32, BF16, U32 = jnp.float32, jnp.bfloat16, jnp.uint32
K_, Q_, V_, O_, GU_ = 0, 1, 2, 3, 4
DN_ = 2 * (GU_ + NCH)


import contextlib
def _scope(n):
    return jax.named_scope(n) if E("SCOPES", 0) else contextlib.nullcontext()


def _scoped(n, deco):
    def go(f):
        with _scope(n):
            return deco(f)
    return go


def _ds(start, n, align):
    return pl.ds(start if isinstance(start, int) else pl.multiple_of(start, align), n)


def _rows(start, n):
    return _ds(start, n, 16)


def _put(ref, idx, start, v):
    ref[(*idx, _rows(start, v.shape[0]))] = v.astype(BF16)


def _get(ref, idx, start=0, n=None):
    return pltpu.bitcast(ref.bitcast(U32)[(*idx, _ds(start >> 1, (n or ref.shape[-2]) // 2, 8))], BF16)


def _skew4(vs, pos, unit):
    cur = [vs[(-t) % 4] for t in range(4)]
    for b in (1, 2):
        m = (pos & (b * unit)) != 0
        cur = [jnp.where(m, cur[(t - b) % 4], cur[t]) for t in range(4)]
    return cur


def _perm_lanes(vs):
    lane = jax.lax.broadcasted_iota(jnp.int32, vs[0].shape, 1)
    lo, hi = _skew4(vs[:4], lane, 4), _skew4(vs[4:], lane, 4)
    m = (lane & 16) != 0
    mixed = [jnp.where(m, b, a) for a, b in zip(lo, hi)] + [jnp.where(m, a, b) for a, b in zip(lo, hi)]
    return [v if t == 0 else
            jnp.take_along_axis(v, ((lane & 115) ^ (t // 4 * 16)) | ((lane + t % 4 * 4) & 12), axis=1)
            for t, v in enumerate(mixed)]


def _perm_words(vs):
    row = jax.lax.broadcasted_iota(jnp.int32, vs[0].shape, 0)
    return [v if t == 0 else pltpu.roll(v, 8 - 2 * t, 0) for t, v in enumerate(_skew4(vs, row, 2))]


def _lhs_ops(a11, a12, a21, a22):
    return (a11 + a22, a21 + a22, a11, a22, a11 + a12, a21 - a11, a12 - a22)


def _rhs_ops(b11, b12, b21, b22, raw=False):
    f11, f12, f21, f22 = (v.astype(F32) for v in (b11, b12, b21, b22))
    return (f11 + f22, f11, f12 - f22, f21 - f11, f22, f11 + f12, f21 + f22)


def _combine(m):
    m1, m2, m3, m4, m5, m6, m7 = m
    return (m1 + m4 - m5 + m7, m3 + m5, m2 + m4, m1 - m2 + m3 + m6)


ORDER = (1, 3, 4, 2, 0, 6, 5)
DONE = {3: 2, 2: 1, 6: 0, 5: 3}
LHS = (((0, 1), (3, 1)), ((2, 1), (3, 1)), ((0, 1),), ((3, 1),), ((0, 1), (1, 1)), ((2, 1), (0, -1)), ((1, 1), (3, -1)))
RHS = (((0, 1), (3, 1)), ((0, 1),), ((1, 1), (3, -1)), ((2, 1), (0, -1)), ((3, 1),), ((0, 1), (1, 1)), ((2, 1), (3, 1)))
OUT = (((6, 1), (0, 1), (3, 1), (4, -1)), ((2, 1), (4, 1)), ((3, 1), (1, 1)), ((5, 1), (0, 1), (1, -1), (2, 1)))


def _lin(terms, get):
    acc = get(terms[0][0])
    for i, sign in terms[1:]:
        acc = acc + get(i) if sign > 0 else acc - get(i)
    return acc


def _mm(a, b):
    cat = lambda v: v[0] if len(v) == 1 else jnp.concatenate(v, axis=1)
    return jnp.dot(cat(a), cat(b), preferred_element_type=F32)


def _merge(*lists):
    keyed = []
    for xs in lists:
        tot, done = sum(w for w, _ in xs), 0
        for w, f in xs:
            keyed.append(((done + w / 2) / tot, w, f))
            done += w
    return [(w, f) for _, w, f in sorted(keyed, key=lambda t: t[0])]


def _pipeline(jobs, dist):
    n, out = len(jobs[0]), []
    for i in range(len(jobs) + (n - 1) * dist):
        for st in range(n):
            if 0 <= i - st * dist < len(jobs):
                out += jobs[i - st * dist][st]
    return out


def _interleave(dots, side, lag=0):
    tot, share = sum(w for w, _ in side), sum(w for w, _ in dots)
    outs, done, j, cum = [], 0, 0, 0
    for i, (_, dot) in enumerate(dots):
        outs.append(dot())
        if i < lag:
            continue
        src = outs[i - lag]
        lo = tot * cum / share
        cum += dots[i - lag][0]
        hi = tot * cum / share
        while j < len(side) and done < hi - 1e-6:
            pos = min(max((done - lo) / (hi - lo), 0.0), 0.999) * (src.shape[1] // 128)
            r0, c0 = int(pos % 1 * src.shape[0]) // 8 * 8, int(pos) * 128
            side[j][1](src[r0:r0 + 8, c0:c0 + 128])
            done += side[j][0]
            j += 1
    assert j == len(side)


def _kernel(x_hbm, wqkv_hbm, wo_hbm, wg_hbm, wu_hbm, wd_hbm, o_hbm,
            x_v, w_v, a_s, b1_s, g1_s, b2_s, h_s, acc_s, qkv_s, t_s, a2_s, m_s,
            sem_x, sem_k, sem_w, sem_f, sem_o):
    part = functools.partial
    ao_s = a_s
    count = [0, 0]

    def zero():
        count[0] += 1
        return jax.lax.shift_right_logical(count[1] + count[0], 24) * 16

    def tie_x(tok):
        if tok is not None:
            x_v[0, _rows(zero() + SH, 16), pl.ds(0, 128)] = pltpu.bitcast(tok, BF16)

    def tie_w(tok):
        if tok is not None:
            w_v[0, _rows(zero() + DHF, 16), pl.ds(0, 128)] = pltpu.bitcast(tok, BF16)

    def tie_qkv(tok):
        qkv_s[0, 0, _ds(zero() + S + HALO, 8, 8), :] = tok

    def x_copy(b):
        return pltpu.make_async_copy(x_hbm.at[:, _rows(b * XB, XB)], x_v.at[:, _rows(b * XB, XB)], sem_x.at[b])

    def k_copy(s):
        return pltpu.make_async_copy(wqkv_hbm.at[:, _rows(s * 128, 128), pl.ds(D, D)],
                                     w_v.at[pl.ds(2 * K_, 2), _rows(s * 128, 128)], sem_k.at[s])

    def w_copy(i):
        src = wo_hbm if i == O_ else wqkv_hbm.at[:, :, pl.ds(0 if i == Q_ else 2 * D, D)]
        return pltpu.make_async_copy(src, w_v.at[pl.ds(2 * i, 2), pl.ds(0, DHF)], sem_w.at[i])

    def f_copies(c):
        col, dst = pl.ds(c * FC, FC), pl.ds(2 * (GU_ + c), 2)
        return [pltpu.make_async_copy(wg_hbm.at[:, :, col], w_v.at[dst, pl.ds(0, DHF), pl.ds(0, FC)], sem_f.at[3 * c]),
                pltpu.make_async_copy(wu_hbm.at[:, :, col], w_v.at[dst, pl.ds(0, DHF), pl.ds(FC, FC)], sem_f.at[3 * c + 1]),
                pltpu.make_async_copy(wd_hbm.at[col, :], w_v.at[DN_ + c, pl.ds(0, DHF)], sem_f.at[3 * c + 2])]

    def o_copy(i, r, n):
        rows = _rows(i * P_OUT + r, n)
        return pltpu.make_async_copy(x_v.at[:, rows], o_hbm.at[:, rows], sem_o.at[i])

    def row_mean(x):
        y = functools.reduce(jnp.add, [x[:, c:c + 128] for c in range(0, D, 128)])
        return jnp.sum(y, axis=-1, keepdims=True) * (1.0 / D)

    def ln_stats(st, p, hf, tok):
        tie_x(tok)
        x = x_v[hf, _rows(p, 16), :].astype(F32)
        mu = row_mean(x)
        xc = x - mu
        st[hf] = (mu, jax.lax.rsqrt(row_mean(xc * xc) + 1e-5))
        for i in range(2):
            acc_s[0, _rows(p, 16), pl.ds(i * 256 + hf * 128, 128)] = jnp.broadcast_to(st[hf][i], (16, 128))

    def ln_apply(st, p, t, tok):
        tie_x(tok)
        qs = [(x_v[hf, _rows(p, 16), pl.ds(c + t * 128, 128)].astype(F32) - st[hf][0]) * st[hf][1]
              for hf in range(2) for c in (0, DHF)]
        for m, v in enumerate(_lhs_ops(*qs)):
            _put(a_s, (m, t), p, v)

    def ln(p, n, dist=E('LND', 4)):
        jobs = []
        for r in range(0, n, 16):
            st = {}
            jobs.append([[(90, part(ln_stats, st, p + r, hf)) for hf in range(2)],
                         [(45, part(ln_apply, st, p + r, t)) for t in range(4)]])
        return _pipeline(jobs, dist)

    def perm_half(st, src, k, n, hf, tok):
        tie_w(tok)
        st[hf] = _perm_lanes([pltpu.bitcast(w_v[2 * src + hf, _rows(k, n), pl.ds(j * 128, 128)], U32) for j in range(8)])

    def perm_ops(st, slot, k, n, t, tok):
        for m, v in enumerate(_rhs_ops(*[pltpu.bitcast(st[hf][t + c], BF16) for hf in range(2) for c in (0, 4)], raw=True)):
            _put(b1_s[t // 2], (slot, m, t % 2), k, v)

    def prep_qkv(src, slot, k, rows, n, ts=range(4)):
        jobs = []
        for r in range(0, rows, n):
            st = {}
            jobs.append([[(E('PW0', 25), part(perm_half, st, src, k + r, n, hf)) for hf in range(2)],
                         [(E('PW1', 22), part(perm_ops, st, slot, k + r, n, t)) for t in ts]])
        return _pipeline(jobs, E("PD", 1))

    def wo_rows(st, hl, jh, c, i, tok):
        tie_w(tok)
        st[i] = _perm_words([pltpu.bitcast(w_v[2 * O_ + jh, _rows(jl * 128 + hl * 32 + (i // 2 ^ jh) * 16, 16),
                                               pl.ds(i % 2 * DHF + c, 128)], U32) for jl in range(4)])

    def wo_ops(st, hl, jh, c, tl, tok):
        for m, v in enumerate(_rhs_ops(*[pltpu.bitcast(st[i][tl], BF16) for i in range(4)], raw=True)):
            _put(b1_s[c // 256], (1, m, c // 128 % 2), tl * 128 + hl * 32 + jh * 16, v)

    def prep_wo(hl, jh, c):
        st = {}
        return ([(15, part(wo_rows, st, hl, jh, c, i)) for i in range(4)] +
                [(25, part(wo_ops, st, hl, jh, c, i)) for i in range(4)])

    def g_at(mo, mi):
        g = ORDER.index(mo)
        return (g1_s[0], g * 7 + mi) if g < GA else (g1_s[1], (g - GA) * 7 + mi)

    def gu_sum(st, src, k, n, mo, tok):
        tie_w(tok)
        blk = lambda qo, qi: w_v[src + qo // 2, _rows(k + qi // 2 * 256, 16),
                                 pl.ds(n * FC + qo % 2 * 256 + qi % 2 * 128, 128)].astype(F32)
        st["q"] = [_lin(RHS[mo], lambda qo: blk(qo, qi)) for qi in range(4)]

    def gu_ops(st, slot, k, n, mo, ms, tok):
        for mi in ms:
            _put(g_at(mo, mi)[0], (slot, g_at(mo, mi)[1], n), k, _lin(RHS[mi], st["q"].__getitem__))

    def prep_gu(src, slot, k, n, mo):
        st = {}
        return [(E("G0", 24), part(gu_sum, st, src, k, n, mo)), (E("G1", 9), part(gu_ops, st, slot, k, n, mo, (0, 1, 2, 3))),
                (E("G1", 9), part(gu_ops, st, slot, k, n, mo, (4, 5, 6)))]

    def x_sum(st, r, t, mo, qi, tok):
        tie_x(tok)
        rows = _rows(qi // 2 * (SH // 2) + r, 16)

        def blk(qo):
            x = x_v[qo // 2, rows, pl.ds(qo % 2 * DHF + qi % 2 * 256 + t * 128, 128)].astype(F32)
            return (x - acc_s[0, rows, pl.ds(qo // 2 * 128, 128)]) * acc_s[0, rows, pl.ds(256 + qo // 2 * 128, 128)]
        st[qi] = _lin(LHS[mo], blk)

    def x_ops(st, r, t, mo, tok):
        for mi, terms in enumerate(LHS):
            _put(a2_s, (mo * 7 + mi, t), r, _lin(terms, st.get))

    def lhs2(r, t, mo):
        st = {}
        return [(E("A0", 14), part(x_sum, st, r, t, mo, qi)) for qi in range(4)] + [(E("A1", 17), part(x_ops, st, r, t, mo))]

    def prep_d(src, slot, k, c, tok):
        tie_w(tok)
        qs = [w_v[src, _rows(k + r0, 16), pl.ds(c + c0, 128)] for r0 in (0, FC // 2) for c0 in (0, DHF)]
        for m, v in enumerate(_rhs_ops(*qs, raw=b2_s.dtype == U32)):
            _put(b2_s, (slot, m, c // 128), k, v)

    def prep_ffn(src_gu, src_d, slot, i, n):
        kk = DHF // n
        gu = [[x for r in range(0, kk // 2, 16) for c in range(2) for mo in ms
               for x in prep_gu(src_gu, slot, i * (kk // 2) + r, c, mo)] for ms in (ORDER[:GA], ORDER[GA:])]
        return (gu[0], gu[1],
                [(E('DP', 25), part(prep_d, src_d, slot, i * (kk // 2) + r, c)) for r in range(0, kk // 2, 16)
                 for c in range(0, DHF, 128)])

    def clear_acc(m, r, tok):
        acc_s[0, _ds(zero() + SH, 8, 8), pl.ds(0, 128)] = tok
        acc_s[m, _ds(r, E('CR', 16), 8), :] = jnp.zeros((E('CR', 16), DHF), F32)

    def lane_add(x, bit):
        lane = jax.lax.broadcasted_iota(jnp.int32, x.shape, 1)
        return x + jnp.take_along_axis(x, lane ^ bit, axis=1)

    def qk(st, r, w0, tok):
        tie_qkv(tok)
        if w0 == 0:
            st["q"] = [qkv_s[Q_, t, pl.ds(r + HALO, 8), :] for t in range(8)]
            st["l"] = []
        for w in range(w0, w0 + AG):
            l = functools.reduce(jnp.add, [st["q"][t] * qkv_s[K_, t, pl.ds(r + (HALO - DIL * w), 8), :] for t in range(8)])
            st["l"].append(lane_add(l, 1))

    def logits(st, r, masked, tok):
        row = r + jax.lax.broadcasted_iota(jnp.int32, (8, 128), 0)
        ls = [lane_add(l, 2) * DH ** -0.5 for l in st["l"]]
        st["l"] = [jnp.where(row >= DIL * w, l, -1e9) if masked and w else l for w, l in enumerate(ls)]

    def soft_exp(st, tok):
        mx = functools.reduce(jnp.maximum, st["l"])
        st["e"] = [jnp.exp(l - mx) for l in st["l"]]

    def soft_norm(st, tok):
        inv = 1.0 / functools.reduce(jnp.add, st["e"])
        st["p"] = [e * inv for e in st["e"]]

    def pv(st, r, dst, t0, tok):
        tie_qkv(tok)
        for t in range(t0, t0 + AG):
            t_s[dst[0], dst[1], t, pl.ds(dst[2], 8), :] = functools.reduce(
                jnp.add, [st["p"][w] * qkv_s[V_, t, pl.ds(r + (HALO - DIL * w), 8), :] for w in range(W)])

    def attn_ops(p, s, t, tok):
        t_s[2, 0, 0, _ds(zero(), 8, 8), :] = tok
        for m, v in enumerate(_lhs_ops(t_s[s, 0, t], t_s[s, 0, t + 4], t_s[s, 1, t], t_s[s, 1, t + 4])):
            _put(ao_s, (m, t), p, v)

    def attend(ps):
        out, late, n = [], [], 8 // AG
        for i, p in enumerate(ps):
            for hf in range(2):
                for sub in (0, 8):
                    st, r = {}, hf * SH + p + sub
                    cut = [late[len(late) * j // 4:len(late) * (j + 1) // 4] for j in range(4)]
                    out += [(16 * AG, part(qk, st, r, w0)) for w0 in range(0, W, AG)] + cut[0]
                    out += [(30, part(logits, st, r, hf == 0))] + cut[1]
                    out += [(30, part(soft_exp, st))] + cut[2]
                    out += [(25, part(soft_norm, st))] + cut[3]
                    late = [(15 * AG, part(pv, st, r, (i % 2, hf, sub), t0)) for t0 in range(0, 8, AG)]
            late += [(17, part(attn_ops, p, i % 2, t)) for t in range(4)]
        return out + late

    def project(u, slot, p, n):
        ms = {}

        def dot(m, t):
            r = p + (0 if isinstance(p, int) else zero())
            ms[m] = _mm([_get(a_s, (m, i), r, n) for i in range(4)], [_get(b1_s[t // 2], (slot, m, t % 2))])
            for r in range(0, n, 32) if m in DONE else ():
                i = DONE[m]
                qkv_s[u, (i % 2) * 4 + t, _ds(HALO + (i // 2) * SH + p + r, 32, 8), :] = _lin(OUT[i], lambda j: ms[j][r:r + 32])
            return ms[m]
        return [(n, part(dot, m, t)) for t in range(4) for m in ORDER]

    def glu(slot, r0, first):
        n = P // 2
        inner, outer, hs = {}, {}, {}
        zs = zero() * 2

        def up(mo, mi):
            r = r0 + zero()
            y = inner[mi] = _mm([_get(a2_s, (mo * 7 + mi, i), r, n) for i in range(2)],
                                [_get(g_at(mo, mi)[0], (slot, g_at(mo, mi)[1], i)) for i in range(2)])
            done = E("IDONE", {3: (2,), 2: (1,), 6: (0,), 5: (3,)}).get(mi, ())
            for r in range(0, n, 16):
                for ci in done:
                    outer[mo, ci, r] = _lin(OUT[ci], lambda j: inner[j][r:r + 16])
                    if OX and mo not in (6, 5):
                        m_s[mo, ci, pl.ds(r, 16), :] = outer[mo, ci, r]
                    if mo in DONE:
                        co = DONE[mo]
                        gu = _lin(OUT[co], lambda j: m_s[j, ci, pl.ds(r, 16) if co < 2 or co == 2 else _rows(r + zs, 16), :] if OX and j != mo else outer[j, ci, r])
                        hs[co, ci, r] = gu[:, :128] * gu[:, 128:]
                        for j, terms in enumerate(LHS):
                            need = [i for i, _ in terms]
                            if co in need and all((i, ci, r) in hs for i in need):
                                _put(h_s, (j, ci % 2), ci // 2 * n + r, _lin(terms, lambda i: hs[i, ci, r]))
            return y

        def down(m):
            y = _mm([_get(h_s, (m, i)) for i in range(2)], [_get(b2_s, (slot, m, t)) for t in range(4)])
            for t in range(0, DHF, E("DC", 256)):
                for r in range(0, P, E("DR", 64)):
                    idx = (m, _rows(r0 + r // n * (SH // 2) + r % n, E("DR", 64)), pl.ds(t, E("DC", 256)))
                    acc_s[idx] = jnp.where(first, 0.0, acc_s[idx]) + y[r:r + E("DR", 64), t:t + E("DC", 256)]
            return y
        w6 = E("W7", (1, 1, 1, 1, 1, 0.8, 0.6))
        return ([(w6[k], part(up, mo, mi)) for k, mo in enumerate(ORDER) for mi in ORDER] +
                [(E('DW', 3) if k < 7 - E('TAILF', 1) else 0, part(down, m)) for k, m in enumerate((2, 4, 5, 3, 6, 1, 0))])

    x_copy(0).start()
    x_copy(1).start()
    for s in range(4):
        k_copy(s).start()
    for b in range(2, SH // XB):
        x_copy(b).start()
    w_copy(Q_).start()
    w_copy(V_).start()
    for c in range(NCH if E('PH', 'pafo') == 'pafo' else 1):
        for cp in f_copies(c):
            cp.start()
    w_copy(O_).start()
    qkv_s[K_, :, pl.ds(0, HALO), :] = jnp.zeros((8, HALO, 128), F32)


    def first_rows(i, c):
        x_copy(i).wait()
        for _, f in ln(i * XB, XB):
            f(None)
        return (c + i) >> 1

    z0 = count[1] = jax.lax.fori_loop(0, 2, first_rows, 0)
    k_copy(0).wait()
    for _, f in prep_qkv(K_, 0, 0, 128, E("PN", 32)):
        f(None)

    def k_slice(s, m):
        y = _mm([_get(a_s, (m, s), 0, 2 * XB)], [_get(b1_s[t // 2], (0, m, t % 2), s * 128, 128) for t in range(4)])
        for t in range(4):
            v = y[:, t * 128:(t + 1) * 128]
            at = lambda j: (V_, t, pl.ds(j * 2 * XB, 2 * XB))
            if s:
                v = qkv_s[at(m)] + v
            if s < 3 or m not in (6, 5):
                qkv_s[at(m)] = v
            if s == 3 and m in DONE:
                i = DONE[m]
                qkv_s[K_, (i % 2) * 4 + t, pl.ds(HALO + (i // 2) * SH, 2 * XB), :] = _lin(
                    OUT[i], lambda j: v if j == m else qkv_s[at(j)])
        return y

    if 'p' in E('PH', 'pafo'):
        for s, blocks in enumerate(E("XS", ((), (), (2,), (3,), (4, 5, 6, 7)))):
            side = []
            if s < 3:
                k_copy(s + 1).wait()
                side.append(prep_qkv(K_, 0, (s + 1) * 128, 128, E("PN1", 16)))
            for b in blocks:
                x_copy(b).wait()
            if blocks:
                side.append(ln(blocks[0] * XB, len(blocks) * XB))
            if s < 4:
                dots = [(int(k < E("KW", 7)), part(k_slice, s, m)) for k, m in enumerate(ORDER)]
            else:
                dots = project(K_, 0, 2 * XB, 2 * XB)
                dots = dots[:-E("TAIL0", 1)] + [(0, f) for _, f in dots[-E("TAIL0", 1):]]
            _interleave(dots, _merge(*side))

    w_copy(Q_).wait()

    @(_scoped('loopA', pl.loop(0, 5)) if 'a' in E('PH', 'pafo') else (lambda f: None))
    def _(it):
        count[1] = it
        u = (it + 1) >> 1

        @pl.when(it == 1)
        def _():
            w_copy(V_).wait()
            for cp in f_copies(0):
                cp.wait()

        perm = [prep_qkv(jnp.minimum(u + 1, V_), 1 - (u & 1), 0, DHF, 16, ts) for ts in ((0, 1), (2, 3))]
        ga, gb, dn = prep_ffn(jnp.where(it == 0, 0, 2 * GU_), jnp.where(it == 0, 0, DN_), 0, jnp.maximum(it - 1, 0), 4)
        dots = project(u, u & 1, ((it + 1) & 1) * P, P)
        dots = dots[:-E('TAILA', 1)] + [(0, f) for _, f in dots[-E('TAILA', 1):]]
        r0 = jnp.maximum(it - 1, 0) * (SH // 4)
        a2 = [x for r in range(0, 128, 16) for t in range(2) for mo in range(7)
              for x in lhs2(jnp.maximum(it - 1, 0) * 128 + r, t, mo)]
        rest = _merge(ga + gb, dn, a2)
        h = len(rest) // 2
        _interleave([(0 if i == 13 else w, f) for i, (w, f) in enumerate(dots[:14])], _merge(perm[1], rest[:h]))
        _interleave(dots[14:], _merge(perm[0], rest[h:]))

    for t in range(8):
        qkv_s[V_, t, pl.ds(0, HALO), :] = jnp.broadcast_to(qkv_s[V_, t, pl.ds(HALO, 1), :], (HALO, 128))
    w_copy(O_).wait()
    for c in range(1, NCH if E('PH', 'pafo') == 'pafo' else 1):
        for cp in f_copies(c):
            cp.wait()

    nf = SH // P
    groups = SH // 16
    per = -(-groups // (NCH * nf))

    @(_scoped('ffn', pl.loop(0, NCH * nf)) if 'f' in E('PH', 'pafo') else (lambda f: None))
    def _(it):
        count[1] = it
        c, b = it >> 1, it & 1
        nxt = jnp.minimum(c + 1, NCH - 1)
        ga, gb, dn = prep_ffn(2 * (GU_ + nxt), DN_ + nxt, 1 - (c & 1), b, nf)
        att = attend([it * 64 + i * 16 for i in range(4)] + [NCH * nf * 64 + jnp.minimum(it, 7) * 16])
        j = jnp.minimum(it, 7)
        wo = [x for col in range(0, DHF, 128) for x in prep_wo(j >> 1, j & 1, col)]
        dots = glu(c & 1, b * (P // 2), c == 0)
        rest = _merge(att, wo)
        h0, h1 = (int(len(rest) * f) for f in E("HH", (0.25, 0.8)))
        g0 = int(len(ga) // 3 * E("GG", 0.5)) * 3
        _interleave(dots[:7 * GA - 1] + [(0, dots[7 * GA - 1][1])], _merge(gb, rest[:h0]))
        _interleave(dots[7 * GA:48] + [(0, dots[48][1])], _merge(dn + ga[:g0], rest[h0:h1]))
        _interleave(dots[49:], _merge(ga[g0:], rest[h1:]))

    count[1] = z0

    @_scoped('out', pl.loop(0, SH // P_OUT))
    def _(it):
        count[1] = it
        r = 0
        for n in R_OUT:
            p = it * P_OUT + r
            for t in range(4):
                col = pl.ds(t * 128, 128)
                q = p + zero()
                ms = [acc_s[m, _rows(p, n), col] + _mm([_get(ao_s, (m, i), q, n) for i in range(4)], [_get(b1_s[t // 2], (1, m, t % 2))])
                      for m in range(7)]
                for i, v in enumerate(_combine(ms)):
                    idx = (i // 2, _rows(p, n), pl.ds((i % 2) * DHF + t * 128, 128))
                    x_v[idx] = (x_v[idx].astype(F32) + v).astype(BF16)
            r += n
            if r in O_CUT:
                lo = ([0] + list(O_CUT))[O_CUT.index(r)]
                o_copy(it, lo, r - lo).start()

    count[1] = z0
    for i in range(SH // P_OUT):
        o_copy(i, 0, P_OUT).wait()
    if E('PH', 'pafo') != 'pafo':
        x_v[0, pl.ds(0, 16), pl.ds(0, 128)] = qkv_s[zero(), 0, pl.ds(0, 16), :].astype(BF16)
        x_v[0, pl.ds(16, 16), pl.ds(0, 128)] = _get(a_s, (zero(), 0), 0, 16) + _get(b1_s[0], (zero(), 0, 0), 0, 16) + _get(b1_s[1], (zero(), 0, 0), 0, 16) + _get(g1_s[0], (zero(), 0, 0), 0, 16) + _get(g1_s[1], (zero(), 0, 0), 0, 16) + _get(a2_s, (zero(), 0), 0, 16) + _get(b2_s, (zero(), 0, 0), 0, 16)
        o_copy(0, 0, 16).start()
        o_copy(0, 0, 16).wait()


@jax.jit
def pallas_parallel_sum__sliding_local_dilated__glu_gated_bilinear__prompt_kernel(A_x, A_wqkv, A_wo, B_x, B_w_gate, B_w_up, B_w_down):
    hbm = pl.BlockSpec(memory_space=pl.ANY)
    V = pltpu.VMEM
    dma = pltpu.SemaphoreType.DMA
    op = lambda k, *s: V((*s[:-1], s[-1] // 2, 128), U32) if k in "" else V((*s, 128), BF16)
    out = pl.pallas_call(
        _kernel,
        grid=(1,),
        in_specs=[hbm] * 6,
        out_specs=hbm,
        out_shape=jax.ShapeDtypeStruct((2, SH, D), BF16),
        scratch_shapes=[
            V((2, SH + 16, D), BF16), V((DN_ + NCH if E('PH', 'pafo') == 'pafo' else DN_ + 1, DHF + 16, D), BF16), op("a", 7, 4, SH),
            [op("b", 2, 7, 2, DHF)] * 2, [op("g", 2, 7 * GA, 2, 256), op("g", 2, 7 * (7 - GA), 2, 256)], op("d", 2, 7, 4, FC // 2),
            op("h", 7, 2, P), V((7, SH, DHF), F32),
            V((3, 8, S + HALO + 8, 128), F32), V((3, 2, 8, 16, 128), F32), op("A", 49, 2, SH // 2), V((5 if OX else 1, 4, P // 2 if OX else 8, 256), F32),
            dma((SH // XB,)), dma((4,)), dma((4,)), dma((3 * NCH,)), dma((SH // P_OUT,)),
        ],
        compiler_params=pltpu.CompilerParams(vmem_limit_bytes=int(E('VL', 127) * 2**20), flags=E("FLAGS", None)),
        name="fused",
    )(A_x.reshape(2, SH, D), A_wqkv.reshape(2, DHF, 3 * D), A_wo.reshape(2, DHF, D),
      B_w_gate.reshape(2, DHF, F), B_w_up.reshape(2, DHF, F), B_w_down)
    return out.reshape(A_x.shape)
```

```python
import functools

import jax
import jax.numpy as jnp
import jax.experimental.pallas as pl
import jax.experimental.pallas.tpu as pltpu

S, D, F = 2048, 1024, 3584
DH, W, DIL = 32, 8, 2
HALO = 16
SH, DHF = S // 2, D // 2
FC = 512
NCH = F // FC
XB = 128
P = 512
P_OUT = 256
R_OUT = (192, 64)
GA = 3
F32, BF16, U32 = jnp.float32, jnp.bfloat16, jnp.uint32
K_, Q_, V_, O_, GU_ = 0, 1, 2, 3, 4
DN_ = 2 * (GU_ + NCH)

LHS = (((0, 1), (3, 1)), ((2, 1), (3, 1)), ((0, 1),), ((3, 1),),
       ((0, 1), (1, 1)), ((2, 1), (0, -1)), ((1, 1), (3, -1)))
RHS = (((0, 1), (3, 1)), ((0, 1),), ((1, 1), (3, -1)), ((2, 1), (0, -1)),
       ((3, 1),), ((0, 1), (1, 1)), ((2, 1), (3, 1)))
OUT = (((6, 1), (0, 1), (3, 1), (4, -1)), ((2, 1), (4, 1)),
       ((3, 1), (1, 1)), ((5, 1), (0, 1), (1, -1), (2, 1)))
ORDER = (1, 3, 4, 2, 0, 6, 5)
DONE = {3: 2, 2: 1, 6: 0, 5: 3}


def _lin(terms, get):
    acc = get(terms[0][0])
    for i, sign in terms[1:]:
        acc = acc + get(i) if sign > 0 else acc - get(i)
    return acc


def _ds(start, n, align):
    return pl.ds(start if isinstance(start, int) else pl.multiple_of(start, align), n)


def _rows(start, n):
    return _ds(start, n, 16)


def _put(ref, idx, start, v):
    ref[(*idx, _rows(start, v.shape[0]))] = v.astype(BF16)


def _get(ref, idx, start=0, n=None):
    words = ref.bitcast(U32)[(*idx, _ds(start >> 1, (n or ref.shape[-2]) // 2, 8))]
    return pltpu.bitcast(words, BF16)


def _mm(a, b):
    cat = lambda v: v[0] if len(v) == 1 else jnp.concatenate(v, axis=1)
    return jnp.dot(cat(a), cat(b), preferred_element_type=F32)


def _skew4(vs, pos, unit):
    cur = [vs[(-t) % 4] for t in range(4)]
    for b in (1, 2):
        m = (pos & (b * unit)) != 0
        cur = [jnp.where(m, cur[(t - b) % 4], cur[t]) for t in range(4)]
    return cur


def _perm_lanes(vs):
    lane = jax.lax.broadcasted_iota(jnp.int32, vs[0].shape, 1)
    lo, hi = _skew4(vs[:4], lane, 4), _skew4(vs[4:], lane, 4)
    m = (lane & 16) != 0
    mixed = [jnp.where(m, b, a) for a, b in zip(lo, hi)] + [jnp.where(m, a, b) for a, b in zip(lo, hi)]
    return [v if t == 0 else
            jnp.take_along_axis(v, ((lane & 115) ^ (t // 4 * 16)) | ((lane + t % 4 * 4) & 12), axis=1)
            for t, v in enumerate(mixed)]


def _perm_words(vs):
    row = jax.lax.broadcasted_iota(jnp.int32, vs[0].shape, 0)
    return [v if t == 0 else pltpu.roll(v, 8 - 2 * t, 0) for t, v in enumerate(_skew4(vs, row, 2))]


def _merge(*lists):
    keyed = []
    for xs in lists:
        tot, done = sum(w for w, _ in xs), 0
        for w, f in xs:
            keyed.append(((done + w / 2) / tot, w, f))
            done += w
    return [(w, f) for _, w, f in sorted(keyed, key=lambda t: t[0])]


def _pipeline(jobs, dist):
    n, out = len(jobs[0]), []
    for i in range(len(jobs) + (n - 1) * dist):
        for st in range(n):
            if 0 <= i - st * dist < len(jobs):
                out += jobs[i - st * dist][st]
    return out


def _interleave(dots, side):
    tot, share = sum(w for w, _ in side), sum(w for w, _ in dots)
    done, j, cum = 0, 0, 0
    for w, dot in dots:
        src = dot()
        lo = tot * cum / share
        cum += w
        hi = tot * cum / share
        while j < len(side) and done < hi - 1e-6:
            pos = min(max((done - lo) / (hi - lo), 0.0), 0.999) * (src.shape[1] // 128)
            r0, c0 = int(pos % 1 * src.shape[0]) // 8 * 8, int(pos) * 128
            side[j][1](src[r0:r0 + 8, c0:c0 + 128])
            done += side[j][0]
            j += 1
    assert j == len(side)


def _quiet_tail(dots):
    return dots[:-1] + [(0, dots[-1][1])]


def _kernel(x_hbm, wqkv_hbm, wo_hbm, wg_hbm, wu_hbm, wd_hbm, o_hbm,
            x_v, w_v, a_s, a2_s, b1_s, g_s, b2_s, h_s, m_s, acc_s, qkv_s, t_s,
            sem_x, sem_k, sem_w, sem_f, sem_o):
    part = functools.partial
    step = [0, None]

    def zero():
        step[0] += 1
        return jax.lax.shift_right_logical(step[1] + step[0], 24) * 16

    def tie_x(tok):
        if tok is not None:
            x_v[0, _rows(zero() + SH, 16), pl.ds(0, 128)] = pltpu.bitcast(tok, BF16)

    def tie_w(tok):
        if tok is not None:
            w_v[0, _rows(zero() + DHF, 16), pl.ds(0, 128)] = pltpu.bitcast(tok, BF16)

    def tie_qkv(tok):
        qkv_s[0, 0, _ds(zero() + S + HALO, 8, 8), :] = tok

    def x_copy(b):
        rows = _rows(b * XB, XB)
        return pltpu.make_async_copy(x_hbm.at[:, rows], x_v.at[:, rows], sem_x.at[b])

    def k_copy(s):
        rows = pl.ds(s * 128, 128)
        return pltpu.make_async_copy(wqkv_hbm.at[:, rows, pl.ds(D, D)], w_v.at[pl.ds(2 * K_, 2), rows], sem_k.at[s])

    def w_copy(i):
        src = wo_hbm if i == O_ else wqkv_hbm.at[:, :, pl.ds(0 if i == Q_ else 2 * D, D)]
        return pltpu.make_async_copy(src, w_v.at[pl.ds(2 * i, 2), pl.ds(0, DHF)], sem_w.at[i])

    def f_copies(c):
        col, dst, rows = pl.ds(c * FC, FC), pl.ds(2 * (GU_ + c), 2), pl.ds(0, DHF)
        return [pltpu.make_async_copy(wg_hbm.at[:, :, col], w_v.at[dst, rows, pl.ds(0, FC)], sem_f.at[3 * c]),
                pltpu.make_async_copy(wu_hbm.at[:, :, col], w_v.at[dst, rows, pl.ds(FC, FC)], sem_f.at[3 * c + 1]),
                pltpu.make_async_copy(wd_hbm.at[col, :], w_v.at[DN_ + c, rows], sem_f.at[3 * c + 2])]

    def o_copy(i, j):
        rows = _rows(i * P_OUT + sum(R_OUT[:j]), R_OUT[j])
        return pltpu.make_async_copy(x_v.at[:, rows], o_hbm.at[:, rows], sem_o.at[i * len(R_OUT) + j])

    def row_mean(x):
        y = functools.reduce(jnp.add, [x[:, c:c + 128] for c in range(0, D, 128)])
        return jnp.sum(y, axis=-1, keepdims=True) * (1.0 / D)

    def ln_stats(st, p, hf, tok):
        tie_x(tok)
        x = x_v[hf, _rows(p, 16), :].astype(F32)
        mu = row_mean(x)
        xc = x - mu
        st[hf] = (mu, jax.lax.rsqrt(row_mean(xc * xc) + 1e-5))
        for i in range(2):
            acc_s[0, _rows(p, 16), pl.ds(i * 256 + hf * 128, 128)] = jnp.broadcast_to(st[hf][i], (16, 128))

    def ln_ops(st, p, t, tok):
        tie_x(tok)
        qs = [(x_v[hf, _rows(p, 16), pl.ds(c + t * 128, 128)].astype(F32) - st[hf][0]) * st[hf][1]
              for hf in range(2) for c in (0, DHF)]
        for m, terms in enumerate(LHS):
            _put(a_s, (m, t), p, _lin(terms, qs.__getitem__))

    def layer_norm(p, n):
        jobs = []
        for r in range(0, n, 16):
            st = {}
            jobs.append([[(90, part(ln_stats, st, p + r, hf)) for hf in range(2)],
                         [(45, part(ln_ops, st, p + r, t)) for t in range(4)]])
        return _pipeline(jobs, 4)

    def x_sum(st, r, t, mo, qi, tok):
        tie_x(tok)
        rows = _rows(qi // 2 * (SH // 2) + r, 16)

        def block(qo):
            x = x_v[qo // 2, rows, pl.ds(qo % 2 * DHF + qi % 2 * 256 + t * 128, 128)].astype(F32)
            return (x - acc_s[0, rows, pl.ds(qo // 2 * 128, 128)]) * acc_s[0, rows, pl.ds(256 + qo // 2 * 128, 128)]
        st[qi] = _lin(LHS[mo], block)

    def x_ops(st, r, t, mo, tok):
        for mi, terms in enumerate(LHS):
            _put(a2_s, (mo * 7 + mi, t), r, _lin(terms, st.get))

    def prep_x2(r, t, mo):
        st = {}
        return [(14, part(x_sum, st, r, t, mo, qi)) for qi in range(4)] + [(10, part(x_ops, st, r, t, mo))]

    def b1_at(slot, m, t):
        return b1_s[t // 2], (slot, m, t % 2)

    def g_at(slot, mo, mi, n):
        g = ORDER.index(mo)
        return (g_s[0], (slot, g * 7 + mi, n)) if g < GA else (g_s[1], (slot, (g - GA) * 7 + mi, n))

    def qkv_cols(st, src, k, n, hf, tok):
        tie_w(tok)
        st[hf] = _perm_lanes([pltpu.bitcast(w_v[2 * src + hf, _rows(k, n), pl.ds(j * 128, 128)], U32)
                              for j in range(8)])

    def qkv_ops(st, slot, k, t, tok):
        qs = [pltpu.bitcast(st[hf][t + c], BF16).astype(F32) for hf in range(2) for c in (0, 4)]
        for m, terms in enumerate(RHS):
            _put(*b1_at(slot, m, t), k, _lin(terms, qs.__getitem__))

    def prep_qkv(src, slot, k, rows, n=16, tiles=range(4)):
        jobs = []
        for r in range(0, rows, n):
            st = {}
            jobs.append([[(20, part(qkv_cols, st, src, k + r, n, hf)) for hf in range(2)],
                         [(22, part(qkv_ops, st, slot, k + r, t)) for t in tiles]])
        return _pipeline(jobs, 1)

    def wo_rows(st, h, jh, c, i, tok):
        tie_w(tok)
        st[i] = _perm_words([pltpu.bitcast(w_v[2 * O_ + jh, _rows(jl * 128 + h * 32 + (i // 2 ^ jh) * 16, 16),
                                               pl.ds(i % 2 * DHF + c * 128, 128)], U32) for jl in range(4)])

    def wo_ops(st, h, jh, c, tl, tok):
        qs = [pltpu.bitcast(st[i][tl], BF16).astype(F32) for i in range(4)]
        for m, terms in enumerate(RHS):
            _put(*b1_at(1, m, c), tl * 128 + h * 32 + jh * 16, _lin(terms, qs.__getitem__))

    def prep_wo(h, jh, c):
        st = {}
        return ([(15, part(wo_rows, st, h, jh, c, i)) for i in range(4)] +
                [(25, part(wo_ops, st, h, jh, c, i)) for i in range(4)])

    def gu_sum(st, src, k, n, mo, tok):
        tie_w(tok)
        block = lambda qo, qi: w_v[src + qo // 2, _rows(k + qi // 2 * 256, 16),
                                   pl.ds(n * FC + qo % 2 * 256 + qi % 2 * 128, 128)].astype(F32)
        st["q"] = [_lin(RHS[mo], lambda qo: block(qo, qi)) for qi in range(4)]

    def gu_ops(st, slot, k, n, mo, inner, tok):
        for mi in inner:
            _put(*g_at(slot, mo, mi, n), k, _lin(RHS[mi], st["q"].__getitem__))

    def prep_gu(src, slot, k, n, mo):
        st = {}
        return [(24, part(gu_sum, st, src, k, n, mo)),
                (9, part(gu_ops, st, slot, k, n, mo, (0, 1, 2, 3))), (9, part(gu_ops, st, slot, k, n, mo, (4, 5, 6)))]

    def prep_down(src, slot, k, t, tok):
        tie_w(tok)
        qs = [w_v[src, _rows(k + r0, 16), pl.ds(t * 128 + c0, 128)].astype(F32)
              for r0 in (0, FC // 2) for c0 in (0, DHF)]
        for m, terms in enumerate(RHS):
            _put(b2_s, (slot, m, t), k, _lin(terms, qs.__getitem__))

    def prep_glu(src_gu, src_d, slot, i, n):
        kk = 256 // n
        gu = [[x for r in range(0, kk, 16) for c in range(2) for mo in outer
               for x in prep_gu(src_gu, slot, i * kk + r, c, mo)] for outer in (ORDER[:GA], ORDER[GA:])]
        return gu[0], gu[1], [(25, part(prep_down, src_d, slot, i * kk + r, t))
                              for r in range(0, kk, 16) for t in range(4)]

    def lane_add(x, bit):
        lane = jax.lax.broadcasted_iota(jnp.int32, x.shape, 1)
        return x + jnp.take_along_axis(x, lane ^ bit, axis=1)

    def qk(st, r, t0, tok):
        tie_qkv(tok)
        for t in range(t0, t0 + 4):
            q = qkv_s[Q_, t, pl.ds(r + HALO, 8), :]
            ys = [q * qkv_s[K_, t, pl.ds(r + (HALO - DIL * w), 8), :] for w in range(W)]
            st["l"] = ys if t == 0 else [l + y for l, y in zip(st["l"], ys)]
        if t0:
            st["l"] = [lane_add(l, 1) for l in st["l"]]

    def logits(st, r, edge, tok):
        row = r + jax.lax.broadcasted_iota(jnp.int32, (8, 128), 0)
        ls = [lane_add(l, 2) * DH ** -0.5 for l in st["l"]]
        st["l"] = [jnp.where(row >= DIL * w, l, -1e9) if edge and w else l for w, l in enumerate(ls)]

    def softmax(st, tok):
        mx = functools.reduce(jnp.maximum, st["l"])
        es = [jnp.exp(l - mx) for l in st["l"]]
        inv = 1.0 / functools.reduce(jnp.add, es)
        st["p"] = [e * inv for e in es]

    def pv(st, r, s, hf, sub, t0, tok):
        tie_qkv(tok)
        for t in range(t0, t0 + 4):
            t_s[s, hf, t, pl.ds(sub, 8), :] = functools.reduce(
                jnp.add, [st["p"][w] * qkv_s[V_, t, pl.ds(r + (HALO - DIL * w), 8), :] for w in range(W)])

    def attn_ops(p, s, t, tok):
        t_s[2, 0, 0, _ds(zero(), 8, 8), :] = tok
        qs = [t_s[s, hf, t + c] for hf in range(2) for c in (0, 4)]
        for m, terms in enumerate(LHS):
            _put(a_s, (m, t), p, _lin(terms, qs.__getitem__))

    def attend(ps):
        out, late = [], []
        for i, p in enumerate(ps):
            for hf in range(2):
                for sub in (0, 8):
                    st, r = {}, hf * SH + p + sub
                    out += [(64, part(qk, st, r, t0)) for t0 in (0, 4)] + late[:len(late) // 2]
                    out += [(30, part(logits, st, r, (i, hf) == (0, 0)))] + late[len(late) // 2:]
                    out += [(55, part(softmax, st))]
                    late = [(60, part(pv, st, r, i % 2, hf, sub, t0)) for t0 in (0, 4)]
            late += [(17, part(attn_ops, p, i % 2, t)) for t in range(4)]
        return out + late

    def project(u, slot, p, n):
        ms = {}

        def dot(m, t):
            r = p + (0 if isinstance(p, int) else zero())
            ms[m] = _mm([_get(a_s, (m, i), r, n) for i in range(4)], [_get(*b1_at(slot, m, t))])
            for r in range(0, n, 32) if m in DONE else ():
                i = DONE[m]
                qkv_s[u, (i % 2) * 4 + t, _ds(HALO + (i // 2) * SH + p + r, 32, 8), :] = _lin(
                    OUT[i], lambda j: ms[j][r:r + 32])
            return ms[m]
        share = (1, 0.8, 1.1, 0.8, 1.1, 0.8, 0.8)
        return _quiet_tail([(share[i], part(dot, m, t)) for t in range(4) for i, m in enumerate(ORDER)])

    def project_slice(s, m):
        n = 2 * XB
        y = _mm([_get(a_s, (m, s), 0, n)], [_get(*b1_at(0, m, t), s * 128, 128) for t in range(4)])
        for t in range(4):
            at = lambda j: (V_, t, pl.ds(j * n, n))
            v = y[:, t * 128:(t + 1) * 128]
            if s:
                v = qkv_s[at(m)] + v
            if s < 3 or m not in ORDER[-2:]:
                qkv_s[at(m)] = v
            if s == 3 and m in DONE:
                i = DONE[m]
                qkv_s[K_, (i % 2) * 4 + t, pl.ds(HALO + (i // 2) * SH, n), :] = _lin(
                    OUT[i], lambda j: v if j == m else qkv_s[at(j)])
        return y

    def glu(slot, r0, first):
        n = P // 2
        inner, hs = {}, {}
        again = zero() * 2

        def up(mo, mi):
            r = r0 + zero()
            y = inner[mi] = _mm([_get(a2_s, (mo * 7 + mi, i), r, n) for i in range(2)],
                                [_get(*g_at(slot, mo, mi, i)) for i in range(2)])
            for r in range(0, n, 16) if mi in DONE else ():
                ci = DONE[mi]
                v = _lin(OUT[ci], lambda j: inner[j][r:r + 16])
                if mo not in ORDER[-2:]:
                    m_s[mo, ci, pl.ds(r, 16), :] = v
                if mo in DONE:
                    co = DONE[mo]
                    rows = _rows(r + again if co in (0, 3) else r, 16)
                    gu = _lin(OUT[co], lambda j: v if j == mo else m_s[j, ci, rows, :])
                    hs[co, ci, r] = gu[:, :128] * gu[:, 128:]
                    for j, terms in enumerate(LHS):
                        need = [i for i, _ in terms]
                        if co in need and all((i, ci, r) in hs for i in need):
                            _put(h_s, (j, ci % 2), ci // 2 * n + r, _lin(terms, lambda i: hs[i, ci, r]))
            return y

        def down(m, t):
            r = zero() * 4 if t else 0
            y = _mm([_get(h_s, (m, i), r, P) for i in range(2)], [_get(b2_s, (slot, m, t + i)) for i in range(2)])
            for hf in range(2):
                idx = (m, _rows(r0 + hf * (SH // 2), n), pl.ds(t * 128, 256))
                acc_s[idx] = jnp.where(first, 0.0, acc_s[idx]) + y[hf * n:(hf + 1) * n]
            return y
        so, si, sd = (1, 1, 1, 1, 1, 0.8, 0.3), (1, 0.8, 1.1, 0.8, 1.1, 1, 0.9), (0.8, 1, 1, 1, 1, 0.9, 0)
        return ([(so[k] * si[i], part(up, mo, mi)) for k, mo in enumerate(ORDER) for i, mi in enumerate(ORDER)],
                [(sd[k], part(down, m, t)) for k, m in enumerate((2, 4, 5, 3, 6, 1, 0)) for t in (0, 2)])

    x_copy(0).start()
    x_copy(1).start()
    for s in range(4):
        k_copy(s).start()
    for b in range(2, SH // XB):
        x_copy(b).start()
    w_copy(Q_).start()
    w_copy(V_).start()
    for c in range(NCH):
        for cp in f_copies(c):
            cp.start()
    w_copy(O_).start()
    qkv_s[K_, :, pl.ds(0, HALO), :] = jnp.zeros((8, HALO, 128), F32)

    def first_rows(i, c):
        x_copy(i).wait()
        for _, f in layer_norm(i * XB, XB):
            f(None)
        return (c + i) >> 1

    step[1] = jax.lax.fori_loop(0, 2, first_rows, 0)
    k_copy(0).wait()
    for _, f in prep_qkv(K_, 0, 0, 128, 32):
        f(None)
    for s, blocks in enumerate(((), (), (2,), (3,), (4, 5, 6, 7))):
        side = []
        if s < 3:
            k_copy(s + 1).wait()
            side.append(prep_qkv(K_, 0, (s + 1) * 128, 128))
        for b in blocks:
            x_copy(b).wait()
        if blocks:
            side.append(layer_norm(blocks[0] * XB, len(blocks) * XB))
        dots = (_quiet_tail([(1, part(project_slice, s, m)) for m in ORDER]) if s < 4 else
                project(K_, 0, 2 * XB, 2 * XB))
        _interleave(dots, _merge(*side))

    w_copy(Q_).wait()

    @pl.loop(0, 5)
    def _(it):
        step[1] = it
        u, quarter = (it + 1) >> 1, jnp.maximum(it - 1, 0)

        @pl.when(it == 1)
        def _():
            w_copy(V_).wait()
            for cp in f_copies(0):
                cp.wait()

        nxt = [prep_qkv(jnp.minimum(u + 1, V_), 1 - (u & 1), 0, DHF, tiles=ts) for ts in ((0, 1), (2, 3))]
        ga, gb, dn = prep_glu(jnp.where(it == 0, 0, 2 * GU_), jnp.where(it == 0, 0, DN_), 0, quarter, 4)
        x2 = [x for r in range(0, 128, 16) for t in range(2) for mo in range(7)
              for x in prep_x2(quarter * 128 + r, t, mo)]
        rest = _merge(ga + gb, dn, x2)
        dots = project(u, u & 1, ((it + 1) & 1) * P, P)
        _interleave(_quiet_tail(dots[:14]), _merge(nxt[1], rest[:len(rest) // 2]))
        _interleave(dots[14:], _merge(nxt[0], rest[len(rest) // 2:]))

    for t in range(8):
        qkv_s[V_, t, pl.ds(0, HALO), :] = jnp.broadcast_to(qkv_s[V_, t, pl.ds(HALO, 1), :], (HALO, 128))
    w_copy(O_).wait()
    for c in range(1, NCH):
        for cp in f_copies(c):
            cp.wait()

    @pl.loop(0, 2 * NCH)
    def _(it):
        step[1] = it
        c, b = it >> 1, it & 1
        nxt = jnp.minimum(c + 1, NCH - 1)
        extra = jnp.where(it < 8, it, 0)
        ga, gb, dn = prep_glu(2 * (GU_ + nxt), DN_ + nxt, 1 - (c & 1), b, 2)
        rest = _merge(attend([it * 64 + i * 16 for i in range(4)] + [2 * NCH * 64 + extra * 16]),
                      [x for t in range(4) for x in prep_wo(extra >> 1, extra & 1, t)])
        ups, downs = glu(c & 1, b * (P // 2), c == 0)
        h0, h1, g0 = int(len(rest) * 0.35), int(len(rest) * 0.84), int(len(ga) // 3 * 0.3) * 3
        _interleave(_quiet_tail(ups[:7 * GA]), _merge(gb, rest[:h0]))
        _interleave(_quiet_tail(ups[7 * GA:]), _merge(dn + ga[:g0], rest[h0:h1]))
        _interleave(downs, _merge(ga[g0:], rest[h1:]))

    @pl.loop(0, SH // P_OUT)
    def _(it):
        step[1] = it
        for j, n in enumerate(R_OUT):
            p = it * P_OUT + sum(R_OUT[:j])
            for t in range(4):
                r = p + zero()
                ms = [acc_s[m, _rows(p, n), pl.ds(t * 128, 128)] +
                      _mm([_get(a_s, (m, i), r, n) for i in range(4)], [_get(*b1_at(1, m, t))]) for m in range(7)]
                for i, terms in enumerate(OUT):
                    idx = (i // 2, _rows(p, n), pl.ds((i % 2) * DHF + t * 128, 128))
                    x_v[idx] = (x_v[idx].astype(F32) + _lin(terms, ms.__getitem__)).astype(BF16)
            o_copy(it, j).start()

    for i in range(SH // P_OUT):
        for j in range(len(R_OUT)):
            o_copy(i, j).wait()


@jax.jit
def pallas_parallel_sum__sliding_local_dilated__glu_gated_bilinear__prompt_kernel(
    A_x: jax.Array,
    A_wqkv: jax.Array,
    A_wo: jax.Array,
    B_x: jax.Array,
    B_w_gate: jax.Array,
    B_w_up: jax.Array,
    B_w_down: jax.Array,
):
    del B_x
    hbm = pl.BlockSpec(memory_space=pl.ANY)
    vmem, dma = pltpu.VMEM, pltpu.SemaphoreType.DMA
    operand = lambda *shape: vmem((*shape, 128), BF16)
    out = pl.pallas_call(
        _kernel,
        in_specs=[hbm] * 6,
        out_specs=hbm,
        out_shape=jax.ShapeDtypeStruct((2, SH, D), BF16),
        scratch_shapes=[
            vmem((2, SH + 16, D), BF16),
            vmem((DN_ + NCH, DHF + 16, D), BF16),
            operand(7, 4, SH),
            operand(49, 2, SH // 2),
            [operand(2, 7, 2, DHF)] * 2,
            [operand(2, 7 * GA, 2, 256), operand(2, 7 * (7 - GA), 2, 256)],
            operand(2, 7, 4, FC // 2),
            operand(7, 2, P),
            vmem((5, 4, P // 2, 256), F32),
            vmem((7, SH, DHF), F32),
            vmem((3, 8, S + HALO + 8, 128), F32),
            vmem((3, 2, 8, 16, 128), F32),
            dma((SH // XB,)), dma((4,)), dma((4,)), dma((3 * NCH,)), dma((SH // P_OUT * len(R_OUT),)),
        ],
        compiler_params=pltpu.CompilerParams(vmem_limit_bytes=127 * 2**20),
        name="fused",
    )(A_x.reshape(2, SH, D), A_wqkv.reshape(2, DHF, 3 * D), A_wo.reshape(2, DHF, D),
      B_w_gate.reshape(2, DHF, F), B_w_up.reshape(2, DHF, F), B_w_down)
    return out.reshape(A_x.shape)
```

```python
import functools

import jax
import jax.numpy as jnp
import jax.experimental.pallas as pl
import jax.experimental.pallas.tpu as pltpu

S, D, F = 2048, 1024, 3584
DH, W, DIL = 32, 8, 2
HALO = 16
SH, DHF = S // 2, D // 2
FC = 512
NCH = F // FC
XB = 128
P = 512
P_OUT = 256
R_OUT = (192, 64)
GA = 3
F32, BF16, U32 = jnp.float32, jnp.bfloat16, jnp.uint32
K_, Q_, V_, O_, GU_ = 0, 1, 2, 3, 4
DN_ = 2 * (GU_ + NCH)

LHS = (((0, 1), (3, 1)), ((2, 1), (3, 1)), ((0, 1),), ((3, 1),),
       ((0, 1), (1, 1)), ((2, 1), (0, -1)), ((1, 1), (3, -1)))
RHS = (((0, 1), (3, 1)), ((0, 1),), ((1, 1), (3, -1)), ((2, 1), (0, -1)),
       ((3, 1),), ((0, 1), (1, 1)), ((2, 1), (3, 1)))
OUT = (((6, 1), (0, 1), (3, 1), (4, -1)), ((2, 1), (4, 1)),
       ((3, 1), (1, 1)), ((5, 1), (0, 1), (1, -1), (2, 1)))
ORDER = (1, 3, 4, 2, 0, 6, 5)
DONE = {3: 2, 2: 1, 6: 0, 5: 3}


def _lin(terms, get):
    acc = get(terms[0][0])
    for i, sign in terms[1:]:
        acc = acc + get(i) if sign > 0 else acc - get(i)
    return acc


def _ds(start, n, align):
    return pl.ds(start if isinstance(start, int) else pl.multiple_of(start, align), n)


def _rows(start, n):
    return _ds(start, n, 16)


def _put(ref, idx, start, v):
    ref[(*idx, _rows(start, v.shape[0]))] = v.astype(BF16)


def _get(ref, idx, start=0, n=None):
    words = ref.bitcast(U32)[(*idx, _ds(start >> 1, (n or ref.shape[-2]) // 2, 8))]
    return pltpu.bitcast(words, BF16)


def _mm(a, b):
    cat = lambda v: v[0] if len(v) == 1 else jnp.concatenate(v, axis=1)
    return jnp.dot(cat(a), cat(b), preferred_element_type=F32)


def _skew4(vs, pos, unit):
    cur = [vs[(-t) % 4] for t in range(4)]
    for b in (1, 2):
        m = (pos & (b * unit)) != 0
        cur = [jnp.where(m, cur[(t - b) % 4], cur[t]) for t in range(4)]
    return cur


def _perm_lanes(vs):
    lane = jax.lax.broadcasted_iota(jnp.int32, vs[0].shape, 1)
    lo, hi = _skew4(vs[:4], lane, 4), _skew4(vs[4:], lane, 4)
    m = (lane & 16) != 0
    mixed = [jnp.where(m, b, a) for a, b in zip(lo, hi)] + [jnp.where(m, a, b) for a, b in zip(lo, hi)]
    return [v if t == 0 else
            jnp.take_along_axis(v, ((lane & 115) ^ (t // 4 * 16)) | ((lane + t % 4 * 4) & 12), axis=1)
            for t, v in enumerate(mixed)]


def _perm_words(vs):
    row = jax.lax.broadcasted_iota(jnp.int32, vs[0].shape, 0)
    return [v if t == 0 else pltpu.roll(v, 8 - 2 * t, 0) for t, v in enumerate(_skew4(vs, row, 2))]


def _merge(*lists):
    keyed = []
    for xs in lists:
        tot, done = sum(w for w, _ in xs), 0
        for w, f in xs:
            keyed.append(((done + w / 2) / tot, w, f))
            done += w
    return [(w, f) for _, w, f in sorted(keyed, key=lambda t: t[0])]


def _pipeline(jobs, dist):
    n, out = len(jobs[0]), []
    for i in range(len(jobs) + (n - 1) * dist):
        for st in range(n):
            if 0 <= i - st * dist < len(jobs):
                out += jobs[i - st * dist][st]
    return out


def _interleave(dots, side):
    tot, share = sum(w for w, _ in side), sum(w for w, _ in dots)
    done, j, cum = 0, 0, 0
    for w, dot in dots:
        src = dot()
        lo = tot * cum / share
        cum += w
        hi = tot * cum / share
        while j < len(side) and done < hi - 1e-6:
            pos = min(max((done - lo) / (hi - lo), 0.0), 0.999) * (src.shape[1] // 128)
            r0, c0 = int(pos % 1 * src.shape[0]) // 8 * 8, int(pos) * 128
            side[j][1](src[r0:r0 + 8, c0:c0 + 128])
            done += side[j][0]
            j += 1
    assert j == len(side)


def _quiet_tail(dots):
    return dots[:-1] + [(0, dots[-1][1])]


def _kernel(x_hbm, wqkv_hbm, wo_hbm, wg_hbm, wu_hbm, wd_hbm, o_hbm,
            x_v, w_v, a_s, a2_s, b1_s, g_s, b2_s, h_s, m_s, acc_s, qkv_s, t_s,
            sem_x, sem_k, sem_w, sem_f, sem_o):
    part = functools.partial
    step = [0, None]

    def zero():
        step[0] += 1
        return jax.lax.shift_right_logical(step[1] + step[0], 24) * 16

    def tie_x(tok):
        if tok is not None:
            x_v[0, _rows(zero() + SH, 16), pl.ds(0, 128)] = pltpu.bitcast(tok, BF16)

    def tie_w(tok):
        if tok is not None:
            w_v[0, _rows(zero() + DHF, 16), pl.ds(0, 128)] = pltpu.bitcast(tok, BF16)

    def tie_qkv(tok):
        qkv_s[0, 0, _ds(zero() + S + HALO, 8, 8), :] = tok

    def x_copy(b):
        rows = _rows(b * XB, XB)
        return pltpu.make_async_copy(x_hbm.at[:, rows], x_v.at[:, rows], sem_x.at[b])

    def k_copy(s):
        rows = pl.ds(s * 128, 128)
        return pltpu.make_async_copy(wqkv_hbm.at[:, rows, pl.ds(D, D)], w_v.at[pl.ds(2 * K_, 2), rows], sem_k.at[s])

    def w_copy(i):
        src = wo_hbm if i == O_ else wqkv_hbm.at[:, :, pl.ds(0 if i == Q_ else 2 * D, D)]
        return pltpu.make_async_copy(src, w_v.at[pl.ds(2 * i, 2), pl.ds(0, DHF)], sem_w.at[i])

    def f_copies(c):
        col, dst, rows = pl.ds(c * FC, FC), pl.ds(2 * (GU_ + c), 2), pl.ds(0, DHF)
        return [pltpu.make_async_copy(wg_hbm.at[:, :, col], w_v.at[dst, rows, pl.ds(0, FC)], sem_f.at[3 * c]),
                pltpu.make_async_copy(wu_hbm.at[:, :, col], w_v.at[dst, rows, pl.ds(FC, FC)], sem_f.at[3 * c + 1]),
                pltpu.make_async_copy(wd_hbm.at[col, :], w_v.at[DN_ + c, rows], sem_f.at[3 * c + 2])]

    def o_copy(i, j):
        rows = _rows(i * P_OUT + sum(R_OUT[:j]), R_OUT[j])
        return pltpu.make_async_copy(x_v.at[:, rows], o_hbm.at[:, rows], sem_o.at[i * len(R_OUT) + j])

    def row_mean(x):
        y = functools.reduce(jnp.add, [x[:, c:c + 128] for c in range(0, D, 128)])
        return jnp.sum(y, axis=-1, keepdims=True) * (1.0 / D)

    def ln_stats(st, p, hf, tok):
        tie_x(tok)
        x = x_v[hf, _rows(p, 16), :].astype(F32)
        mu = row_mean(x)
        xc = x - mu
        st[hf] = (mu, jax.lax.rsqrt(row_mean(xc * xc) + 1e-5))
        for i in range(2):
            acc_s[0, _rows(p, 16), pl.ds(i * 256 + hf * 128, 128)] = jnp.broadcast_to(st[hf][i], (16, 128))

    def ln_ops(st, p, t, tok):
        tie_x(tok)
        qs = [(x_v[hf, _rows(p, 16), pl.ds(c + t * 128, 128)].astype(F32) - st[hf][0]) * st[hf][1]
              for hf in range(2) for c in (0, DHF)]
        for m, terms in enumerate(LHS):
            _put(a_s, (m, t), p, _lin(terms, qs.__getitem__))

    def layer_norm(p, n):
        jobs = []
        for r in range(0, n, 16):
            st = {}
            jobs.append([[(90, part(ln_stats, st, p + r, hf)) for hf in range(2)],
                         [(45, part(ln_ops, st, p + r, t)) for t in range(4)]])
        return _pipeline(jobs, 4)

    def x_sum(st, r, t, mo, qi, tok):
        tie_x(tok)
        rows = _rows(qi // 2 * (SH // 2) + r, 16)

        def block(qo):
            x = x_v[qo // 2, rows, pl.ds(qo % 2 * DHF + qi % 2 * 256 + t * 128, 128)].astype(F32)
            return (x - acc_s[0, rows, pl.ds(qo // 2 * 128, 128)]) * acc_s[0, rows, pl.ds(256 + qo // 2 * 128, 128)]
        st[qi] = _lin(LHS[mo], block)

    def x_ops(st, r, t, mo, tok):
        for mi, terms in enumerate(LHS):
            _put(a2_s, (mo * 7 + mi, t), r, _lin(terms, st.get))

    def prep_x2(r, t, mo):
        st = {}
        return [(14, part(x_sum, st, r, t, mo, qi)) for qi in range(4)] + [(10, part(x_ops, st, r, t, mo))]

    def b1_at(slot, m, t):
        return b1_s[t // 2], (slot, m, t % 2)

    def g_at(slot, mo, mi, n):
        g = ORDER.index(mo)
        return (g_s[0], (slot, g * 7 + mi, n)) if g < GA else (g_s[1], (slot, (g - GA) * 7 + mi, n))

    def qkv_cols(st, src, k, n, hf, tok):
        tie_w(tok)
        st[hf] = _perm_lanes([pltpu.bitcast(w_v[2 * src + hf, _rows(k, n), pl.ds(j * 128, 128)], U32)
                              for j in range(8)])

    def qkv_ops(st, slot, k, t, tok):
        qs = [pltpu.bitcast(st[hf][t + c], BF16).astype(F32) for hf in range(2) for c in (0, 4)]
        for m, terms in enumerate(RHS):
            _put(*b1_at(slot, m, t), k, _lin(terms, qs.__getitem__))

    def prep_qkv(src, slot, k, rows, n=16, tiles=range(4)):
        jobs = []
        for r in range(0, rows, n):
            st = {}
            jobs.append([[(20, part(qkv_cols, st, src, k + r, n, hf)) for hf in range(2)],
                         [(22, part(qkv_ops, st, slot, k + r, t)) for t in tiles]])
        return _pipeline(jobs, 1)

    def wo_rows(st, h, jh, c, i, tok):
        tie_w(tok)
        st[i] = _perm_words([pltpu.bitcast(w_v[2 * O_ + jh, _rows(jl * 128 + h * 32 + (i // 2 ^ jh) * 16, 16),
                                               pl.ds(i % 2 * DHF + c * 128, 128)], U32) for jl in range(4)])

    def wo_ops(st, h, jh, c, tl, tok):
        qs = [pltpu.bitcast(st[i][tl], BF16).astype(F32) for i in range(4)]
        for m, terms in enumerate(RHS):
            _put(*b1_at(1, m, c), tl * 128 + h * 32 + jh * 16, _lin(terms, qs.__getitem__))

    def prep_wo(h, jh, c):
        st = {}
        return ([(15, part(wo_rows, st, h, jh, c, i)) for i in range(4)] +
                [(25, part(wo_ops, st, h, jh, c, i)) for i in range(4)])

    def gu_sum(st, src, k, n, mo, tok):
        tie_w(tok)
        block = lambda qo, qi: w_v[src + qo // 2, _rows(k + qi // 2 * 256, 16),
                                   pl.ds(n * FC + qo % 2 * 256 + qi % 2 * 128, 128)].astype(F32)
        st["q"] = [_lin(RHS[mo], lambda qo: block(qo, qi)) for qi in range(4)]

    def gu_ops(st, slot, k, n, mo, inner, tok):
        for mi in inner:
            _put(*g_at(slot, mo, mi, n), k, _lin(RHS[mi], st["q"].__getitem__))

    def prep_gu(src, slot, k, n, mo):
        st = {}
        return [(24, part(gu_sum, st, src, k, n, mo)),
                (12, part(gu_ops, st, slot, k, n, mo, (0, 1, 2, 3))), (12, part(gu_ops, st, slot, k, n, mo, (4, 5, 6)))]

    def prep_down(src, slot, k, t, tok):
        tie_w(tok)
        qs = [w_v[src, _rows(k + r0, 16), pl.ds(t * 128 + c0, 128)].astype(F32)
              for r0 in (0, FC // 2) for c0 in (0, DHF)]
        for m, terms in enumerate(RHS):
            _put(b2_s, (slot, m, t), k, _lin(terms, qs.__getitem__))

    def prep_glu(src_gu, src_d, slot, i, n):
        kk = 256 // n
        gu = [[x for r in range(0, kk, 16) for c in range(2) for mo in outer
               for x in prep_gu(src_gu, slot, i * kk + r, c, mo)] for outer in (ORDER[:GA], ORDER[GA:])]
        return gu[0], gu[1], [(25, part(prep_down, src_d, slot, i * kk + r, t))
                              for r in range(0, kk, 16) for t in range(4)]

    def lane_add(x, bit):
        lane = jax.lax.broadcasted_iota(jnp.int32, x.shape, 1)
        return x + jnp.take_along_axis(x, lane ^ bit, axis=1)

    def qk(st, r, t0, tok):
        tie_qkv(tok)
        for t in range(t0, t0 + 4):
            q = qkv_s[Q_, t, pl.ds(r + HALO, 8), :]
            ys = [q * qkv_s[K_, t, pl.ds(r + (HALO - DIL * w), 8), :] for w in range(W)]
            st["l"] = ys if t == 0 else [l + y for l, y in zip(st["l"], ys)]
        if t0:
            st["l"] = [lane_add(l, 1) for l in st["l"]]

    def logits(st, r, edge, tok):
        row = r + jax.lax.broadcasted_iota(jnp.int32, (8, 128), 0)
        ls = [lane_add(l, 2) * DH ** -0.5 for l in st["l"]]
        st["l"] = [jnp.where(row >= DIL * w, l, -1e9) if edge and w else l for w, l in enumerate(ls)]

    def softmax(st, tok):
        mx = functools.reduce(jnp.maximum, st["l"])
        es = [jnp.exp(l - mx) for l in st["l"]]
        inv = 1.0 / functools.reduce(jnp.add, es)
        st["p"] = [e * inv for e in es]

    def pv(st, r, s, hf, sub, t0, tok):
        tie_qkv(tok)
        for t in range(t0, t0 + 4):
            t_s[s, hf, t, pl.ds(sub, 8), :] = functools.reduce(
                jnp.add, [st["p"][w] * qkv_s[V_, t, pl.ds(r + (HALO - DIL * w), 8), :] for w in range(W)])

    def attn_ops(p, s, t, tok):
        t_s[2, 0, 0, _ds(zero(), 8, 8), :] = tok
        qs = [t_s[s, hf, t + c] for hf in range(2) for c in (0, 4)]
        for m, terms in enumerate(LHS):
            _put(a_s, (m, t), p, _lin(terms, qs.__getitem__))

    def attend(ps):
        out, late = [], []
        for i, p in enumerate(ps):
            for hf in range(2):
                for sub in (0, 8):
                    st, r = {}, hf * SH + p + sub
                    out += [(64, part(qk, st, r, t0)) for t0 in (0, 4)] + late[:len(late) // 2]
                    out += [(30, part(logits, st, r, (i, hf) == (0, 0)))] + late[len(late) // 2:]
                    out += [(40, part(softmax, st))]
                    late = [(60, part(pv, st, r, i % 2, hf, sub, t0)) for t0 in (0, 4)]
            late += [(17, part(attn_ops, p, i % 2, t)) for t in range(4)]
        return out + late

    def project(u, slot, p, n):
        ms = {}

        def dot(m, t):
            r = p + (0 if isinstance(p, int) else zero())
            ms[m] = _mm([_get(a_s, (m, i), r, n) for i in range(4)], [_get(*b1_at(slot, m, t))])
            for r in range(0, n, 32) if m in DONE else ():
                i = DONE[m]
                qkv_s[u, (i % 2) * 4 + t, _ds(HALO + (i // 2) * SH + p + r, 32, 8), :] = _lin(
                    OUT[i], lambda j: ms[j][r:r + 32])
            return ms[m]
        share = (1, 0.8, 1.1, 0.8, 1.1, 0.8, 0.8)
        return _quiet_tail([(share[i], part(dot, m, t)) for t in range(4) for i, m in enumerate(ORDER)])

    def project_slice(ks, p, n, m):
        y = _mm([_get(a_s, (m, s), p, n) for s in ks],
                [_get(*b1_at(0, m, t), ks[0] * 128, len(ks) * 128) for t in range(4)])
        for t in range(4):
            at = lambda j: (V_, t, pl.ds(j * 2 * XB + p, n))
            v = y[:, t * 128:(t + 1) * 128]
            if ks[0]:
                v = qkv_s[at(m)] + v
            if ks[-1] < 3 or m not in ORDER[-2:]:
                qkv_s[at(m)] = v
            if ks[-1] == 3 and m in DONE:
                i = DONE[m]
                qkv_s[K_, (i % 2) * 4 + t, pl.ds(HALO + (i // 2) * SH + p, n), :] = _lin(
                    OUT[i], lambda j: v if j == m else qkv_s[at(j)])
        return y

    def glu(slot, r0, first):
        n = P // 2
        inner, hs = {}, {}
        again = zero() * 2

        def up(mo, mi):
            r = r0 + zero()
            y = inner[mi] = _mm([_get(a2_s, (mo * 7 + mi, i), r, n) for i in range(2)],
                                [_get(*g_at(slot, mo, mi, i)) for i in range(2)])
            for r in range(0, n, 16) if mi in DONE else ():
                ci = DONE[mi]
                vs = [_lin(OUT[ci], lambda j: inner[j][r:r + 16, c:c + 128]) for c in (0, 128)]
                if mo not in ORDER[-2:]:
                    for i in range(2):
                        m_s[mo, pl.ds((2 * ci + i) * n + r, 16), :] = vs[i]
                if mo in DONE:
                    co = DONE[mo]
                    r1 = r + again if co == 3 else r
                    g, u = (_lin(OUT[co], lambda j: vs[i] if j == mo else m_s[j, _rows((2 * ci + i) * n + r1, 16), :])
                            for i in range(2))
                    hs[co, ci, r] = g * u
                    for j, terms in enumerate(LHS):
                        need = [i for i, _ in terms]
                        if co in need and all((i, ci, r) in hs for i in need):
                            _put(h_s, (j, ci % 2), ci // 2 * n + r, _lin(terms, lambda i: hs[i, ci, r]))
            return y

        def down(m, t):
            r = zero() * 4 if t else 0
            y = _mm([_get(h_s, (m, i), r, P) for i in range(2)], [_get(b2_s, (slot, m, t + i)) for i in range(2)])
            for hf in range(2):
                idx = (m, _rows(r0 + hf * (SH // 2), n), pl.ds(t * 128, 256))
                acc_s[idx] = jnp.where(first, 0.0, acc_s[idx]) + y[hf * n:(hf + 1) * n]
            return y
        so, si, sd = (1, 1, 1, 1, 1, 0.7, 0.4), (1, 1, 1, 1, 1, 1, 1), (1, 1, 1, 1, 1, 0.7, 0)
        return ([(so[k] * si[i], part(up, mo, mi)) for k, mo in enumerate(ORDER) for i, mi in enumerate(ORDER)],
                [(sd[k], part(down, m, t)) for k, m in enumerate((2, 4, 5, 3, 6, 1, 0)) for t in (0, 2)])

    for cp in (x_copy(0), k_copy(0), k_copy(1), x_copy(1), k_copy(2), k_copy(3)):
        cp.start()
    for b in range(2, SH // XB):
        x_copy(b).start()
    w_copy(Q_).start()
    w_copy(V_).start()
    for c in range(NCH):
        for cp in f_copies(c):
            cp.start()
    w_copy(O_).start()
    qkv_s[K_, :, pl.ds(0, HALO), :] = jnp.zeros((8, HALO, 128), F32)

    def first_rows(i, c):
        for _, f in layer_norm(i * (XB // 2), XB // 2):
            f(None)
        return (c + i) >> 1

    x_copy(0).wait()
    step[1] = jax.lax.fori_loop(0, 2, first_rows, 0)
    k_copy(0).wait()
    for _, f in prep_qkv(K_, 0, 0, 128, 32):
        f(None)
    for ks, p, n, s, blocks in (((0,), 0, XB, 1, ()), ((1,), 0, XB, 0, (1,)), ((0, 1), XB, XB, 2, ()),
                                ((2,), 0, 2 * XB, 3, (2,)), ((3,), 0, 2 * XB, 0, (3,)),
                                ((), 2 * XB, 2 * XB, 0, (4, 5, 6, 7))):
        side = []
        if s:
            k_copy(s).wait()
            side.append(prep_qkv(K_, 0, s * 128, 128))
        for b in blocks:
            x_copy(b).wait()
        if blocks:
            side.append(layer_norm(blocks[0] * XB, len(blocks) * XB))
        dots = _quiet_tail([(1, part(project_slice, ks, p, n, m)) for m in ORDER]) if ks else project(K_, 0, p, n)
        _interleave(dots, _merge(*side))

    w_copy(Q_).wait()

    @pl.loop(0, 5)
    def _(it):
        step[1] = it
        u, quarter = (it + 1) >> 1, jnp.maximum(it - 1, 0)

        @pl.when(it == 1)
        def _():
            w_copy(V_).wait()
            for cp in f_copies(0):
                cp.wait()

        nxt = [prep_qkv(jnp.minimum(u + 1, V_), 1 - (u & 1), 0, DHF, tiles=ts) for ts in ((0, 1), (2, 3))]
        ga, gb, dn = prep_glu(jnp.where(it == 0, 0, 2 * GU_), jnp.where(it == 0, 0, DN_), 0, quarter, 4)
        x2 = [x for r in range(0, 128, 16) for t in range(2) for mo in range(7)
              for x in prep_x2(quarter * 128 + r, t, mo)]
        rest = _merge(ga + gb, dn, x2)
        dots = project(u, u & 1, ((it + 1) & 1) * P, P)
        _interleave(_quiet_tail(dots[:14]), _merge(nxt[1], rest[:len(rest) // 2]))
        _interleave(dots[14:], _merge(nxt[0], rest[len(rest) // 2:]))

    for t in range(8):
        qkv_s[V_, t, pl.ds(0, HALO), :] = jnp.broadcast_to(qkv_s[V_, t, pl.ds(HALO, 1), :], (HALO, 128))
    w_copy(O_).wait()
    for c in range(1, NCH):
        for cp in f_copies(c):
            cp.wait()

    @pl.loop(0, 2 * NCH)
    def _(it):
        step[1] = it
        c, b = it >> 1, it & 1
        nxt = jnp.minimum(c + 1, NCH - 1)
        extra = jnp.where(it < 8, it, 0)
        ga, gb, dn = prep_glu(2 * (GU_ + nxt), DN_ + nxt, 1 - (c & 1), b, 2)
        rest = _merge(attend([it * 64 + i * 16 for i in range(4)] + [2 * NCH * 64 + extra * 16]),
                      [x for t in range(4) for x in prep_wo(extra >> 1, extra & 1, t)])
        ups, downs = glu(c & 1, b * (P // 2), c == 0)
        h0, h1, g0 = int(len(rest) * 0.37), int(len(rest) * 0.84), int(len(ga) // 3 * 0.14) * 3
        _interleave(_quiet_tail(ups[:7 * GA]), _merge(gb, rest[:h0]))
        _interleave(_quiet_tail(ups[7 * GA:]), _merge(dn + ga[:g0], rest[h0:h1]))
        _interleave(downs, _merge(ga[g0:], rest[h1:]))

    @pl.loop(0, SH // P_OUT)
    def _(it):
        step[1] = it
        for j, n in enumerate(R_OUT):
            p = it * P_OUT + sum(R_OUT[:j])
            for t in range(4):
                r = p + zero()
                ms = [acc_s[m, _rows(p, n), pl.ds(t * 128, 128)] +
                      _mm([_get(a_s, (m, i), r, n) for i in range(4)], [_get(*b1_at(1, m, t))]) for m in range(7)]
                for i, terms in enumerate(OUT):
                    idx = (i // 2, _rows(p, n), pl.ds((i % 2) * DHF + t * 128, 128))
                    x_v[idx] = (x_v[idx].astype(F32) + _lin(terms, ms.__getitem__)).astype(BF16)
            o_copy(it, j).start()

    for i in range(SH // P_OUT):
        for j in range(len(R_OUT)):
            o_copy(i, j).wait()


@jax.jit
def pallas_parallel_sum__sliding_local_dilated__glu_gated_bilinear__prompt_kernel(
    A_x: jax.Array,
    A_wqkv: jax.Array,
    A_wo: jax.Array,
    B_x: jax.Array,
    B_w_gate: jax.Array,
    B_w_up: jax.Array,
    B_w_down: jax.Array,
):
    del B_x
    hbm = pl.BlockSpec(memory_space=pl.ANY)
    vmem, dma = pltpu.VMEM, pltpu.SemaphoreType.DMA
    operand = lambda *shape: vmem((*shape, 128), BF16)
    out = pl.pallas_call(
        _kernel,
        in_specs=[hbm] * 6,
        out_specs=hbm,
        out_shape=jax.ShapeDtypeStruct((2, SH, D), BF16),
        scratch_shapes=[
            vmem((2, SH + 16, D), BF16),
            vmem((DN_ + NCH, DHF + 16, D), BF16),
            operand(7, 4, SH),
            operand(49, 2, SH // 2),
            [operand(2, 7, 2, DHF)] * 2,
            [operand(2, 7 * GA, 2, 256), operand(2, 7 * (7 - GA), 2, 256)],
            operand(2, 7, 4, FC // 2),
            operand(7, 2, P),
            vmem((5, 4 * P, 128), F32),
            vmem((7, SH, DHF), F32),
            vmem((3, 8, S + HALO + 8, 128), F32),
            vmem((3, 2, 8, 16, 128), F32),
            dma((SH // XB,)), dma((4,)), dma((4,)), dma((3 * NCH,)), dma((SH // P_OUT * len(R_OUT),)),
        ],
        compiler_params=pltpu.CompilerParams(vmem_limit_bytes=127 * 2**20),
        name="fused",
    )(A_x.reshape(2, SH, D), A_wqkv.reshape(2, DHF, 3 * D), A_wo.reshape(2, DHF, D),
      B_w_gate.reshape(2, DHF, F), B_w_up.reshape(2, DHF, F), B_w_down)
    return out.reshape(A_x.shape)
```

```python
import functools

import jax
import jax.numpy as jnp
import jax.experimental.pallas as pl
import jax.experimental.pallas.tpu as pltpu

S, D, F = 2048, 1024, 3584
DH, W, DIL = 32, 8, 2
HALO = 16
SH, DHF = S // 2, D // 2
FC = 512
NCH = F // FC
XB = 128
P = 512
P_OUT = 256
R_OUT = (192, 64)
GA = 3
F32, BF16, U32 = jnp.float32, jnp.bfloat16, jnp.uint32
K_, Q_, V_, O_, GU_ = 0, 1, 2, 3, 4
DN_ = 2 * (GU_ + NCH)

LHS = (((0, 1), (3, 1)), ((2, 1), (3, 1)), ((0, 1),), ((3, 1),),
       ((0, 1), (1, 1)), ((2, 1), (0, -1)), ((1, 1), (3, -1)))
RHS = (((0, 1), (3, 1)), ((0, 1),), ((1, 1), (3, -1)), ((2, 1), (0, -1)),
       ((3, 1),), ((0, 1), (1, 1)), ((2, 1), (3, 1)))
OUT = (((6, 1), (0, 1), (3, 1), (4, -1)), ((2, 1), (4, 1)),
       ((3, 1), (1, 1)), ((5, 1), (0, 1), (1, -1), (2, 1)))
ORDER = (1, 3, 4, 2, 0, 6, 5)
DONE = {3: 2, 2: 1, 6: 0, 5: 3}


def _lin(terms, get):
    acc = get(terms[0][0])
    for i, sign in terms[1:]:
        acc = acc + get(i) if sign > 0 else acc - get(i)
    return acc


def _ds(start, n, align):
    return pl.ds(start if isinstance(start, int) else pl.multiple_of(start, align), n)


def _rows(start, n):
    return _ds(start, n, 16)


def _put(ref, idx, start, v):
    ref[(*idx, _rows(start, v.shape[0]))] = v.astype(BF16)


def _get(ref, idx, start=0, n=None):
    words = ref.bitcast(U32)[(*idx, _ds(start >> 1, (n or ref.shape[-2]) // 2, 8))]
    return pltpu.bitcast(words, BF16)


def _mm(a, b):
    cat = lambda v: v[0] if len(v) == 1 else jnp.concatenate(v, axis=1)
    return jnp.dot(cat(a), cat(b), preferred_element_type=F32)


def _skew4(vs, pos, unit):
    cur = [vs[(-t) % 4] for t in range(4)]
    for b in (1, 2):
        m = (pos & (b * unit)) != 0
        cur = [jnp.where(m, cur[(t - b) % 4], cur[t]) for t in range(4)]
    return cur


def _perm_lanes(vs):
    lane = jax.lax.broadcasted_iota(jnp.int32, vs[0].shape, 1)
    lo, hi = _skew4(vs[:4], lane, 4), _skew4(vs[4:], lane, 4)
    m = (lane & 16) != 0
    mixed = [jnp.where(m, b, a) for a, b in zip(lo, hi)] + [jnp.where(m, a, b) for a, b in zip(lo, hi)]
    return [v if t == 0 else
            jnp.take_along_axis(v, ((lane & 115) ^ (t // 4 * 16)) | ((lane + t % 4 * 4) & 12), axis=1)
            for t, v in enumerate(mixed)]


def _perm_words(vs):
    row = jax.lax.broadcasted_iota(jnp.int32, vs[0].shape, 0)
    return [v if t == 0 else pltpu.roll(v, 8 - 2 * t, 0) for t, v in enumerate(_skew4(vs, row, 2))]


def _merge(*lists):
    keyed = []
    for xs in lists:
        tot, done = sum(w for w, _ in xs), 0
        for w, f in xs:
            keyed.append(((done + w / 2) / tot, w, f))
            done += w
    return [(w, f) for _, w, f in sorted(keyed, key=lambda t: t[0])]


def _pipeline(jobs, dist):
    n, out = len(jobs[0]), []
    for i in range(len(jobs) + (n - 1) * dist):
        for st in range(n):
            if 0 <= i - st * dist < len(jobs):
                out += jobs[i - st * dist][st]
    return out


def _interleave(dots, side):
    tot, share = sum(w for w, _ in side), sum(w for w, _ in dots)
    done, j, cum = 0, 0, 0
    for w, dot in dots:
        src = dot()
        lo = tot * cum / share
        cum += w
        hi = tot * cum / share
        while j < len(side) and done < hi - 1e-6:
            pos = min(max((done - lo) / (hi - lo), 0.0), 0.999) * (src.shape[1] // 128)
            r0, c0 = int(pos % 1 * src.shape[0]) // 8 * 8, int(pos) * 128
            side[j][1](src[r0:r0 + 8, c0:c0 + 128])
            done += side[j][0]
            j += 1
    assert j == len(side)


def _quiet_tail(dots):
    return dots[:-1] + [(0, dots[-1][1])]


def _kernel(x_hbm, wqkv_hbm, wo_hbm, wg_hbm, wu_hbm, wd_hbm, o_hbm,
            x_v, w_v, a_s, a2_s, b1_s, g_s, b2_s, h_s, m_s, acc_s, qkv_s, t_s,
            sem_x, sem_k, sem_w, sem_f, sem_o):
    part = functools.partial
    step = [0, None]

    def zero():
        step[0] += 1
        return jax.lax.shift_right_logical(step[1] + step[0], 24) * 16

    def tie_x(tok):
        if tok is not None:
            x_v[0, _rows(zero() + SH, 16), pl.ds(0, 128)] = pltpu.bitcast(tok, BF16)

    def tie_w(tok):
        if tok is not None:
            w_v[0, _rows(zero() + DHF, 16), pl.ds(0, 128)] = pltpu.bitcast(tok, BF16)

    def tie_qkv(tok):
        qkv_s[0, 0, _ds(zero() + S + HALO, 8, 8), :] = tok

    def x_copy(b):
        rows = _rows(b * XB, XB)
        return pltpu.make_async_copy(x_hbm.at[:, rows], x_v.at[:, rows], sem_x.at[b])

    def k_copy(s):
        rows = pl.ds(s * 128, 128)
        return pltpu.make_async_copy(wqkv_hbm.at[:, rows, pl.ds(D, D)], w_v.at[pl.ds(2 * K_, 2), rows], sem_k.at[s])

    def w_copy(i):
        src = wo_hbm if i == O_ else wqkv_hbm.at[:, :, pl.ds(0 if i == Q_ else 2 * D, D)]
        return pltpu.make_async_copy(src, w_v.at[pl.ds(2 * i, 2), pl.ds(0, DHF)], sem_w.at[i])

    def f_copies(c):
        col, dst, rows = pl.ds(c * FC, FC), pl.ds(2 * (GU_ + c), 2), pl.ds(0, DHF)
        return [pltpu.make_async_copy(wg_hbm.at[:, :, col], w_v.at[dst, rows, pl.ds(0, FC)], sem_f.at[3 * c]),
                pltpu.make_async_copy(wu_hbm.at[:, :, col], w_v.at[dst, rows, pl.ds(FC, FC)], sem_f.at[3 * c + 1]),
                pltpu.make_async_copy(wd_hbm.at[col, :], w_v.at[DN_ + c, rows], sem_f.at[3 * c + 2])]

    def o_copy(i, j):
        rows = _rows(i * P_OUT + sum(R_OUT[:j]), R_OUT[j])
        return pltpu.make_async_copy(x_v.at[:, rows], o_hbm.at[:, rows], sem_o.at[i * len(R_OUT) + j])

    def row_mean(x):
        y = functools.reduce(jnp.add, [x[:, c:c + 128] for c in range(0, D, 128)])
        return jnp.sum(y, axis=-1, keepdims=True) * (1.0 / D)

    def ln_stats(st, p, hf, tok):
        tie_x(tok)
        x = x_v[hf, _rows(p, 16), :].astype(F32)
        mu = row_mean(x)
        xc = x - mu
        st[hf] = (mu, jax.lax.rsqrt(row_mean(xc * xc) + 1e-5))
        for i in range(2):
            acc_s[0, _rows(p, 16), pl.ds(i * 256 + hf * 128, 128)] = jnp.broadcast_to(st[hf][i], (16, 128))

    def ln_ops(st, p, t, tok):
        tie_x(tok)
        qs = [(x_v[hf, _rows(p, 16), pl.ds(c + t * 128, 128)].astype(F32) - st[hf][0]) * st[hf][1]
              for hf in range(2) for c in (0, DHF)]
        for m, terms in enumerate(LHS):
            _put(a_s, (m, t), p, _lin(terms, qs.__getitem__))

    def layer_norm(p, n):
        jobs = []
        for r in range(0, n, 16):
            st = {}
            jobs.append([[(70, part(ln_stats, st, p + r, hf)) for hf in range(2)],
                         [(45, part(ln_ops, st, p + r, t)) for t in range(4)]])
        return _pipeline(jobs, 6)

    def x_sum(st, r, t, mo, qi, tok):
        tie_x(tok)
        rows = _rows(qi // 2 * (SH // 2) + r, 16)

        def block(qo):
            x = x_v[qo // 2, rows, pl.ds(qo % 2 * DHF + qi % 2 * 256 + t * 128, 128)].astype(F32)
            return (x - acc_s[0, rows, pl.ds(qo // 2 * 128, 128)]) * acc_s[0, rows, pl.ds(256 + qo // 2 * 128, 128)]
        st[qi] = _lin(LHS[mo], block)

    def x_ops(st, r, t, mo, tok):
        for mi, terms in enumerate(LHS):
            _put(a2_s, (mo * 7 + mi, t), r, _lin(terms, st.get))

    def prep_x2(r, t, mo):
        st = {}
        return [(18, part(x_sum, st, r, t, mo, qi)) for qi in range(4)] + [(7, part(x_ops, st, r, t, mo))]

    def b1_at(slot, m, t):
        return b1_s[t // 2], (slot, m, t % 2)

    def g_at(slot, mo, mi, n):
        g = ORDER.index(mo)
        return (g_s[0], (slot, g * 7 + mi, n)) if g < GA else (g_s[1], (slot, (g - GA) * 7 + mi, n))

    def qkv_cols(st, src, k, n, hf, tok):
        tie_w(tok)
        st[hf] = _perm_lanes([pltpu.bitcast(w_v[2 * src + hf, _rows(k, n), pl.ds(j * 128, 128)], U32)
                              for j in range(8)])

    def qkv_ops(st, slot, k, t, tok):
        qs = [pltpu.bitcast(st[hf][t + c], BF16).astype(F32) for hf in range(2) for c in (0, 4)]
        for m, terms in enumerate(RHS):
            _put(*b1_at(slot, m, t), k, _lin(terms, qs.__getitem__))

    def prep_qkv(src, slot, k, rows, n=16, tiles=range(4)):
        jobs = []
        for r in range(0, rows, n):
            st = {}
            jobs.append([[(20, part(qkv_cols, st, src, k + r, n, hf)) for hf in range(2)],
                         [(28, part(qkv_ops, st, slot, k + r, t)) for t in tiles]])
        return _pipeline(jobs, 1)

    def wo_rows(st, h, jh, c, i, tok):
        tie_w(tok)
        st[i] = _perm_words([pltpu.bitcast(w_v[2 * O_ + jh, _rows(jl * 128 + h * 32 + (i // 2 ^ jh) * 16, 16),
                                               pl.ds(i % 2 * DHF + c * 128, 128)], U32) for jl in range(4)])

    def wo_ops(st, h, jh, c, tl, tok):
        qs = [pltpu.bitcast(st[i][tl], BF16).astype(F32) for i in range(4)]
        for m, terms in enumerate(RHS):
            _put(*b1_at(1, m, c), tl * 128 + h * 32 + jh * 16, _lin(terms, qs.__getitem__))

    def prep_wo(h, jh, c):
        st = {}
        return ([(15, part(wo_rows, st, h, jh, c, i)) for i in range(4)] +
                [(25, part(wo_ops, st, h, jh, c, i)) for i in range(4)])

    def gu_sum(st, src, k, n, mo, tok):
        tie_w(tok)
        block = lambda qo, qi: w_v[src + qo // 2, _rows(k + qi // 2 * 256, 16),
                                   pl.ds(n * FC + qo % 2 * 256 + qi % 2 * 128, 128)].astype(F32)
        st["q"] = [_lin(RHS[mo], lambda qo: block(qo, qi)) for qi in range(4)]

    def gu_ops(st, slot, k, n, mo, inner, tok):
        for mi in inner:
            _put(*g_at(slot, mo, mi, n), k, _lin(RHS[mi], st["q"].__getitem__))

    def prep_gu(src, slot, k, n, mo):
        st = {}
        return [(24, part(gu_sum, st, src, k, n, mo)),
                (6, part(gu_ops, st, slot, k, n, mo, (0, 1, 2, 3))), (6, part(gu_ops, st, slot, k, n, mo, (4, 5, 6)))]

    def prep_down(src, slot, k, t, tok):
        tie_w(tok)
        qs = [w_v[src, _rows(k + r0, 16), pl.ds(t * 128 + c0, 128)].astype(F32)
              for r0 in (0, FC // 2) for c0 in (0, DHF)]
        for m, terms in enumerate(RHS):
            _put(b2_s, (slot, m, t), k, _lin(terms, qs.__getitem__))

    def prep_glu(src_gu, src_d, slot, i, n):
        kk = 256 // n
        gu = [[x for r in range(0, kk, 16) for c in range(2) for mo in outer
               for x in prep_gu(src_gu, slot, i * kk + r, c, mo)] for outer in (ORDER[:GA], ORDER[GA:])]
        return gu[0], gu[1], [(25, part(prep_down, src_d, slot, i * kk + r, t))
                              for r in range(0, kk, 16) for t in range(4)]

    def lane_add(x, bit):
        lane = jax.lax.broadcasted_iota(jnp.int32, x.shape, 1)
        return x + jnp.take_along_axis(x, lane ^ bit, axis=1)

    def qk(st, r, t0, tok):
        tie_qkv(tok)
        for t in range(t0, t0 + 4):
            q = qkv_s[Q_, t, pl.ds(r + HALO, 8), :]
            ys = [q * qkv_s[K_, t, pl.ds(r + (HALO - DIL * w), 8), :] for w in range(W)]
            st["l"] = ys if t == 0 else [l + y for l, y in zip(st["l"], ys)]
        if t0:
            st["l"] = [lane_add(l, 1) for l in st["l"]]

    def logits(st, r, edge, tok):
        row = r + jax.lax.broadcasted_iota(jnp.int32, (8, 128), 0)
        ls = [lane_add(l, 2) * DH ** -0.5 for l in st["l"]]
        st["l"] = [jnp.where(row >= DIL * w, l, -1e9) if edge and w else l for w, l in enumerate(ls)]

    def softmax(st, tok):
        mx = functools.reduce(jnp.maximum, st["l"])
        es = [jnp.exp(l - mx) for l in st["l"]]
        inv = 1.0 / functools.reduce(jnp.add, es)
        st["p"] = [e * inv for e in es]

    def pv(st, r, s, hf, sub, t0, tok):
        tie_qkv(tok)
        for t in range(t0, t0 + 4):
            t_s[s, hf, t, pl.ds(sub, 8), :] = functools.reduce(
                jnp.add, [st["p"][w] * qkv_s[V_, t, pl.ds(r + (HALO - DIL * w), 8), :] for w in range(W)])

    def attn_ops(p, s, t, tok):
        t_s[2, 0, 0, _ds(zero(), 8, 8), :] = tok
        qs = [t_s[s, hf, t + c] for hf in range(2) for c in (0, 4)]
        for m, terms in enumerate(LHS):
            _put(a_s, (m, t), p, _lin(terms, qs.__getitem__))

    def attend(ps):
        out, late = [], []
        for i, p in enumerate(ps):
            for hf in range(2):
                for sub in (0, 8):
                    st, r = {}, hf * SH + p + sub
                    out += [(64, part(qk, st, r, t0)) for t0 in (0, 4)] + late[:len(late) // 2]
                    out += [(30, part(logits, st, r, (i, hf) == (0, 0)))] + late[len(late) // 2:]
                    out += [(55, part(softmax, st))]
                    late = [(60, part(pv, st, r, i % 2, hf, sub, t0)) for t0 in (0, 4)]
            late += [(17, part(attn_ops, p, i % 2, t)) for t in range(4)]
        return out + late

    def project(u, slot, p, n):
        ms = {}

        def dot(m, t):
            r = p + (0 if isinstance(p, int) else zero())
            ms[m] = _mm([_get(a_s, (m, i), r, n) for i in range(4)], [_get(*b1_at(slot, m, t))])
            for r in range(0, n, 32) if m in DONE else ():
                i = DONE[m]
                qkv_s[u, (i % 2) * 4 + t, _ds(HALO + (i // 2) * SH + p + r, 32, 8), :] = _lin(
                    OUT[i], lambda j: ms[j][r:r + 32])
            return ms[m]
        share = (1, 0.7, 1.1, 0.7, 1.1, 0.8, 0.7)
        return _quiet_tail([(share[i], part(dot, m, t)) for t in range(4) for i, m in enumerate(ORDER)])

    def project_slice(ks, p, n, m):
        y = _mm([_get(a_s, (m, s), p, n) for s in ks],
                [_get(*b1_at(0, m, t), ks[0] * 128, len(ks) * 128) for t in range(4)])
        for t in range(4):
            at = lambda j: (V_, t, pl.ds(j * 2 * XB + p, n))
            v = y[:, t * 128:(t + 1) * 128]
            if ks[0]:
                v = qkv_s[at(m)] + v
            if ks[-1] < 3 or m not in ORDER[-2:]:
                qkv_s[at(m)] = v
            if ks[-1] == 3 and m in DONE:
                i = DONE[m]
                qkv_s[K_, (i % 2) * 4 + t, pl.ds(HALO + (i // 2) * SH + p, n), :] = _lin(
                    OUT[i], lambda j: v if j == m else qkv_s[at(j)])
        return y

    def glu(slot, r0, first):
        n = P // 2
        inner, hs = {}, {}
        again = zero() * 2

        def up(mo, mi):
            r = r0 + zero()
            y = inner[mi] = _mm([_get(a2_s, (mo * 7 + mi, i), r, n) for i in range(2)],
                                [_get(*g_at(slot, mo, mi, i)) for i in range(2)])
            for r in range(0, n, 16) if mi in DONE else ():
                ci = DONE[mi]
                vs = [_lin(OUT[ci], lambda j: inner[j][r:r + 16, c:c + 128]) for c in (0, 128)]
                if mo not in ORDER[-2:]:
                    for i in range(2):
                        m_s[mo, pl.ds((2 * ci + i) * n + r, 16), :] = vs[i]
                if mo in DONE:
                    co = DONE[mo]
                    r1 = r + again if co == 3 else r
                    g, u = (_lin(OUT[co], lambda j: vs[i] if j == mo else m_s[j, _rows((2 * ci + i) * n + r1, 16), :])
                            for i in range(2))
                    hs[co, ci, r] = g * u
                    for j, terms in enumerate(LHS):
                        need = [i for i, _ in terms]
                        if co in need and all((i, ci, r) in hs for i in need):
                            _put(h_s, (j, ci % 2), ci // 2 * n + r, _lin(terms, lambda i: hs[i, ci, r]))
            return y

        def down(m, t):
            r = zero() * 4 if t else 0
            y = _mm([_get(h_s, (m, i), r, P) for i in range(2)], [_get(b2_s, (slot, m, t + i)) for i in range(2)])
            for hf in range(2):
                idx = (m, _rows(r0 + hf * (SH // 2), n), pl.ds(t * 128, 256))
                acc_s[idx] = jnp.where(first, 0.0, acc_s[idx]) + y[hf * n:(hf + 1) * n]
            return y
        so, si, sd = (0.9, 1, 1, 1, 1, 0.8, 0.4), (1, 0.8, 1.1, 0.8, 1.1, 1, 0.9), (0.7, 1, 1, 1, 0.8, 0.7, 0)
        return ([(so[k] * si[i], part(up, mo, mi)) for k, mo in enumerate(ORDER) for i, mi in enumerate(ORDER)],
                [(sd[k], part(down, m, t)) for k, m in enumerate((2, 4, 5, 3, 6, 1, 0)) for t in (0, 2)])

    for cp in (x_copy(0), k_copy(0), k_copy(1), x_copy(1), k_copy(2), k_copy(3)):
        cp.start()
    for b in range(2, SH // XB):
        x_copy(b).start()
    w_copy(Q_).start()
    w_copy(V_).start()
    for c in range(NCH):
        for cp in f_copies(c):
            cp.start()
    w_copy(O_).start()
    qkv_s[K_, :, pl.ds(0, HALO), :] = jnp.zeros((8, HALO, 128), F32)

    def first_rows(i, c):
        for _, f in layer_norm(i * (XB // 2), XB // 2):
            f(None)
        return (c + i) >> 1

    x_copy(0).wait()
    step[1] = jax.lax.fori_loop(0, 2, first_rows, 0)
    k_copy(0).wait()
    for _, f in prep_qkv(K_, 0, 0, 128, 32):
        f(None)
    for ks, p, n, s, blocks in (((0,), 0, XB, 1, ()), ((1,), 0, XB, 0, (1,)), ((0, 1), XB, XB, 2, ()),
                                ((2,), 0, 2 * XB, 3, (2,)), ((3,), 0, 2 * XB, 0, (3,)),
                                ((), 2 * XB, 2 * XB, 0, (4, 5, 6, 7))):
        side = []
        if s:
            k_copy(s).wait()
            side.append(prep_qkv(K_, 0, s * 128, 128))
        for b in blocks:
            x_copy(b).wait()
        if blocks:
            side.append(layer_norm(blocks[0] * XB, len(blocks) * XB))
        dots = _quiet_tail([(1, part(project_slice, ks, p, n, m)) for m in ORDER]) if ks else project(K_, 0, p, n)
        _interleave(dots, _merge(*side))

    w_copy(Q_).wait()

    @pl.loop(0, 5)
    def _(it):
        step[1] = it
        u, quarter = (it + 1) >> 1, jnp.maximum(it - 1, 0)

        @pl.when(it == 1)
        def _():
            w_copy(V_).wait()
            for cp in f_copies(0):
                cp.wait()

        nxt = [prep_qkv(jnp.minimum(u + 1, V_), 1 - (u & 1), 0, DHF, tiles=ts) for ts in ((0, 1), (2, 3))]
        ga, gb, dn = prep_glu(jnp.where(it == 0, 0, 2 * GU_), jnp.where(it == 0, 0, DN_), 0, quarter, 4)
        x2 = [x for r in range(0, 128, 16) for t in range(2) for mo in range(7)
              for x in prep_x2(quarter * 128 + r, t, mo)]
        rest = _merge(ga + gb, dn, x2)
        dots = project(u, u & 1, ((it + 1) & 1) * P, P)
        half = int(len(rest) * 0.526)
        _interleave(_quiet_tail(dots[:14]), _merge(nxt[1], rest[:half]))
        _interleave(dots[14:], _merge(nxt[0], rest[half:]))

    for t in range(8):
        qkv_s[V_, t, pl.ds(0, HALO), :] = jnp.broadcast_to(qkv_s[V_, t, pl.ds(HALO, 1), :], (HALO, 128))
    w_copy(O_).wait()
    for c in range(1, NCH):
        for cp in f_copies(c):
            cp.wait()

    @pl.loop(0, 2 * NCH)
    def _(it):
        step[1] = it
        c, b = it >> 1, it & 1
        nxt = jnp.minimum(c + 1, NCH - 1)
        extra = jnp.where(it < 8, it, 0)
        ga, gb, dn = prep_glu(2 * (GU_ + nxt), DN_ + nxt, 1 - (c & 1), b, 2)
        rest = _merge(attend([it * 64 + i * 16 for i in range(4)] + [2 * NCH * 64 + extra * 16]),
                      [x for t in range(4) for x in prep_wo(extra >> 1, extra & 1, t)])
        ups, downs = glu(c & 1, b * (P // 2), c == 0)
        h0, h1, g0 = int(len(rest) * 0.302), int(len(rest) * 0.897), int(len(ga) // 3 * 0.08) * 3
        _interleave(_quiet_tail(ups[:7 * GA]), _merge(gb, rest[:h0]))
        _interleave(_quiet_tail(ups[7 * GA:]), _merge(dn + ga[:g0], rest[h0:h1]))
        _interleave(downs, _merge(ga[g0:], rest[h1:]))

    @pl.loop(0, SH // P_OUT)
    def _(it):
        step[1] = it
        for j, n in enumerate(R_OUT):
            p = it * P_OUT + sum(R_OUT[:j])
            for t in range(4):
                r = p + zero()
                ms = [acc_s[m, _rows(p, n), pl.ds(t * 128, 128)] +
                      _mm([_get(a_s, (m, i), r, n) for i in range(4)], [_get(*b1_at(1, m, t))]) for m in range(7)]
                for i, terms in enumerate(OUT):
                    idx = (i // 2, _rows(p, n), pl.ds((i % 2) * DHF + t * 128, 128))
                    x_v[idx] = (x_v[idx].astype(F32) + _lin(terms, ms.__getitem__)).astype(BF16)
            o_copy(it, j).start()

    for i in range(SH // P_OUT):
        for j in range(len(R_OUT)):
            o_copy(i, j).wait()


@jax.jit
def pallas_parallel_sum__sliding_local_dilated__glu_gated_bilinear__prompt_kernel(
    A_x: jax.Array,
    A_wqkv: jax.Array,
    A_wo: jax.Array,
    B_x: jax.Array,
    B_w_gate: jax.Array,
    B_w_up: jax.Array,
    B_w_down: jax.Array,
):
    del B_x
    hbm = pl.BlockSpec(memory_space=pl.ANY)
    vmem, dma = pltpu.VMEM, pltpu.SemaphoreType.DMA
    operand = lambda *shape: vmem((*shape, 128), BF16)
    out = pl.pallas_call(
        _kernel,
        in_specs=[hbm] * 6,
        out_specs=hbm,
        out_shape=jax.ShapeDtypeStruct((2, SH, D), BF16),
        scratch_shapes=[
            vmem((2, SH + 16, D), BF16),
            vmem((DN_ + NCH, DHF + 16, D), BF16),
            operand(7, 4, SH),
            operand(49, 2, SH // 2),
            [operand(2, 7, 2, DHF)] * 2,
            [operand(2, 7 * GA, 2, 256), operand(2, 7 * (7 - GA), 2, 256)],
            operand(2, 7, 4, FC // 2),
            operand(7, 2, P),
            vmem((5, 4 * P, 128), F32),
            vmem((7, SH, DHF), F32),
            vmem((3, 8, S + HALO + 8, 128), F32),
            vmem((3, 2, 8, 16, 128), F32),
            dma((SH // XB,)), dma((4,)), dma((4,)), dma((3 * NCH,)), dma((SH // P_OUT * len(R_OUT),)),
        ],
        compiler_params=pltpu.CompilerParams(vmem_limit_bytes=127 * 2**20,
                                             flags={"XLA_TPU_EVENLY_DISTRIBUTE_CRITICAL_NODES": True}),
        name="fused",
    )(A_x.reshape(2, SH, D), A_wqkv.reshape(2, DHF, 3 * D), A_wo.reshape(2, DHF, D),
      B_w_gate.reshape(2, DHF, F), B_w_up.reshape(2, DHF, F), B_w_down)
    return out.reshape(A_x.shape)
```

```python
import functools

import jax
import jax.numpy as jnp
import jax.experimental.pallas as pl
import jax.experimental.pallas.tpu as pltpu

S, D, F = 2048, 1024, 3584
DH, W, DIL = 32, 8, 2
HALO = 16
SH, DHF = S // 2, D // 2
FC = 512
NCH = F // FC
XB = 128
P = 512
P_OUT = 256
R_OUT = (192, 64)
GA = 3
F32, BF16, U32 = jnp.float32, jnp.bfloat16, jnp.uint32
K_, Q_, V_, O_, GU_ = 0, 1, 2, 3, 4
DN_ = 2 * (GU_ + NCH)

LHS = (((0, 1), (3, 1)), ((2, 1), (3, 1)), ((0, 1),), ((3, 1),),
       ((0, 1), (1, 1)), ((2, 1), (0, -1)), ((1, 1), (3, -1)))
RHS = (((0, 1), (3, 1)), ((0, 1),), ((1, 1), (3, -1)), ((2, 1), (0, -1)),
       ((3, 1),), ((0, 1), (1, 1)), ((2, 1), (3, 1)))
OUT = (((6, 1), (0, 1), (3, 1), (4, -1)), ((2, 1), (4, 1)),
       ((3, 1), (1, 1)), ((5, 1), (0, 1), (1, -1), (2, 1)))
ORDER = (1, 3, 4, 2, 0, 6, 5)
DONE = {3: 2, 2: 1, 6: 0, 5: 3}


def _lin(terms, get):
    acc = get(terms[0][0])
    for i, sign in terms[1:]:
        acc = acc + get(i) if sign > 0 else acc - get(i)
    return acc


def _ds(start, n, align):
    return pl.ds(start if isinstance(start, int) else pl.multiple_of(start, align), n)


def _rows(start, n):
    return _ds(start, n, 16)


def _put(ref, idx, start, v):
    ref[(*idx, _rows(start, v.shape[0]))] = v.astype(BF16)


def _get(ref, idx, start=0, n=None):
    words = ref.bitcast(U32)[(*idx, _ds(start >> 1, (n or ref.shape[-2]) // 2, 8))]
    return pltpu.bitcast(words, BF16)


def _mm(a, b):
    cat = lambda v: v[0] if len(v) == 1 else jnp.concatenate(v, axis=1)
    return jnp.dot(cat(a), cat(b), preferred_element_type=F32)


def _skew4(vs, pos, unit):
    cur = [vs[(-t) % 4] for t in range(4)]
    for b in (1, 2):
        m = (pos & (b * unit)) != 0
        cur = [jnp.where(m, cur[(t - b) % 4], cur[t]) for t in range(4)]
    return cur


def _perm_lanes(vs):
    lane = jax.lax.broadcasted_iota(jnp.int32, vs[0].shape, 1)
    lo, hi = _skew4(vs[:4], lane, 4), _skew4(vs[4:], lane, 4)
    m = (lane & 16) != 0
    mixed = [jnp.where(m, b, a) for a, b in zip(lo, hi)] + [jnp.where(m, a, b) for a, b in zip(lo, hi)]
    return [v if t == 0 else
            jnp.take_along_axis(v, ((lane & 115) ^ (t // 4 * 16)) | ((lane + t % 4 * 4) & 12), axis=1)
            for t, v in enumerate(mixed)]


def _perm_words(vs):
    row = jax.lax.broadcasted_iota(jnp.int32, vs[0].shape, 0)
    return [v if t == 0 else pltpu.roll(v, 8 - 2 * t, 0) for t, v in enumerate(_skew4(vs, row, 2))]


def _merge(*lists):
    keyed = []
    for xs in lists:
        tot, done = sum(w for w, _ in xs), 0
        for w, f in xs:
            keyed.append(((done + w / 2) / tot, w, f))
            done += w
    return [(w, f) for _, w, f in sorted(keyed, key=lambda t: t[0])]


def _pipeline(jobs, dist):
    n, out = len(jobs[0]), []
    for i in range(len(jobs) + (n - 1) * dist):
        for st in range(n):
            if 0 <= i - st * dist < len(jobs):
                out += jobs[i - st * dist][st]
    return out


def _interleave(dots, side):
    tot, share = sum(w for w, _ in side), sum(w for w, _ in dots)
    done, j, cum = 0, 0, 0
    for w, dot in dots:
        src = dot()
        lo = tot * cum / share
        cum += w
        hi = tot * cum / share
        while j < len(side) and done < hi - 1e-6:
            pos = min(max((done - lo) / (hi - lo), 0.0), 0.999) * (src.shape[1] // 128)
            r0, c0 = int(pos % 1 * src.shape[0]) // 8 * 8, int(pos) * 128
            side[j][1](src[r0:r0 + 8, c0:c0 + 128])
            done += side[j][0]
            j += 1
    assert j == len(side)


def _quiet_tail(dots):
    return dots[:-1] + [(0, dots[-1][1])]


def _kernel(x_hbm, wqkv_hbm, wo_hbm, wg_hbm, wu_hbm, wd_hbm, o_hbm,
            x_v, w_v, a_s, a2_s, b1_s, g_s, b2_s, h_s, m_s, acc_s, qkv_s, t_s,
            sem_x, sem_k, sem_w, sem_o):
    part = functools.partial
    step = [0, None]

    def zero():
        step[0] += 1
        return jax.lax.shift_right_logical(step[1] + step[0], 24) * 16

    def tie_x(tok):
        if tok is not None:
            x_v[0, _rows(zero() + SH, 16), pl.ds(0, 128)] = pltpu.bitcast(tok, BF16)

    def tie_w(tok):
        if tok is not None:
            w_v[0, _rows(zero() + DHF, 16), pl.ds(0, 128)] = pltpu.bitcast(tok, BF16)

    def tie_qkv(tok):
        qkv_s[0, 0, _ds(zero() + S + HALO, 8, 8), :] = tok

    def x_copy(b):
        rows = _rows(b * XB, XB)
        return pltpu.make_async_copy(x_hbm.at[:, rows], x_v.at[:, rows], sem_x.at[b])

    def k_copy(s):
        rows = pl.ds(s * 128, 128)
        return pltpu.make_async_copy(wqkv_hbm.at[:, rows, pl.ds(D, D)], w_v.at[pl.ds(2 * K_, 2), rows], sem_k.at[s])

    def w_copy(i):
        src = wo_hbm if i == O_ else wqkv_hbm.at[:, :, pl.ds(0 if i == Q_ else 2 * D, D)]
        return pltpu.make_async_copy(src, w_v.at[pl.ds(2 * i, 2), pl.ds(0, DHF)], sem_w.at[i - Q_])

    def f_copies(c):
        col, dst, rows = pl.ds(c * FC, FC), pl.ds(2 * (GU_ + c), 2), pl.ds(0, DHF)
        sem = sem_w.at[(O_ if c else V_) - Q_]
        return [pltpu.make_async_copy(wg_hbm.at[:, :, col], w_v.at[dst, rows, pl.ds(0, FC)], sem),
                pltpu.make_async_copy(wu_hbm.at[:, :, col], w_v.at[dst, rows, pl.ds(FC, FC)], sem),
                pltpu.make_async_copy(wd_hbm.at[col, :], w_v.at[DN_ + c, rows], sem)]

    def o_copy(i, j):
        rows = _rows(i * P_OUT + sum(R_OUT[:j]), R_OUT[j])
        return pltpu.make_async_copy(x_v.at[:, rows], o_hbm.at[:, rows], sem_o.at[0])

    def row_mean(x):
        y = functools.reduce(jnp.add, [x[:, c:c + 128] for c in range(0, D, 128)])
        return jnp.sum(y, axis=-1, keepdims=True) * (1.0 / D)

    def ln_stats(st, p, hf, tok):
        tie_x(tok)
        x = x_v[hf, _rows(p, 16), :].astype(F32)
        mu = row_mean(x)
        xc = x - mu
        st[hf] = (mu, jax.lax.rsqrt(row_mean(xc * xc) + 1e-5))
        for i in range(2):
            acc_s[0, _rows(p, 16), pl.ds(i * 256 + hf * 128, 128)] = jnp.broadcast_to(st[hf][i], (16, 128))

    def ln_ops(st, p, t, tok):
        tie_x(tok)
        qs = [(x_v[hf, _rows(p, 16), pl.ds(c + t * 128, 128)].astype(F32) - st[hf][0]) * st[hf][1]
              for hf in range(2) for c in (0, DHF)]
        for m, terms in enumerate(LHS):
            _put(a_s, (m, t), p, _lin(terms, qs.__getitem__))

    def layer_norm(p, n):
        jobs = []
        for r in range(0, n, 16):
            st = {}
            jobs.append([[(70, part(ln_stats, st, p + r, hf)) for hf in range(2)],
                         [(45, part(ln_ops, st, p + r, t)) for t in range(4)]])
        return _pipeline(jobs, 6)

    def x_sum(st, r, t, mo, qi, tok):
        tie_x(tok)
        rows = _rows(qi // 2 * (SH // 2) + r, 16)

        def block(qo):
            x = x_v[qo // 2, rows, pl.ds(qo % 2 * DHF + qi % 2 * 256 + t * 128, 128)].astype(F32)
            return (x - acc_s[0, rows, pl.ds(qo // 2 * 128, 128)]) * acc_s[0, rows, pl.ds(256 + qo // 2 * 128, 128)]
        st[qi] = _lin(LHS[mo], block)

    def x_ops(st, r, t, mo, tok):
        for mi, terms in enumerate(LHS):
            _put(a2_s, (mo * 7 + mi, t), r, _lin(terms, st.get))

    def prep_x2(r, t, mo):
        st = {}
        return [(18, part(x_sum, st, r, t, mo, qi)) for qi in range(4)] + [(7, part(x_ops, st, r, t, mo))]

    def b1_at(slot, m, t):
        return b1_s[t // 2], (slot, m, t % 2)

    def g_at(slot, mo, mi, n):
        g = ORDER.index(mo)
        return (g_s[0], (slot, g * 7 + mi, n)) if g < GA else (g_s[1], (slot, (g - GA) * 7 + mi, n))

    def qkv_cols(st, src, k, n, hf, tok):
        tie_w(tok)
        st[hf] = _perm_lanes([pltpu.bitcast(w_v[2 * src + hf, _rows(k, n), pl.ds(j * 128, 128)], U32)
                              for j in range(8)])

    def qkv_ops(st, slot, k, t, tok):
        qs = [pltpu.bitcast(st[hf][t + c], BF16).astype(F32) for hf in range(2) for c in (0, 4)]
        for m, terms in enumerate(RHS):
            _put(*b1_at(slot, m, t), k, _lin(terms, qs.__getitem__))

    def prep_qkv(src, slot, k, rows, n=16, tiles=range(4)):
        jobs = []
        for r in range(0, rows, n):
            st = {}
            jobs.append([[(20, part(qkv_cols, st, src, k + r, n, hf)) for hf in range(2)],
                         [(28, part(qkv_ops, st, slot, k + r, t)) for t in tiles]])
        return _pipeline(jobs, 1)

    def wo_rows(st, h, jh, c, i, tok):
        tie_w(tok)
        st[i] = _perm_words([pltpu.bitcast(w_v[2 * O_ + jh, _rows(jl * 128 + h * 32 + (i // 2 ^ jh) * 16, 16),
                                               pl.ds(i % 2 * DHF + c * 128, 128)], U32) for jl in range(4)])

    def wo_ops(st, h, jh, c, tl, tok):
        qs = [pltpu.bitcast(st[i][tl], BF16).astype(F32) for i in range(4)]
        for m, terms in enumerate(RHS):
            _put(*b1_at(1, m, c), tl * 128 + h * 32 + jh * 16, _lin(terms, qs.__getitem__))

    def prep_wo(h, jh, c):
        st = {}
        return ([(15, part(wo_rows, st, h, jh, c, i)) for i in range(4)] +
                [(25, part(wo_ops, st, h, jh, c, i)) for i in range(4)])

    def gu_sum(st, src, k, n, mo, tok):
        tie_w(tok)
        block = lambda qo, qi: w_v[src + qo // 2, _rows(k + qi // 2 * 256, 16),
                                   pl.ds(n * FC + qo % 2 * 256 + qi % 2 * 128, 128)].astype(F32)
        st["q"] = [_lin(RHS[mo], lambda qo: block(qo, qi)) for qi in range(4)]

    def gu_ops(st, slot, k, n, mo, inner, tok):
        for mi in inner:
            _put(*g_at(slot, mo, mi, n), k, _lin(RHS[mi], st["q"].__getitem__))

    def prep_gu(src, slot, k, n, mo):
        st = {}
        return [(24, part(gu_sum, st, src, k, n, mo)),
                (6, part(gu_ops, st, slot, k, n, mo, (0, 1, 2, 3))), (6, part(gu_ops, st, slot, k, n, mo, (4, 5, 6)))]

    def prep_down(src, slot, k, t, tok):
        tie_w(tok)
        qs = [w_v[src, _rows(k + r0, 16), pl.ds(t * 128 + c0, 128)].astype(F32)
              for r0 in (0, FC // 2) for c0 in (0, DHF)]
        for m, terms in enumerate(RHS):
            _put(b2_s, (slot, m, t), k, _lin(terms, qs.__getitem__))

    def prep_glu(src_gu, src_d, slot, i, n):
        kk = 256 // n
        gu = [[x for r in range(0, kk, 16) for c in range(2) for mo in outer
               for x in prep_gu(src_gu, slot, i * kk + r, c, mo)] for outer in (ORDER[:GA], ORDER[GA:])]
        return gu[0], gu[1], [(25, part(prep_down, src_d, slot, i * kk + r, t))
                              for r in range(0, kk, 16) for t in range(4)]

    def lane_add(x, bit):
        lane = jax.lax.broadcasted_iota(jnp.int32, x.shape, 1)
        return x + jnp.take_along_axis(x, lane ^ bit, axis=1)

    def qk(st, r, t0, tok):
        tie_qkv(tok)
        for t in range(t0, t0 + 4):
            q = qkv_s[Q_, t, pl.ds(r + HALO, 8), :]
            ys = [q * qkv_s[K_, t, pl.ds(r + (HALO - DIL * w), 8), :] for w in range(W)]
            st["l"] = ys if t == 0 else [l + y for l, y in zip(st["l"], ys)]
        if t0:
            st["l"] = [lane_add(l, 1) for l in st["l"]]

    def logits(st, r, edge, tok):
        row = r + jax.lax.broadcasted_iota(jnp.int32, (8, 128), 0)
        ls = [lane_add(l, 2) * DH ** -0.5 for l in st["l"]]
        st["l"] = [jnp.where(row >= DIL * w, l, -1e9) if edge and w else l for w, l in enumerate(ls)]

    def softmax(st, tok):
        mx = functools.reduce(jnp.maximum, st["l"])
        es = [jnp.exp(l - mx) for l in st["l"]]
        inv = 1.0 / functools.reduce(jnp.add, es)
        st["p"] = [e * inv for e in es]

    def pv(st, r, s, hf, sub, t0, tok):
        tie_qkv(tok)
        for t in range(t0, t0 + 4):
            t_s[s, hf, t, pl.ds(sub, 8), :] = functools.reduce(
                jnp.add, [st["p"][w] * qkv_s[V_, t, pl.ds(r + (HALO - DIL * w), 8), :] for w in range(W)])

    def attn_ops(p, s, t, tok):
        t_s[2, 0, 0, _ds(zero(), 8, 8), :] = tok
        qs = [t_s[s, hf, t + c] for hf in range(2) for c in (0, 4)]
        for m, terms in enumerate(LHS):
            _put(a_s, (m, t), p, _lin(terms, qs.__getitem__))

    def attend(ps):
        out, late = [], []
        for i, p in enumerate(ps):
            for hf in range(2):
                for sub in (0, 8):
                    st, r = {}, hf * SH + p + sub
                    out += [(64, part(qk, st, r, t0)) for t0 in (0, 4)] + late[:len(late) // 2]
                    out += [(30, part(logits, st, r, (i, hf) == (0, 0)))] + late[len(late) // 2:]
                    out += [(55, part(softmax, st))]
                    late = [(60, part(pv, st, r, i % 2, hf, sub, t0)) for t0 in (0, 4)]
            late += [(17, part(attn_ops, p, i % 2, t)) for t in range(4)]
        return out + late

    def project(u, slot, p, n):
        ms = {}

        def dot(m, t):
            r = p + (0 if isinstance(p, int) else zero())
            ms[m] = _mm([_get(a_s, (m, i), r, n) for i in range(4)], [_get(*b1_at(slot, m, t))])
            for r in range(0, n, 32) if m in DONE else ():
                i = DONE[m]
                qkv_s[u, (i % 2) * 4 + t, _ds(HALO + (i // 2) * SH + p + r, 32, 8), :] = _lin(
                    OUT[i], lambda j: ms[j][r:r + 32])
            return ms[m]
        share = (1, 0.7, 1.1, 0.7, 1.1, 0.8, 0.7)
        return _quiet_tail([(share[i], part(dot, m, t)) for t in range(4) for i, m in enumerate(ORDER)])

    def project_slice(ks, p, n, m):
        y = _mm([_get(a_s, (m, s), p, n) for s in ks],
                [_get(*b1_at(0, m, t), ks[0] * 128, len(ks) * 128) for t in range(4)])
        for t in range(4):
            at = lambda j: (V_, t, pl.ds(j * 2 * XB + p, n))
            v = y[:, t * 128:(t + 1) * 128]
            if ks[0]:
                v = qkv_s[at(m)] + v
            if ks[-1] < 3 or m not in ORDER[-2:]:
                qkv_s[at(m)] = v
            if ks[-1] == 3 and m in DONE:
                i = DONE[m]
                qkv_s[K_, (i % 2) * 4 + t, pl.ds(HALO + (i // 2) * SH + p, n), :] = _lin(
                    OUT[i], lambda j: v if j == m else qkv_s[at(j)])
        return y

    def glu(slot, r0, first):
        n = P // 2
        inner, hs = {}, {}
        again = zero() * 2

        def up(mo, mi):
            r = r0 + zero()
            y = inner[mi] = _mm([_get(a2_s, (mo * 7 + mi, i), r, n) for i in range(2)],
                                [_get(*g_at(slot, mo, mi, i)) for i in range(2)])
            for r in range(0, n, 16) if mi in DONE else ():
                ci = DONE[mi]
                vs = [_lin(OUT[ci], lambda j: inner[j][r:r + 16, c:c + 128]) for c in (0, 128)]
                if mo not in ORDER[-2:]:
                    for i in range(2):
                        m_s[mo, pl.ds((2 * ci + i) * n + r, 16), :] = vs[i]
                if mo in DONE:
                    co = DONE[mo]
                    r1 = r + again if co == 3 else r
                    g, u = (_lin(OUT[co], lambda j: vs[i] if j == mo else m_s[j, _rows((2 * ci + i) * n + r1, 16), :])
                            for i in range(2))
                    hs[co, ci, r] = g * u
                    for j, terms in enumerate(LHS):
                        need = [i for i, _ in terms]
                        if co in need and all((i, ci, r) in hs for i in need):
                            _put(h_s, (j, ci % 2), ci // 2 * n + r, _lin(terms, lambda i: hs[i, ci, r]))
            return y

        def down(m, t):
            r = zero() * 4 if t else 0
            y = _mm([_get(h_s, (m, i), r, P) for i in range(2)], [_get(b2_s, (slot, m, t + i)) for i in range(2)])
            for hf in range(2):
                idx = (m, _rows(r0 + hf * (SH // 2), n), pl.ds(t * 128, 256))
                acc_s[idx] = jnp.where(first, 0.0, acc_s[idx]) + y[hf * n:(hf + 1) * n]
            return y
        so, si, sd = (0.9, 1, 1, 1, 1, 0.8, 0.4), (1, 0.8, 1.1, 0.8, 1.1, 1, 0.9), (0.7, 1, 1, 1, 0.8, 0.7, 0)
        return ([(so[k] * si[i], part(up, mo, mi)) for k, mo in enumerate(ORDER) for i, mi in enumerate(ORDER)],
                [(sd[k], part(down, m, t)) for k, m in enumerate((2, 4, 5, 3, 6, 1, 0)) for t in (0, 2)])

    for cp in (x_copy(0), k_copy(0), k_copy(1), x_copy(1), k_copy(2), k_copy(3)):
        cp.start()
    for b in range(2, SH // XB):
        x_copy(b).start()
    w_copy(Q_).start()
    w_copy(V_).start()
    for c in range(NCH):
        for cp in f_copies(c):
            cp.start()
    w_copy(O_).start()
    qkv_s[K_, :, pl.ds(0, HALO), :] = jnp.zeros((8, HALO, 128), F32)

    def first_rows(i, c):
        for _, f in layer_norm(i * (XB // 2), XB // 2):
            f(None)
        return (c + i) >> 1

    x_copy(0).wait()
    step[1] = jax.lax.fori_loop(0, 2, first_rows, 0)
    k_copy(0).wait()
    for _, f in prep_qkv(K_, 0, 0, 128, 32):
        f(None)
    for ks, p, n, s, blocks in (((0,), 0, XB, 1, ()), ((1,), 0, XB, 0, (1,)), ((0, 1), XB, XB, 2, ()),
                                ((2,), 0, 2 * XB, 3, (2,)), ((3,), 0, 2 * XB, 0, (3,)),
                                ((), 2 * XB, 2 * XB, 0, (4, 5, 6, 7))):
        side = []
        if s:
            k_copy(s).wait()
            side.append(prep_qkv(K_, 0, s * 128, 128))
        for b in blocks:
            x_copy(b).wait()
        if blocks:
            side.append(layer_norm(blocks[0] * XB, len(blocks) * XB))
        dots = _quiet_tail([(1, part(project_slice, ks, p, n, m)) for m in ORDER]) if ks else project(K_, 0, p, n)
        _interleave(dots, _merge(*side))

    w_copy(Q_).wait()

    @pl.loop(0, 5)
    def _(it):
        step[1] = it
        u, quarter = (it + 1) >> 1, jnp.maximum(it - 1, 0)

        @pl.when(it == 1)
        def _():
            w_copy(V_).wait()
            for cp in f_copies(0):
                cp.wait()

        nxt = [prep_qkv(jnp.minimum(u + 1, V_), 1 - (u & 1), 0, DHF, tiles=ts) for ts in ((0, 1), (2, 3))]
        ga, gb, dn = prep_glu(jnp.where(it == 0, 0, 2 * GU_), jnp.where(it == 0, 0, DN_), 0, quarter, 4)
        x2 = [x for r in range(0, 128, 16) for t in range(2) for mo in range(7)
              for x in prep_x2(quarter * 128 + r, t, mo)]
        rest = _merge(ga + gb, dn, x2)
        dots = project(u, u & 1, ((it + 1) & 1) * P, P)
        half = int(len(rest) * 0.526)
        _interleave(_quiet_tail(dots[:14]), _merge(nxt[1], rest[:half]))
        _interleave(dots[14:], _merge(nxt[0], rest[half:]))

    for t in range(8):
        qkv_s[V_, t, pl.ds(0, HALO), :] = jnp.broadcast_to(qkv_s[V_, t, pl.ds(HALO, 1), :], (HALO, 128))
    w_copy(O_).wait()
    for c in range(1, NCH):
        for cp in f_copies(c):
            cp.wait()

    @pl.loop(0, 2 * NCH)
    def _(it):
        step[1] = it
        c, b = it >> 1, it & 1
        nxt = jnp.minimum(c + 1, NCH - 1)
        extra = jnp.where(it < 8, it, 0)
        ga, gb, dn = prep_glu(2 * (GU_ + nxt), DN_ + nxt, 1 - (c & 1), b, 2)
        rest = _merge(attend([it * 64 + i * 16 for i in range(4)] + [2 * NCH * 64 + extra * 16]),
                      [x for t in range(4) for x in prep_wo(extra >> 1, extra & 1, t)])
        ups, downs = glu(c & 1, b * (P // 2), c == 0)
        h0, h1, g0 = int(len(rest) * 0.302), int(len(rest) * 0.897), int(len(ga) // 3 * 0.08) * 3
        _interleave(_quiet_tail(ups[:7 * GA]), _merge(gb, rest[:h0]))
        _interleave(_quiet_tail(ups[7 * GA:]), _merge(dn + ga[:g0], rest[h0:h1]))
        _interleave(downs, _merge(ga[g0:], rest[h1:]))

    @pl.loop(0, SH // P_OUT)
    def _(it):
        step[1] = it
        for j, n in enumerate(R_OUT):
            p = it * P_OUT + sum(R_OUT[:j])
            for t in range(4):
                r = p + zero()
                ms = [acc_s[m, _rows(p, n), pl.ds(t * 128, 128)] +
                      _mm([_get(a_s, (m, i), r, n) for i in range(4)], [_get(*b1_at(1, m, t))]) for m in range(7)]
                for i, terms in enumerate(OUT):
                    idx = (i // 2, _rows(p, n), pl.ds((i % 2) * DHF + t * 128, 128))
                    x_v[idx] = (x_v[idx].astype(F32) + _lin(terms, ms.__getitem__)).astype(BF16)
            o_copy(it, j).start()

    for i in range(SH // P_OUT):
        for j in range(len(R_OUT)):
            o_copy(i, j).wait()


@jax.jit
def pallas_parallel_sum__sliding_local_dilated__glu_gated_bilinear__prompt_kernel(
    A_x: jax.Array,
    A_wqkv: jax.Array,
    A_wo: jax.Array,
    B_x: jax.Array,
    B_w_gate: jax.Array,
    B_w_up: jax.Array,
    B_w_down: jax.Array,
):
    del B_x
    hbm = pl.BlockSpec(memory_space=pl.ANY)
    vmem, dma = pltpu.VMEM, pltpu.SemaphoreType.DMA
    operand = lambda *shape: vmem((*shape, 128), BF16)
    out = pl.pallas_call(
        _kernel,
        in_specs=[hbm] * 6,
        out_specs=hbm,
        out_shape=jax.ShapeDtypeStruct((2, SH, D), BF16),
        scratch_shapes=[
            vmem((2, SH + 16, D), BF16),
            vmem((DN_ + NCH, DHF + 16, D), BF16),
            operand(7, 4, SH),
            operand(49, 2, SH // 2),
            [operand(2, 7, 2, DHF)] * 2,
            [operand(2, 7 * GA, 2, 256), operand(2, 7 * (7 - GA), 2, 256)],
            operand(2, 7, 4, FC // 2),
            operand(7, 2, P),
            vmem((5, 4 * P, 128), F32),
            vmem((7, SH, DHF), F32),
            vmem((3, 8, S + HALO + 8, 128), F32),
            vmem((3, 2, 8, 16, 128), F32),
            dma((SH // XB,)), dma((4,)), dma((3,)), dma((1,)),
        ],
        compiler_params=pltpu.CompilerParams(vmem_limit_bytes=127 * 2**20,
                                             flags={"XLA_TPU_EVENLY_DISTRIBUTE_CRITICAL_NODES": True}),
        name="fused",
    )(A_x.reshape(2, SH, D), A_wqkv.reshape(2, DHF, 3 * D), A_wo.reshape(2, DHF, D),
      B_w_gate.reshape(2, DHF, F), B_w_up.reshape(2, DHF, F), B_w_down)
    return out.reshape(A_x.shape)
```

```python
import functools

import jax
import jax.numpy as jnp
import jax.experimental.pallas as pl
import jax.experimental.pallas.tpu as pltpu

S, D, F = 2048, 1024, 3584
DH, W, DIL = 32, 8, 2
HALO = 16
SH, DHF = S // 2, D // 2
FC = 512
NCH = F // FC
XB = 128
P = 512
P_OUT = 256
R_OUT = (192, 64)
GA = 3
F32, BF16, U32 = jnp.float32, jnp.bfloat16, jnp.uint32
K_, Q_, V_, O_, GU_ = 0, 1, 2, 3, 4
DN_ = 2 * (GU_ + NCH)

LHS = (((0, 1), (3, 1)), ((2, 1), (3, 1)), ((0, 1),), ((3, 1),),
       ((0, 1), (1, 1)), ((2, 1), (0, -1)), ((1, 1), (3, -1)))
RHS = (((0, 1), (3, 1)), ((0, 1),), ((1, 1), (3, -1)), ((2, 1), (0, -1)),
       ((3, 1),), ((0, 1), (1, 1)), ((2, 1), (3, 1)))
OUT = (((6, 1), (0, 1), (3, 1), (4, -1)), ((2, 1), (4, 1)),
       ((3, 1), (1, 1)), ((5, 1), (0, 1), (1, -1), (2, 1)))
ORDER = (1, 3, 4, 2, 0, 6, 5)
DONE = {3: 2, 2: 1, 6: 0, 5: 3}


def _lin(terms, get):
    acc = get(terms[0][0])
    for i, sign in terms[1:]:
        acc = acc + get(i) if sign > 0 else acc - get(i)
    return acc


def _ds(start, n, align):
    return pl.ds(start if isinstance(start, int) else pl.multiple_of(start, align), n)


def _rows(start, n):
    return _ds(start, n, 16)


def _put(ref, idx, start, v):
    ref[(*idx, _rows(start, v.shape[0]))] = v.astype(BF16)


def _get(ref, idx, start=0, n=None):
    words = ref.bitcast(U32)[(*idx, _ds(start >> 1, (n or ref.shape[-2]) // 2, 8))]
    return pltpu.bitcast(words, BF16)


def _mm(a, b):
    cat = lambda v: v[0] if len(v) == 1 else jnp.concatenate(v, axis=1)
    return jnp.dot(cat(a), cat(b), preferred_element_type=F32)


def _skew4(vs, pos, unit):
    cur = [vs[(-t) % 4] for t in range(4)]
    for b in (1, 2):
        m = (pos & (b * unit)) != 0
        cur = [jnp.where(m, cur[(t - b) % 4], cur[t]) for t in range(4)]
    return cur


def _perm_lanes(vs):
    lane = jax.lax.broadcasted_iota(jnp.int32, vs[0].shape, 1)
    lo, hi = _skew4(vs[:4], lane, 4), _skew4(vs[4:], lane, 4)
    m = (lane & 16) != 0
    mixed = [jnp.where(m, b, a) for a, b in zip(lo, hi)] + [jnp.where(m, a, b) for a, b in zip(lo, hi)]
    return [v if t == 0 else
            jnp.take_along_axis(v, ((lane & 115) ^ (t // 4 * 16)) | ((lane + t % 4 * 4) & 12), axis=1)
            for t, v in enumerate(mixed)]


def _perm_words(vs):
    row = jax.lax.broadcasted_iota(jnp.int32, vs[0].shape, 0)
    return [v if t == 0 else pltpu.roll(v, 8 - 2 * t, 0) for t, v in enumerate(_skew4(vs, row, 2))]


def _merge(*lists):
    keyed = []
    for xs in lists:
        tot, done = sum(w for w, _ in xs), 0
        for w, f in xs:
            keyed.append(((done + w / 2) / tot, w, f))
            done += w
    return [(w, f) for _, w, f in sorted(keyed, key=lambda t: t[0])]


def _pipeline(jobs, dist):
    n, out = len(jobs[0]), []
    for i in range(len(jobs) + (n - 1) * dist):
        for st in range(n):
            if 0 <= i - st * dist < len(jobs):
                out += jobs[i - st * dist][st]
    return out


def _interleave(dots, side):
    tot, share = sum(w for w, _ in side), sum(w for w, _ in dots)
    done, j, cum = 0, 0, 0
    for w, dot in dots:
        src = dot()
        lo = tot * cum / share
        cum += w
        hi = tot * cum / share
        while j < len(side) and done < hi - 1e-6:
            pos = min(max((done - lo) / (hi - lo), 0.0), 0.999) * (src.shape[1] // 128)
            r0, c0 = int(pos % 1 * src.shape[0]) // 8 * 8, int(pos) * 128
            side[j][1](src[r0:r0 + 8, c0:c0 + 128])
            done += side[j][0]
            j += 1
    assert j == len(side)


def _quiet_tail(dots):
    return dots[:-1] + [(0, dots[-1][1])]


def _kernel(x_hbm, wqkv_hbm, wo_hbm, wg_hbm, wu_hbm, wd_hbm, o_hbm,
            x_v, w_v, a_s, a2_s, b1_s, g_s, b2_s, h_s, m_s, acc_s, qkv_s, t_s,
            sem_x, sem_k, sem_w, sem_o):
    part = functools.partial
    step = [0, None]

    def zero():
        step[0] += 1
        return jax.lax.shift_right_logical(step[1] + step[0], 24) * 16

    def tie_x(tok):
        if tok is not None:
            x_v[0, _rows(zero() + SH, 16), pl.ds(0, 128)] = pltpu.bitcast(tok, BF16)

    def tie_w(tok):
        if tok is not None:
            w_v[0, _rows(zero() + DHF, 16), pl.ds(0, 128)] = pltpu.bitcast(tok, BF16)

    def tie_qkv(tok):
        qkv_s[0, 0, _ds(zero() + S + HALO, 8, 8), :] = tok

    def x_copy(b):
        rows = _rows(b * XB, XB)
        return pltpu.make_async_copy(x_hbm.at[:, rows], x_v.at[:, rows], sem_x.at[min(b, 4)])

    def k_copy(s):
        rows = pl.ds(s * 128, 128)
        return pltpu.make_async_copy(wqkv_hbm.at[:, rows, pl.ds(D, D)], w_v.at[pl.ds(2 * K_, 2), rows], sem_k.at[s])

    def w_copy(i):
        src = wo_hbm if i == O_ else wqkv_hbm.at[:, :, pl.ds(0 if i == Q_ else 2 * D, D)]
        return pltpu.make_async_copy(src, w_v.at[pl.ds(2 * i, 2), pl.ds(0, DHF)], sem_w.at[i - Q_])

    def f_copies(c):
        col, dst, rows = pl.ds(c * FC, FC), pl.ds(2 * (GU_ + c), 2), pl.ds(0, DHF)
        sem = sem_w.at[(O_ if c else V_) - Q_]
        return [pltpu.make_async_copy(wg_hbm.at[:, :, col], w_v.at[dst, rows, pl.ds(0, FC)], sem),
                pltpu.make_async_copy(wu_hbm.at[:, :, col], w_v.at[dst, rows, pl.ds(FC, FC)], sem),
                pltpu.make_async_copy(wd_hbm.at[col, :], w_v.at[DN_ + c, rows], sem)]

    def o_copy(i, j):
        rows = _rows(i * P_OUT + sum(R_OUT[:j]), R_OUT[j])
        return pltpu.make_async_copy(x_v.at[:, rows], o_hbm.at[:, rows], sem_o.at[0])

    def row_mean(x):
        y = functools.reduce(jnp.add, [x[:, c:c + 128] for c in range(0, D, 128)])
        return jnp.sum(y, axis=-1, keepdims=True) * (1.0 / D)

    def ln_stats(st, p, hf, tok):
        tie_x(tok)
        x = x_v[hf, _rows(p, 16), :].astype(F32)
        mu = row_mean(x)
        xc = x - mu
        st[hf] = (mu, jax.lax.rsqrt(row_mean(xc * xc) + 1e-5))
        for i in range(2):
            acc_s[0, _rows(p, 16), pl.ds(i * 256 + hf * 128, 128)] = jnp.broadcast_to(st[hf][i], (16, 128))

    def ln_ops(st, p, t, tok):
        tie_x(tok)
        qs = [(x_v[hf, _rows(p, 16), pl.ds(c + t * 128, 128)].astype(F32) - st[hf][0]) * st[hf][1]
              for hf in range(2) for c in (0, DHF)]
        for m, terms in enumerate(LHS):
            _put(a_s, (m, t), p, _lin(terms, qs.__getitem__))

    def layer_norm(p, n):
        jobs = []
        for r in range(0, n, 16):
            st = {}
            jobs.append([[(90, part(ln_stats, st, p + r, hf)) for hf in range(2)],
                         [(45, part(ln_ops, st, p + r, t)) for t in range(4)]])
        return _pipeline(jobs, 6)

    def x_sum(st, r, t, mo, qi, tok):
        tie_x(tok)
        rows = _rows(qi // 2 * (SH // 2) + r, 16)

        def block(qo):
            x = x_v[qo // 2, rows, pl.ds(qo % 2 * DHF + qi % 2 * 256 + t * 128, 128)].astype(F32)
            return (x - acc_s[0, rows, pl.ds(qo // 2 * 128, 128)]) * acc_s[0, rows, pl.ds(256 + qo // 2 * 128, 128)]
        st[qi] = _lin(LHS[mo], block)

    def x_ops(st, r, t, mo, tok):
        for mi, terms in enumerate(LHS):
            _put(a2_s, (mo * 7 + mi, t), r, _lin(terms, st.get))

    def prep_x2(r, t, mo):
        st = {}
        return [(10, part(x_sum, st, r, t, mo, qi)) for qi in range(4)] + [(7, part(x_ops, st, r, t, mo))]

    def b1_at(slot, m, t):
        return b1_s[t // 2], (slot, m, t % 2)

    def g_at(slot, mo, mi, n):
        g = ORDER.index(mo)
        return (g_s[0], (slot, g * 7 + mi, n)) if g < GA else (g_s[1], (slot, (g - GA) * 7 + mi, n))

    def qkv_cols(st, src, k, n, hf, tok):
        tie_w(tok)
        st[hf] = _perm_lanes([pltpu.bitcast(w_v[2 * src + hf, _rows(k, n), pl.ds(j * 128, 128)], U32)
                              for j in range(8)])

    def qkv_ops(st, slot, k, t, tok):
        qs = [pltpu.bitcast(st[hf][t + c], BF16).astype(F32) for hf in range(2) for c in (0, 4)]
        for m, terms in enumerate(RHS):
            _put(*b1_at(slot, m, t), k, _lin(terms, qs.__getitem__))

    def prep_qkv(src, slot, k, rows, n=16, tiles=range(4)):
        jobs = []
        for r in range(0, rows, n):
            st = {}
            jobs.append([[(15, part(qkv_cols, st, src, k + r, n, hf)) for hf in range(2)],
                         [(28, part(qkv_ops, st, slot, k + r, t)) for t in tiles]])
        return _pipeline(jobs, 1)

    def wo_rows(st, h, jh, c, i, tok):
        tie_w(tok)
        st[i] = _perm_words([pltpu.bitcast(w_v[2 * O_ + jh, _rows(jl * 128 + h * 32 + (i // 2 ^ jh) * 16, 16),
                                               pl.ds(i % 2 * DHF + c * 128, 128)], U32) for jl in range(4)])

    def wo_ops(st, h, jh, c, tl, tok):
        qs = [pltpu.bitcast(st[i][tl], BF16).astype(F32) for i in range(4)]
        for m, terms in enumerate(RHS):
            _put(*b1_at(1, m, c), tl * 128 + h * 32 + jh * 16, _lin(terms, qs.__getitem__))

    def prep_wo(h, jh, c):
        st = {}
        return ([(15, part(wo_rows, st, h, jh, c, i)) for i in range(4)] +
                [(25, part(wo_ops, st, h, jh, c, i)) for i in range(4)])

    def gu_sum(st, src, k, n, mo, tok):
        tie_w(tok)
        block = lambda qo, qi: w_v[src + qo // 2, _rows(k + qi // 2 * 256, 16),
                                   pl.ds(n * FC + qo % 2 * 256 + qi % 2 * 128, 128)].astype(F32)
        st["q"] = [_lin(RHS[mo], lambda qo: block(qo, qi)) for qi in range(4)]

    def gu_ops(st, slot, k, n, mo, inner, tok):
        for mi in inner:
            _put(*g_at(slot, mo, mi, n), k, _lin(RHS[mi], st["q"].__getitem__))

    def prep_gu(src, slot, k, n, mo):
        st = {}
        return [(24, part(gu_sum, st, src, k, n, mo)),
                (6, part(gu_ops, st, slot, k, n, mo, (0, 1, 2, 3))), (6, part(gu_ops, st, slot, k, n, mo, (4, 5, 6)))]

    def prep_down(src, slot, k, t, tok):
        tie_w(tok)
        qs = [w_v[src, _rows(k + r0, 16), pl.ds(t * 128 + c0, 128)].astype(F32)
              for r0 in (0, FC // 2) for c0 in (0, DHF)]
        for m, terms in enumerate(RHS):
            _put(b2_s, (slot, m, t), k, _lin(terms, qs.__getitem__))

    def prep_glu(src_gu, src_d, slot, i, n):
        kk = 256 // n
        gu = [[x for r in range(0, kk, 16) for c in range(2) for mo in outer
               for x in prep_gu(src_gu, slot, i * kk + r, c, mo)] for outer in (ORDER[:GA], ORDER[GA:])]
        return gu[0], gu[1], [(25, part(prep_down, src_d, slot, i * kk + r, t))
                              for r in range(0, kk, 16) for t in range(4)]

    def lane_add(x, bit):
        lane = jax.lax.broadcasted_iota(jnp.int32, x.shape, 1)
        return x + jnp.take_along_axis(x, lane ^ bit, axis=1)

    def qk(st, r, t0, tok):
        tie_qkv(tok)
        for t in range(t0, t0 + 4):
            q = qkv_s[Q_, t, pl.ds(r + HALO, 8), :]
            ys = [q * qkv_s[K_, t, pl.ds(r + (HALO - DIL * w), 8), :] for w in range(W)]
            st["l"] = ys if t == 0 else [l + y for l, y in zip(st["l"], ys)]
        if t0:
            st["l"] = [lane_add(l, 1) for l in st["l"]]

    def logits(st, r, edge, tok):
        row = r + jax.lax.broadcasted_iota(jnp.int32, (8, 128), 0)
        ls = [lane_add(l, 2) * DH ** -0.5 for l in st["l"]]
        st["l"] = [jnp.where(row >= DIL * w, l, -1e9) if edge and w else l for w, l in enumerate(ls)]

    def softmax(st, tok):
        mx = functools.reduce(jnp.maximum, st["l"])
        es = [jnp.exp(l - mx) for l in st["l"]]
        inv = 1.0 / functools.reduce(jnp.add, es)
        st["p"] = [e * inv for e in es]

    def pv(st, r, s, hf, sub, t0, tok):
        tie_qkv(tok)
        for t in range(t0, t0 + 4):
            t_s[s, hf, t, pl.ds(sub, 8), :] = functools.reduce(
                jnp.add, [st["p"][w] * qkv_s[V_, t, pl.ds(r + (HALO - DIL * w), 8), :] for w in range(W)])

    def attn_ops(p, s, t, tok):
        t_s[2, 0, 0, _ds(zero(), 8, 8), :] = tok
        qs = [t_s[s, hf, t + c] for hf in range(2) for c in (0, 4)]
        for m, terms in enumerate(LHS):
            _put(a_s, (m, t), p, _lin(terms, qs.__getitem__))

    def attend(ps):
        out, late = [], []
        for i, p in enumerate(ps):
            for hf in range(2):
                for sub in (0, 8):
                    st, r = {}, hf * SH + p + sub
                    out += [(64, part(qk, st, r, t0)) for t0 in (0, 4)] + late[:len(late) // 2]
                    out += [(30, part(logits, st, r, (i, hf) == (0, 0)))] + late[len(late) // 2:]
                    out += [(55, part(softmax, st))]
                    late = [(60, part(pv, st, r, i % 2, hf, sub, t0)) for t0 in (0, 4)]
            late += [(17, part(attn_ops, p, i % 2, t)) for t in range(4)]
        return out + late

    def project(u, slot, p, n):
        ms = {}

        def dot(m, t):
            r = p + (0 if isinstance(p, int) else zero())
            ms[m] = _mm([_get(a_s, (m, i), r, n) for i in range(4)], [_get(*b1_at(slot, m, t))])
            for r in range(0, n, 32) if m in DONE else ():
                i = DONE[m]
                qkv_s[u, (i % 2) * 4 + t, _ds(HALO + (i // 2) * SH + p + r, 32, 8), :] = _lin(
                    OUT[i], lambda j: ms[j][r:r + 32])
            return ms[m]
        share = (1, 0.8, 1.1, 0.8, 1.1, 0.8, 0.8)
        return _quiet_tail([(share[i], part(dot, m, t)) for t in range(4) for i, m in enumerate(ORDER)])

    def project_slice(ks, p, n, m):
        y = _mm([_get(a_s, (m, s), p, n) for s in ks],
                [_get(*b1_at(0, m, t), ks[0] * 128, len(ks) * 128) for t in range(4)])
        for t in range(4):
            at = lambda j: (V_, t, pl.ds(j * 2 * XB + p, n))
            v = y[:, t * 128:(t + 1) * 128]
            if ks[0]:
                v = qkv_s[at(m)] + v
            if ks[-1] < 3 or m not in ORDER[-2:]:
                qkv_s[at(m)] = v
            if ks[-1] == 3 and m in DONE:
                i = DONE[m]
                qkv_s[K_, (i % 2) * 4 + t, pl.ds(HALO + (i // 2) * SH + p, n), :] = _lin(
                    OUT[i], lambda j: v if j == m else qkv_s[at(j)])
        return y

    def glu(slot, r0, first):
        n = P // 2
        inner, hs = {}, {}
        again = zero() * 2

        def up(mo, mi):
            r = r0 + zero()
            y = inner[mi] = _mm([_get(a2_s, (mo * 7 + mi, i), r, n) for i in range(2)],
                                [_get(*g_at(slot, mo, mi, i)) for i in range(2)])
            for r in range(0, n, 16) if mi in DONE else ():
                ci = DONE[mi]
                vs = [_lin(OUT[ci], lambda j: inner[j][r:r + 16, c:c + 128]) for c in (0, 128)]
                if mo not in ORDER[-2:]:
                    for i in range(2):
                        m_s[mo, pl.ds((2 * ci + i) * n + r, 16), :] = vs[i]
                if mo in DONE:
                    co = DONE[mo]
                    r1 = r + again if co == 3 else r
                    g, u = (_lin(OUT[co], lambda j: vs[i] if j == mo else m_s[j, _rows((2 * ci + i) * n + r1, 16), :])
                            for i in range(2))
                    hs[co, ci, r] = g * u
                    for j, terms in enumerate(LHS):
                        need = [i for i, _ in terms]
                        if co in need and all((i, ci, r) in hs for i in need):
                            _put(h_s, (j, ci % 2), ci // 2 * n + r, _lin(terms, lambda i: hs[i, ci, r]))
            return y

        def down(m, t):
            r = zero() * 4 if t else 0
            y = _mm([_get(h_s, (m, i), r, P) for i in range(2)], [_get(b2_s, (slot, m, t + i)) for i in range(2)])
            for hf in range(2):
                idx = (m, _rows(r0 + hf * (SH // 2), n), pl.ds(t * 128, 256))
                acc_s[idx] = jnp.where(first, 0.0, acc_s[idx]) + y[hf * n:(hf + 1) * n]
            return y
        so, si, sd = (0.9, 1, 1, 1, 1, 0.8, 0.4), (1, 0.8, 1.1, 0.8, 1.1, 1, 0.9), (0.7, 1, 1, 1, 0.8, 0.7, 0)
        return ([(so[k] * si[i], part(up, mo, mi)) for k, mo in enumerate(ORDER) for i, mi in enumerate(ORDER)],
                [(sd[k], part(down, m, t)) for k, m in enumerate((2, 4, 5, 3, 6, 1, 0)) for t in (0, 2)])

    for cp in (x_copy(0), k_copy(0), k_copy(1), x_copy(1), k_copy(2), k_copy(3)):
        cp.start()
    for b in range(2, SH // XB):
        x_copy(b).start()
    w_copy(Q_).start()
    w_copy(V_).start()
    for c in range(NCH):
        for cp in f_copies(c):
            cp.start()
    w_copy(O_).start()
    qkv_s[K_, :, pl.ds(0, HALO), :] = jnp.zeros((8, HALO, 128), F32)

    def first_rows(i, c):
        for _, f in layer_norm(i * (XB // 2), XB // 2):
            f(None)
        return (c + i) >> 1

    x_copy(0).wait()
    step[1] = jax.lax.fori_loop(0, 2, first_rows, 0)
    k_copy(0).wait()
    for _, f in prep_qkv(K_, 0, 0, 128, 32):
        f(None)
    for ks, p, n, s, blocks in (((0,), 0, XB, 1, ()), ((1,), 0, XB, 0, (1,)), ((0, 1), XB, XB, 2, ()),
                                ((2,), 0, 2 * XB, 3, (2,)), ((3,), 0, 2 * XB, 0, (3,)),
                                ((), 2 * XB, 2 * XB, 0, (4, 5, 6, 7))):
        side = []
        if s:
            k_copy(s).wait()
            side.append(prep_qkv(K_, 0, s * 128, 128))
        for b in blocks:
            x_copy(b).wait()
        if blocks:
            side.append(layer_norm(blocks[0] * XB, len(blocks) * XB))
        dots = _quiet_tail([(1, part(project_slice, ks, p, n, m)) for m in ORDER]) if ks else project(K_, 0, p, n)
        _interleave(dots, _merge(*side))

    w_copy(Q_).wait()

    @pl.loop(0, 5)
    def _(it):
        step[1] = it
        u, quarter = (it + 1) >> 1, jnp.maximum(it - 1, 0)

        @pl.when(it == 1)
        def _():
            w_copy(V_).wait()
            for cp in f_copies(0):
                cp.wait()

        nxt = [prep_qkv(jnp.minimum(u + 1, V_), 1 - (u & 1), 0, DHF, tiles=ts) for ts in ((0, 1), (2, 3))]
        ga, gb, dn = prep_glu(jnp.where(it == 0, 0, 2 * GU_), jnp.where(it == 0, 0, DN_), 0, quarter, 4)
        x2 = [x for r in range(0, 128, 16) for t in range(2) for mo in range(7)
              for x in prep_x2(quarter * 128 + r, t, mo)]
        rest = _merge(ga + gb, dn, x2)
        dots = project(u, u & 1, ((it + 1) & 1) * P, P)
        half = int(len(rest) * 0.457)
        _interleave(_quiet_tail(dots[:14]), _merge(nxt[1], rest[:half]))
        _interleave(dots[14:], _merge(nxt[0], rest[half:]))

    for t in range(8):
        qkv_s[V_, t, pl.ds(0, HALO), :] = jnp.broadcast_to(qkv_s[V_, t, pl.ds(HALO, 1), :], (HALO, 128))
    w_copy(O_).wait()
    for c in range(1, NCH):
        for cp in f_copies(c):
            cp.wait()

    @pl.loop(0, 2 * NCH)
    def _(it):
        step[1] = it
        c, b = it >> 1, it & 1
        nxt = jnp.minimum(c + 1, NCH - 1)
        extra = jnp.where(it < 8, it, 0)
        ga, gb, dn = prep_glu(2 * (GU_ + nxt), DN_ + nxt, 1 - (c & 1), b, 2)
        rest = _merge(attend([it * 64 + i * 16 for i in range(4)] + [2 * NCH * 64 + extra * 16]),
                      [x for t in range(4) for x in prep_wo(extra >> 1, extra & 1, t)])
        ups, downs = glu(c & 1, b * (P // 2), c == 0)
        h0, h1, g0 = int(len(rest) * 0.302), int(len(rest) * 0.897), int(len(ga) // 3 * 0.08) * 3
        _interleave(_quiet_tail(ups[:7 * GA]), _merge(gb, rest[:h0]))
        _interleave(_quiet_tail(ups[7 * GA:]), _merge(dn + ga[:g0], rest[h0:h1]))
        _interleave(downs, _merge(ga[g0:], rest[h1:]))

    @pl.loop(0, SH // P_OUT)
    def _(it):
        step[1] = it
        for j, n in enumerate(R_OUT):
            p = it * P_OUT + sum(R_OUT[:j])
            for t in range(4):
                r = p + zero()
                ms = [acc_s[m, _rows(p, n), pl.ds(t * 128, 128)] +
                      _mm([_get(a_s, (m, i), r, n) for i in range(4)], [_get(*b1_at(1, m, t))]) for m in range(7)]
                for i, terms in enumerate(OUT):
                    idx = (i // 2, _rows(p, n), pl.ds((i % 2) * DHF + t * 128, 128))
                    x_v[idx] = (x_v[idx].astype(F32) + _lin(terms, ms.__getitem__)).astype(BF16)
            o_copy(it, j).start()

    for i in range(SH // P_OUT):
        for j in range(len(R_OUT)):
            o_copy(i, j).wait()


@jax.jit
def pallas_parallel_sum__sliding_local_dilated__glu_gated_bilinear__prompt_kernel(
    A_x: jax.Array,
    A_wqkv: jax.Array,
    A_wo: jax.Array,
    B_x: jax.Array,
    B_w_gate: jax.Array,
    B_w_up: jax.Array,
    B_w_down: jax.Array,
):
    del B_x
    hbm = pl.BlockSpec(memory_space=pl.ANY)
    vmem, dma = pltpu.VMEM, pltpu.SemaphoreType.DMA
    operand = lambda *shape: vmem((*shape, 128), BF16)
    out = pl.pallas_call(
        _kernel,
        in_specs=[hbm] * 6,
        out_specs=hbm,
        out_shape=jax.ShapeDtypeStruct((2, SH, D), BF16),
        scratch_shapes=[
            vmem((2, SH + 16, D), BF16),
            vmem((DN_ + NCH, DHF + 16, D), BF16),
            operand(7, 4, SH),
            operand(49, 2, SH // 2),
            [operand(2, 7, 2, DHF)] * 2,
            [operand(2, 7 * GA, 2, 256), operand(2, 7 * (7 - GA), 2, 256)],
            operand(2, 7, 4, FC // 2),
            operand(7, 2, P),
            vmem((5, 4 * P, 128), F32),
            vmem((7, SH, DHF), F32),
            vmem((3, 8, S + HALO + 8, 128), F32),
            vmem((3, 2, 8, 16, 128), F32),
            dma((5,)), dma((4,)), dma((3,)), dma((1,)),
        ],
        compiler_params=pltpu.CompilerParams(vmem_limit_bytes=127 * 2**20,
                                             flags={"XLA_TPU_EVENLY_DISTRIBUTE_CRITICAL_NODES": True}),
        name="fused",
    )(A_x.reshape(2, SH, D), A_wqkv.reshape(2, DHF, 3 * D), A_wo.reshape(2, DHF, D),
      B_w_gate.reshape(2, DHF, F), B_w_up.reshape(2, DHF, F), B_w_down)
    return out.reshape(A_x.shape)
```
